```python
import os as _os
_os.environ.setdefault("JAX_PLATFORMS", "cpu")
import jax
import jax.numpy as jnp

def _softmax(x, axis=-1):
    return jax.nn.softmax(x, axis=axis)
def _gelu(x):
    return jax.nn.gelu(x, approximate=True)
def _silu(x):
    return jax.nn.silu(x)
def _sigmoid(x):
    return jax.nn.sigmoid(x)
def _layernorm(x, axis=-1, eps=1e-5):
    m = jnp.mean(x, axis=axis, keepdims=True)
    v = jnp.var(x, axis=axis, keepdims=True)
    return (x - m) / jnp.sqrt(v + eps)
def _scatter_add(tgt, idx, src, axis=0):
    return tgt.at[idx].add(src)
def _segment_sum(src, seg, n):
    return jax.ops.segment_sum(src, seg, n)
class _Rng:
    def __init__(self, key):
        self._k = key
    def _next(self):
        self._k, sub = jax.random.split(self._k)
        return sub
    def normal(self, shape):
        return jax.random.normal(self._next(), shape, dtype=jnp.bfloat16)
    def randint(self, lo, hi, shape):
        return jax.random.randint(self._next(), shape, lo, hi, dtype=jnp.int32)
    def uniform(self, shape, lo=0.0, hi=1.0):
        return jax.random.uniform(self._next(), shape, jnp.bfloat16, lo, hi)
    def permutation(self, n):
        return jax.random.permutation(self._next(), n)


kernel_name = 'interleave_layers__gqa_block_cached__dense_activation_silu__decode'

def setup_inputs():
    _rng = _Rng(jax.random.key(int.from_bytes(__import__("os").urandom(4), "little")))
    _w = (lambda a: (lambda t: t.astype(jnp.bfloat16) if jnp.issubdtype(t.dtype, jnp.floating) else t)(jnp.asarray(a)))
    def _A_setup():
        B, Sq, D = 2, 1, 512
        Hq, Hkv, Sk, Dh = 32, 8, 8192, 128
        assert Hq % Hkv == 0, (Hq, Hkv)
        return {
            "x": _w((lambda *s: _rng.normal(s) * 0.1)(B, Sq, D)),
            "k_cache": _w((lambda *s: _rng.normal(s) * 0.8)(B, Hkv, Sk, Dh)),
            "v_cache": _w((lambda *s: _rng.normal(s) * 1.6)(B, Hkv, Sk, Dh)),
            "wq": _w((lambda *s: _rng.normal(s) * 0.8)(D, Hq * Dh) * (D ** -0.5)),
            "wo": _w((lambda *s: _rng.normal(s) * 1.6)(Hq * Dh, D) * ((Hq * Dh) ** -0.5)),
        }
    _A_in = _A_setup()

    def _B_setup():
        B, S, D, F = 2, 1, 512, 1792
        return {
            "x": _w((lambda *s: _rng.normal(s) * 0.1)(B, S, D)),
            "w1": _w((lambda *s: _rng.normal(s) * 0.4)(D, F) * (D ** -0.5)),
            "w2": _w((lambda *s: _rng.normal(s) * 0.4)(F, D) * (F ** -0.5)),
        }
    _B_in = _B_setup()

    return {
        "A_x": _A_in["x"],
        "A_k_cache": _A_in["k_cache"],
        "A_v_cache": _A_in["v_cache"],
        "A_wq": _A_in["wq"],
        "A_wo": _A_in["wo"],
        "B_x": _B_in["x"],
        "B_w1": _B_in["w1"],
        "B_w2": _B_in["w2"],
    }

def reference(A_x, A_k_cache, A_v_cache, A_wq, A_wo, B_x, B_w1, B_w2):
    def _A_ref(x, k_cache, v_cache, wq, wo):
        B, Sq, D = x.shape
        Hq, Dh = 32, 128
        Hkv = k_cache.shape[1]
        rep = Hq // Hkv
        q = (lambda x, *d: x.transpose(*d))((x @ wq).reshape(B, Sq, Hq, Dh), 0, 2, 1, 3)
        k = jnp.repeat(k_cache, rep, axis=1)
        v = jnp.repeat(v_cache, rep, axis=1)
        scores = jnp.einsum("bhqd,bhkd->bhqk", q, k) * (Dh ** -0.5)
        p = _softmax(scores, axis=-1)
        o = jnp.einsum("bhqk,bhkd->bhqd", p, v)
        return (lambda x, *d: x.transpose(*d))(o, 0, 2, 1, 3).reshape(B, Sq, Hq * Dh) @ wo

    def _B_ref(x, w1, w2):
        h = jnp.einsum("bsd,df->bsf", x, w1)
        h = _silu(h)
        out = jnp.einsum("bsf,fd->bsd", h, w2)
        return out

    x = A_x
    x = x + _A_ref(_layernorm(x, axis=-1), A_k_cache, A_v_cache, A_wq, A_wo)
    x = x + _B_ref(_layernorm(x, axis=-1), B_w1, B_w2)
    x = x + _A_ref(_layernorm(x, axis=-1), A_k_cache, A_v_cache, A_wq, A_wo)
    x = x + _B_ref(_layernorm(x, axis=-1), B_w1, B_w2)
    return x
```

```python
import jax
import jax.numpy as jnp
from jax import lax
import jax.experimental.pallas as pl
import jax.experimental.pallas.tpu as pltpu

F32 = jnp.float32
BF16 = jnp.bfloat16


@jax.jit
def pallas_interleave_layers__gqa_block_cached__dense_activation_silu__decode_kernel(
    A_x: jax.Array,
    A_k_cache: jax.Array,
    A_v_cache: jax.Array,
    A_wq: jax.Array,
    A_wo: jax.Array,
    B_x: jax.Array,
    B_w1: jax.Array,
    B_w2: jax.Array,
):
    B, Sq, D = A_x.shape
    _, Hkv, S, Dh = A_k_cache.shape
    Hq = A_wq.shape[1] // Dh
    rep = Hq // Hkv
    Fdim = B_w1.shape[1]
    assert B == 2 and Sq == 1 and rep == 4 and Dh == 128
    G = rep * Dh
    scale = Dh ** -0.5
    eps = 1e-5

    x2d = A_x.reshape(B, D)

    SEM_X, SEM_WQ, SEM_WO, SEM_W1, SEM_W2 = 0, 1, 2, 3, 4
    SEM_K = 5
    SEM_V = SEM_K + B * Hkv
    NSEM = SEM_V + B * Hkv

    def kernel(x_hbm, k_hbm, v_hbm, wq_hbm, wo_hbm, w1_hbm, w2_hbm, o_ref,
               xbuf, kbuf, vbuf, wq, wo, w1, w2, q_scr, acc_scr, sems):
        def cp_k(b, h):
            return pltpu.make_async_copy(k_hbm.at[b, h], kbuf.at[b, h], sems.at[SEM_K + b * Hkv + h])

        def cp_v(b, h):
            return pltpu.make_async_copy(v_hbm.at[b, h], vbuf.at[b, h], sems.at[SEM_V + b * Hkv + h])

        cp_x = pltpu.make_async_copy(x_hbm, xbuf, sems.at[SEM_X])
        cp_wq = pltpu.make_async_copy(wq_hbm, wq, sems.at[SEM_WQ])
        cp_wo = pltpu.make_async_copy(wo_hbm, wo, sems.at[SEM_WO])
        cp_w1 = pltpu.make_async_copy(w1_hbm, w1, sems.at[SEM_W1])
        cp_w2 = pltpu.make_async_copy(w2_hbm, w2, sems.at[SEM_W2])

        cp_x.start()
        cp_wq.start()
        cp_wo.start()
        for h in range(Hkv):
            cp_k(0, h).start()
            cp_v(0, h).start()
            if h == 2:
                cp_w1.start()
                cp_w2.start()
        for h in range(Hkv):
            cp_k(1, h).start()
            cp_v(1, h).start()

        row8 = lax.broadcasted_iota(jnp.int32, (8, Dh), 0)
        rowg = lax.broadcasted_iota(jnp.int32, (8, G), 0)
        colg = lax.broadcasted_iota(jnp.int32, (8, G), 1)
        diag_mask = rowg == (colg // Dh)

        def layernorm(x):
            m = jnp.mean(x, axis=-1, keepdims=True)
            xc = x - m
            v = jnp.mean(xc * xc, axis=-1, keepdims=True)
            return xc * lax.rsqrt(v + eps)

        def compute_q(x):
            xn = layernorm(x).astype(BF16)
            for g in range(Hkv):
                qa = jnp.dot(xn, wq[:, g * G:(g + 1) * G], preferred_element_type=F32) * scale
                qg = jnp.zeros((8, Dh), F32)
                for j in range(rep):
                    qg = jnp.where(row8 == j, qa[:, j * Dh:(j + 1) * Dh], qg)
                q_scr[g] = qg.astype(BF16)

        def attn_head(b, h, wait):
            if wait:
                cp_k(b, h).wait()
            q = q_scr[h]
            s = lax.dot_general(q, kbuf[b, h], (((1,), (1,)), ((), ())), preferred_element_type=F32)
            m = jnp.max(s, axis=1, keepdims=True)
            p = jnp.exp(s - m)
            l = jnp.sum(p, axis=1, keepdims=True)
            if wait:
                cp_v(b, h).wait()
            o = jnp.dot(p.astype(BF16), vbuf[b, h], preferred_element_type=F32)
            o = o / l
            o4 = jnp.concatenate([o] * rep, axis=1)
            o4 = jnp.where(diag_mask, o4, 0.0).astype(BF16)
            off = pl.multiple_of(h * G, G)
            acc_scr[...] += jnp.dot(o4, wo[pl.ds(off, G), :], preferred_element_type=F32)

        def attn_pass(b, wait):
            acc_scr[...] = jnp.zeros_like(acc_scr)

            def body(h, c):
                attn_head(b, h, wait)
                return c
            lax.fori_loop(0, Hkv, body, 0)
            a = jnp.sum(acc_scr[...], axis=0, keepdims=True)
            return jnp.broadcast_to(a, (8, D))

        def ffn(x):
            xn = layernorm(x).astype(BF16)
            hh = jnp.dot(xn, w1[...], preferred_element_type=F32)
            hh = hh * jax.nn.sigmoid(hh)
            return jnp.dot(hh.astype(BF16), w2[...], preferred_element_type=F32)

        cp_x.wait()
        cp_wq.wait()
        cp_wo.wait()
        for b in range(B):
            x = jnp.broadcast_to(xbuf[b:b + 1, :].astype(F32), (8, D))
            compute_q(x)
            x = x + attn_pass(b, True)
            if b == 0:
                cp_w1.wait()
                cp_w2.wait()
            x = x + ffn(x)
            compute_q(x)
            x = x + attn_pass(b, False)
            x = x + ffn(x)
            o_ref[b:b + 1, :] = x[0:1, :].astype(o_ref.dtype)

    out = pl.pallas_call(
        kernel,
        out_shape=jax.ShapeDtypeStruct((B, D), A_x.dtype),
        in_specs=[pl.BlockSpec(memory_space=pl.ANY)] * 7,
        out_specs=pl.BlockSpec(memory_space=pltpu.VMEM),
        scratch_shapes=[
            pltpu.VMEM((B, D), BF16),
            pltpu.VMEM((B, Hkv, S, Dh), BF16),
            pltpu.VMEM((B, Hkv, S, Dh), BF16),
            pltpu.VMEM((D, Hq * Dh), BF16),
            pltpu.VMEM((Hq * Dh, D), BF16),
            pltpu.VMEM((D, Fdim), BF16),
            pltpu.VMEM((Fdim, D), BF16),
            pltpu.VMEM((Hkv, 8, Dh), BF16),
            pltpu.VMEM((8, D), F32),
            pltpu.SemaphoreType.DMA((NSEM,)),
        ],
        compiler_params=pltpu.CompilerParams(vmem_limit_bytes=110 * 1024 * 1024),
    )(x2d, A_k_cache, A_v_cache, A_wq, A_wo, B_w1, B_w2)
    return out.reshape(B, Sq, D)
```

```python
import functools
import jax
import jax.numpy as jnp
from jax import lax
import jax.experimental.pallas as pl
import jax.experimental.pallas.tpu as pltpu

F32 = jnp.float32
BF16 = jnp.bfloat16
U32 = jnp.uint32
NT = (((1,), (1,)), ((), ()))
PLAN_A = "K0:q2 K1:q3 K2:q4 V0:q5 K3:q6 V1:o0 K4:q7 V2:o1 K5 V3:o2 K6 V4:o3 K7 V5:o4 V6:o5 V7"

def make(plan=PLAN_A, dead=4, qdead=True, nch=8, fold=True, cut=0, tchunk=2048, last_chunks=(6144, 1536, 512),
         n_outer=2, scoped=True,
         g0=((0, 4), (4, 6), (6, 7), (7, 8)), gk1=((0, 4), (4, 8)), gv1=((0, 4), (4, 6), (6, 7))):
  @jax.jit
  def f(A_x, A_k_cache, A_v_cache, A_wq, A_wo, B_x, B_w1, B_w2):
    B, Sq, D = A_x.shape
    _, Hkv, S, Dh = A_k_cache.shape
    Hq = A_wq.shape[1] // Dh
    rep = Hq // Hkv
    Fdim = B_w1.shape[1]
    G = rep * Dh
    scale = Dh ** -0.5
    eps = 1e-5
    x2d = A_x.reshape(B, D)
    SEM_W = 0
    SEM_0 = 1
    SEM_K1 = SEM_0 + len(g0)
    SEM_V1 = SEM_K1 + len(gk1)
    SEM_L = SEM_V1 + len(gv1)
    NL = len(last_chunks)
    n_in = NL - n_outer
    NSEM_IN = SEM_L + n_in
    lc_off = [sum(last_chunks[:i]) for i in range(NL)]
    HL = Hkv - 1
    phases = [ph.split(":") for ph in plan.split()]
    hosted = set(ph[1] for ph in phases if len(ph) > 1)
    mxu_q = [g for g in range(Hkv) if "q%d" % g not in hosted]
    mxu_o = [g for g in range(Hkv) if "o%d" % g not in hosted]
    assert HL in mxu_o

    def kernel(x_hbm, k_hbm, v_hbm, wq_hbm, wo_hbm, w1_hbm, w2_hbm, o_ref,
               xbuf, kbuf, vbuf, ktbuf, wq, wo, w1, w2, wqf, wof, wqp, wop, w1p, w2p, cq, c1,
               q_scr, acc_scr, p_scr, l_scr, o_scr, xb_scr, ob_scr, osems, *rest):
        row8 = lax.broadcasted_iota(jnp.int32, (8, Dh), 0)
        rowg = lax.broadcasted_iota(jnp.int32, (8, G), 0)
        colg = lax.broadcasted_iota(jnp.int32, (8, G), 1)
        diag_mask = rowg == (colg // Dh)

        vb32 = vbuf.bitcast(U32)
        def load_v(b, h, off, n):
            return pltpu.bitcast(vb32[b, h, pl.ds(off // 2, n // 2), :], BF16)
        def load_kt(h, off, n):
            return pltpu.bitcast(ktbuf[h, :, pl.ds(off, n)], BF16)

        def ln_stats(x):
            m = jnp.mean(x, axis=-1, keepdims=True)
            xc = x - m
            v = jnp.mean(xc * xc, axis=-1, keepdims=True)
            return m, xc, lax.rsqrt(v + eps)

        def layernorm(x):
            m, xc, r = ln_stats(x)
            return xc * r

        def pick_rows(qa):
            qg = jnp.zeros((8, Dh), F32)
            for j in range(rep):
                qg = jnp.where(row8 == j, qa[:, j * Dh:(j + 1) * Dh], qg)
            return qg

        def diag_lhs(o):
            o4 = jnp.concatenate([o] * rep, axis=1)
            return jnp.where(diag_mask, o4, 0.0).astype(BF16)

        def out_proj_fast(o, g):
            return jnp.dot(diag_lhs(o), pltpu.bitcast(wop[mxu_o.index(g)], BF16), preferred_element_type=F32)

        def rowsum(a):
            return jnp.broadcast_to(jnp.sum(a, axis=0, keepdims=True), (8, D))

        def cp_vl(i, sem):
            sl = pl.ds(lc_off[i], last_chunks[i])
            return pltpu.make_async_copy(v_hbm.at[1, HL, sl], vbuf.at[1, HL, sl], sem)

        def pv_last(i):
            return jnp.dot(p_scr[HL, :, lc_off[i]:lc_off[i] + last_chunks[i]],
                           load_v(1, HL, lc_off[i], last_chunks[i]), preferred_element_type=F32)

        cps_out = [cp_vl(n_in + i, osems.at[i]) for i in range(n_outer)]

        def streaming_part(sems):
            def cp_kv(hbm, buf, b, grp, sem):
                sl = pl.ds(grp[0], grp[1] - grp[0])
                return pltpu.make_async_copy(hbm.at[b, sl], buf.at[b, sl], sems.at[sem])
            cps_w = [pltpu.make_async_copy(s_, d_, sems.at[SEM_W]) for s_, d_ in
                     ((x_hbm, xbuf), (wq_hbm, wq), (wo_hbm, wo), (w1_hbm, w1), (w2_hbm, w2))]
            cps_0 = [(cp_kv(k_hbm, kbuf, 0, g, SEM_0 + i), cp_kv(v_hbm, vbuf, 0, g, SEM_0 + i))
                     for i, g in enumerate(g0)]
            cps_k1 = [cp_kv(k_hbm, kbuf, 1, g, SEM_K1 + i) for i, g in enumerate(gk1)]
            cps_v1 = [cp_kv(v_hbm, vbuf, 1, g, SEM_V1 + i) for i, g in enumerate(gv1)]
            cps_l = [cp_vl(i, sems.at[SEM_L + i]) for i in range(n_in)]
            for c in cps_w: c.start()
            for a, b_ in cps_0:
                a.start(); b_.start()
            for c in cps_k1 + cps_v1 + cps_l + cps_out: c.start()

            def compute_q(x):
                xn = layernorm(x).astype(BF16)
                for g in range(Hkv):
                    qa = jnp.dot(xn, wq[:, g * G:(g + 1) * G], preferred_element_type=F32) * scale
                    q_scr[g] = pick_rows(qa).astype(BF16)

            def softmax_parts(s):
                m = jnp.max(s, axis=1, keepdims=True)
                p = jnp.exp(s - m)
                l = jnp.sum(p, axis=1, keepdims=True)
                return p.astype(BF16), l

            def out_proj(o, h):
                w = wo[pl.ds(pl.multiple_of(h * G, G), G), :]
                return jnp.dot(diag_lhs(o), w, preferred_element_type=F32)

            def transpose_k(h):
                def cb(c, carry):
                    off = pl.multiple_of(c * tchunk, tchunk)
                    ktbuf[h, :, pl.ds(off, tchunk)] = pltpu.bitcast(kbuf[1, h, pl.ds(off, tchunk), :].T, U32)
                    return carry
                lax.fori_loop(0, S // tchunk, cb, 0)

            def attn_head0(h, c):
                s = lax.dot_general(q_scr[h], kbuf[0, h], NT, preferred_element_type=F32)
                p, l = softmax_parts(s)
                o = jnp.dot(p, load_v(0, h, 0, S), preferred_element_type=F32)
                acc_scr[...] += out_proj(o / l, h)
                return c

            def kside1(h, c):
                s = lax.dot_general(q_scr[h], kbuf[1, h], NT, preferred_element_type=F32)
                p, l = softmax_parts(s)
                p_scr[h] = p
                l_scr[h] = jnp.broadcast_to(1.0 / l, (8, Dh))
                transpose_k(h)
                return c

            def vside1(h, c):
                o = jnp.dot(p_scr[h], load_v(1, h, 0, S), preferred_element_type=F32)
                acc_scr[...] += out_proj(o * l_scr[h], h)
                return c

            def ffn(x):
                xn = layernorm(x).astype(BF16)
                hh = jnp.dot(xn, w1[...], preferred_element_type=F32)
                hh = hh * jax.nn.sigmoid(hh)
                return jnp.dot(hh.astype(BF16), w2[...], preferred_element_type=F32)

            for c in cps_w: c.wait()
            def prep_q(i, c):
                off = pl.multiple_of(i * 64, 64)
                wqf[pl.ds(off, 64), :] = wq[pl.ds(off, 64), :].astype(F32)
                return c
            lax.fori_loop(0, D // 64, prep_q, 0)
            def prep_o(i, c):
                off = pl.multiple_of(i * 512, 512)
                wof[pl.ds(off, 512), :] = wo[pl.ds(off, 512), :].astype(F32)
                return c
            lax.fori_loop(0, Hq * Dh // 512, prep_o, 0)
            for i, g in enumerate(mxu_q):
                wqp[i] = pltpu.bitcast(wq[:, g * G:(g + 1) * G], U32)
            for i, g in enumerate(mxu_o):
                wop[i] = pltpu.bitcast(wo[g * G:(g + 1) * G, :], U32)
            w1p[...] = pltpu.bitcast(w1[...], U32)
            w2p[...] = pltpu.bitcast(w2[...], U32)
            ones8 = jnp.ones((8, D), BF16)
            cq[...] = jnp.dot(ones8, wq[...], preferred_element_type=F32)
            c1[...] = jnp.dot(ones8, w1[...], preferred_element_type=F32)

            x = jnp.broadcast_to(xbuf[0:1, :].astype(F32), (8, D))
            compute_q(x)
            acc_scr[...] = jnp.zeros_like(acc_scr)
            for i, g in enumerate(g0):
                cps_0[i][0].wait(); cps_0[i][1].wait()
                lax.fori_loop(g[0], g[1], attn_head0, 0)
            x = x + rowsum(acc_scr[...])
            x = x + ffn(x)
            compute_q(x)
            acc_scr[...] = jnp.zeros_like(acc_scr)
            lax.fori_loop(0, Hkv, attn_head0, 0)
            x = x + rowsum(acc_scr[...])
            x = x + ffn(x)
            o_ref[0:1, :] = x[0:1, :].astype(o_ref.dtype)
            x = jnp.broadcast_to(xbuf[1:2, :].astype(F32), (8, D))
            compute_q(x)
            for i, g in enumerate(gk1):
                cps_k1[i].wait()
                lax.fori_loop(g[0], g[1], kside1, 0)
            acc_scr[...] = jnp.where(lax.broadcasted_iota(jnp.int32, (8, D), 0) == 0, x, 0.0)
            for i, g in enumerate(gv1):
                cps_v1[i].wait()
                lax.fori_loop(g[0], g[1], vside1, 0)
            o_scr[...] = jnp.zeros_like(o_scr)
            for i in range(n_in):
                cps_l[i].wait()
                o_scr[...] += pv_last(i)

        if scoped:
            pl.run_scoped(streaming_part, pltpu.SemaphoreType.DMA((NSEM_IN,)))
        else:
            streaming_part(rest[0])

        for i in range(n_outer - 1):
            cps_out[i].wait()
            o_scr[...] += pv_last(n_in + i)
        cps_out[-1].wait()
        o = o_scr[...] + pv_last(NL - 1)
        if cut == 1:
            o_ref[1:2, :] = jnp.concatenate([o] * 4, axis=1)[0:1, :].astype(o_ref.dtype)
            return

        def ffn_fast(x):
            m, _, r = ln_stats(x)
            y = jnp.dot(x.astype(BF16), pltpu.bitcast(w1p[...], BF16), preferred_element_type=F32)
            hh = (y - m * c1[...]) * r
            hh = hh * jax.nn.sigmoid(hh)
            return jnp.dot(hh.astype(BF16), pltpu.bitcast(w2p[...], BF16), preferred_element_type=F32)

        x = rowsum(acc_scr[...] + out_proj_fast(o * l_scr[HL], HL))
        x = x + ffn_fast(x)
        if cut == 2:
            o_ref[1:2, :] = x[0:1, :].astype(o_ref.dtype)
            return
        m, _, r = ln_stats(x)
        rs = r * scale
        def fin_q(qa, g):
            return pick_rows((qa - m * cq[:, g * G:(g + 1) * G]) * rs)
        x16 = x.astype(BF16)

        def q_mxu(g):
            return fin_q(jnp.dot(x16, pltpu.bitcast(wqp[mxu_q.index(g)], BF16), preferred_element_type=F32), g)

        for c in range(D // Dh):
            xb_scr[0, c * Dh:(c + 1) * Dh, :] = jnp.broadcast_to(x[0:1, c * Dh:(c + 1) * Dh], (Dh, Dh)).T

        NKB = D // 8

        class MatVec:
            def __init__(self, xb_ref, slot, w_ref, row0, cols):
                self.xb_ref, self.slot, self.w_ref, self.row0, self.cols = xb_ref, slot, w_ref, row0, cols
                self.accs = [None] * len(cols)
                self.kb = 0
            def step(self, n, tok):
                for kb in range(self.kb, min(self.kb + n, NKB)):
                    xv = self.xb_ref[self.slot, kb * 8:kb * 8 + 8, :]
                    if tok is not None:
                        xv = xv + tok
                    for i, c0 in enumerate(self.cols):
                        r0 = self.row0 + kb * 8
                        t = xv * self.w_ref[r0:r0 + 8, c0:c0 + Dh]
                        a = self.accs[i]
                        self.accs[i] = t if a is None else a + t
                self.kb = min(self.kb + n, NKB)

        def mk_tok(v):
            return jnp.minimum(jnp.abs(v), 0.0)

        def q_task(g):
            return MatVec(xb_scr, 0, wqf, 0, [g * G + j * Dh for j in range(rep)])
        def q_finish(t, g):
            parts = [jnp.broadcast_to(jnp.sum(a, axis=0, keepdims=True), (8, Dh)) for a in t.accs]
            return fin_q(jnp.concatenate(parts, axis=1), g)
        def o_task(o, g):
            slot = g % 2
            for j in range(rep):
                ob_scr[slot, j * Dh:(j + 1) * Dh, :] = jnp.broadcast_to(o[j:j + 1, :], (Dh, Dh)).T
            return MatVec(ob_scr, slot, wof, g * G, [nb * Dh for nb in range(D // Dh)])

        per = NKB // nch
        SW = S // 2 if fold else S
        CH = SW // nch

        def qk2(q, g, task, dtok):
            outs = []
            for c in range(nch):
                if c == 0 or (dtok is not None and c == dead):
                    qq = q if c == 0 else q + dtok
                    qa = qq.astype(BF16)
                    if fold:
                        qb = pltpu.roll(qq, 4, 0).astype(BF16)
                sc = jnp.dot(qa, load_kt(g, c * CH, CH), preferred_element_type=F32)
                if fold:
                    sc = sc + jnp.dot(qb, load_kt(g, SW + c * CH, CH), preferred_element_type=F32)
                outs.append(sc)
                if task is not None:
                    task.step(per, mk_tok(sc[:, 0:Dh]))
            return jnp.concatenate(outs, axis=1)

        def pv2(p, g, task, dtok):
            o = None; o2 = None
            for c in range(nch):
                pc = p[:, c * CH:(c + 1) * CH]
                if dtok is not None and c == dead:
                    pc = jnp.concatenate([(pc[:, 0:Dh].astype(F32) + dtok).astype(BF16), pc[:, Dh:]], axis=1)
                oc = jnp.dot(pc, load_v(1, g, c * CH, CH), preferred_element_type=F32)
                o = oc if o is None else o + oc
                if fold:
                    oc2 = jnp.dot(pc, load_v(1, g, SW + c * CH, CH), preferred_element_type=F32)
                    o2 = oc2 if o2 is None else o2 + oc2
                if task is not None:
                    task.step(per, mk_tok(oc))
            if fold:
                o = o + pltpu.roll(o2, 4, 0)
            return o

        def softmax2(s):
            m_ = jnp.max(s, axis=1, keepdims=True)
            if fold:
                m_ = jnp.broadcast_to(m_, (8, Dh))
                m_ = jnp.maximum(m_, pltpu.roll(m_, 4, 0))[:, 0:1]
            p = jnp.exp(s - m_)
            lp = p[:, 0:Dh]
            for c in range(1, SW // Dh):
                lp = lp + p[:, c * Dh:(c + 1) * Dh]
            if fold:
                lp = lp + pltpu.roll(lp, 4, 0)
            l = jnp.sum(lp, axis=1, keepdims=True)
            return p.astype(BF16), l, jnp.minimum(lp, 0.0)

        acc = jnp.where(lax.broadcasted_iota(jnp.int32, (8, D), 0) == 0, x, 0.0)
        qs = {}; sm_ = {}; os_ = {}
        for g in mxu_q:
            qs[g] = q_mxu(g)
        pending_o = []
        for i, ph in enumerate(phases):
            kind, g = ph[0][0], int(ph[0][1])
            task = None
            if len(ph) > 1:
                tk, tg = ph[1][0], int(ph[1][1])
                task = q_task(tg) if tk == "q" else o_task(os_[tg] / sm_[tg][1], tg)
            dtok = None
            if dead is not None and i + 1 < len(phases):
                nk, ng = phases[i + 1][0][0], int(phases[i + 1][0][1])
                if nk == "V" and ng in sm_:
                    dtok = sm_[ng][2]
                if nk == "K" and qdead and ng in qs and ng not in mxu_q:
                    dtok = mk_tok(qs[ng])
            if kind == "K":
                sm_[g] = softmax2(qk2(qs[g], g, task, dtok))
            else:
                os_[g] = pv2(sm_[g][0], g, task, dtok)
            for og in pending_o:
                acc = acc + out_proj_fast(os_[og] / sm_[og][1], og)
            pending_o = []
            if kind == "V" and g in mxu_o:
                pending_o.append(g)
            if task is not None:
                if tk == "q":
                    qs[tg] = q_finish(task, tg)
                else:
                    acc = acc + jnp.concatenate(task.accs, axis=1)
        for og in pending_o:
            acc = acc + out_proj_fast(os_[og] / sm_[og][1], og)
        x = rowsum(acc)
        x = x + ffn_fast(x)
        o_ref[1:2, :] = x[0:1, :].astype(o_ref.dtype)

    out = pl.pallas_call(
        kernel,
        out_shape=jax.ShapeDtypeStruct((B, D), A_x.dtype),
        in_specs=[pl.BlockSpec(memory_space=pl.ANY)] * 7,
        out_specs=pl.BlockSpec(memory_space=pltpu.VMEM),
        scratch_shapes=[
            pltpu.VMEM((B, D), BF16),
            pltpu.VMEM((B, Hkv, S, Dh), BF16),
            pltpu.VMEM((B, Hkv, S, Dh), BF16),
            pltpu.VMEM((Hkv, Dh // 2, S), U32),
            pltpu.VMEM((D, Hq * Dh), BF16),
            pltpu.VMEM((Hq * Dh, D), BF16),
            pltpu.VMEM((D, Fdim), BF16),
            pltpu.VMEM((Fdim, D), BF16),
            pltpu.VMEM((D, Hq * Dh), F32),
            pltpu.VMEM((Hq * Dh, D), F32),
            pltpu.VMEM((len(mxu_q), D // 2, G), U32),
            pltpu.VMEM((len(mxu_o), G // 2, D), U32),
            pltpu.VMEM((D // 2, Fdim), U32),
            pltpu.VMEM((Fdim // 2, D), U32),
            pltpu.VMEM((8, Hq * Dh), F32),
            pltpu.VMEM((8, Fdim), F32),
            pltpu.VMEM((Hkv, 8, Dh), BF16),
            pltpu.VMEM((8, D), F32),
            pltpu.VMEM((Hkv, 8, S), BF16),
            pltpu.VMEM((Hkv, 8, Dh), F32),
            pltpu.VMEM((8, Dh), F32),
            pltpu.VMEM((1, D, Dh), F32),
            pltpu.VMEM((2, G, Dh), F32),
            pltpu.SemaphoreType.DMA((n_outer,)),
        ] + ([] if scoped else [pltpu.SemaphoreType.DMA((NSEM_IN,))]),
        compiler_params=pltpu.CompilerParams(vmem_limit_bytes=126 * 1024 * 1024),
    )(x2d, A_k_cache, A_v_cache, A_wq, A_wo, B_w1, B_w2)
    return out.reshape(B, Sq, D)
  return f


_impl = make()


@jax.jit
def pallas_interleave_layers__gqa_block_cached__dense_activation_silu__decode_kernel(
    A_x: jax.Array,
    A_k_cache: jax.Array,
    A_v_cache: jax.Array,
    A_wq: jax.Array,
    A_wo: jax.Array,
    B_x: jax.Array,
    B_w1: jax.Array,
    B_w2: jax.Array,
):
    return _impl(A_x, A_k_cache, A_v_cache, A_wq, A_wo, B_x, B_w1, B_w2)
```

```python
import jax
import jax.numpy as jnp
from jax import lax
import jax.experimental.pallas as pl
import jax.experimental.pallas.tpu as pltpu

F32 = jnp.float32
BF16 = jnp.bfloat16
U32 = jnp.uint32
NT = (((1,), (1,)), ((), ()))
LOG2E = 1.4426950408889634

G0 = ((0, 4), (4, 6), (6, 7), (7, 8))
GK1 = ((0, 4), (4, 8))
GV1 = ((0, 4), (4, 6), (6, 7))
LAST_CHUNKS = (6144, 1536, 512)
N_OUTER = 2
TCHUNK = 2048

ORDER = "K0 K1 K2 K3 V0 K4 V1 K5 V2 K6 V3 K7 V4 V5 V6 V7".split()
QUEUE = "q2 q3 q4 q5 q6 q7 p0 p1 p2 o0 p3 o1 p4 o2 p5 o3 o4 o5".split()
NVP = 8
CB = 2
RATE = 100.5
LAG = 8
ELAG = 9
EUNIT = 4
ECOST = 3
OLAG = 6
PRE = 9
N2 = 2
NF = 6


@jax.jit
def pallas_interleave_layers__gqa_block_cached__dense_activation_silu__decode_kernel(
    A_x: jax.Array,
    A_k_cache: jax.Array,
    A_v_cache: jax.Array,
    A_wq: jax.Array,
    A_wo: jax.Array,
    B_x: jax.Array,
    B_w1: jax.Array,
    B_w2: jax.Array,
):
    B, Sq, D = A_x.shape
    _, Hkv, S, Dh = A_k_cache.shape
    Hq = A_wq.shape[1] // Dh
    rep = Hq // Hkv
    Fdim = B_w1.shape[1]
    assert (B, Sq, rep, Dh, Hkv) == (2, 1, 4, 128, 8) and D == rep * Dh and sum(LAST_CHUNKS) == S
    G = rep * Dh
    scale = Dh ** -0.5
    eps = 1e-5
    SEM_W = 0
    SEM_0 = 1
    SEM_K1 = SEM_0 + len(G0)
    SEM_V1 = SEM_K1 + len(GK1)
    SEM_L = SEM_V1 + len(GV1)
    NL = len(LAST_CHUNKS)
    n_in = NL - N_OUTER
    NSEM_IN = SEM_L + n_in
    lc_off = [sum(LAST_CHUNKS[:i]) for i in range(NL)]
    HL = Hkv - 1
    vpu_q = [g for g in range(Hkv) if "q%d" % g in QUEUE]
    vpu_o = [g for g in range(Hkv) if "o%d" % g in QUEUE]
    vpu_p = [g for g in range(Hkv) if "p%d" % g in QUEUE]
    mxu_q = [g for g in range(Hkv) if g not in vpu_q]
    mxu_o = [g for g in range(Hkv) if g not in vpu_o]
    assert vpu_q == list(range(vpu_q[0], Hkv)) and vpu_o == list(range(len(vpu_o)))
    assert vpu_p == list(range(len(vpu_p))) and set(vpu_p) <= set(vpu_o) and HL in mxu_o
    Q0 = vpu_q[0] * G
    SW = S // 2
    NBLK = SW // Dh
    VP0 = SW - NVP * Dh
    NKB = D // 8
    FM = Fdim - NF * Dh

    def kernel(x_hbm, k_hbm, v_hbm, wq_hbm, wo_hbm, w1_hbm, w2_hbm, o_ref,
               xbuf, kbuf, vbuf, ktbuf, wq, wo, w1, w2, wqf, wof, w2f, w1t, w2g,
               wqp, wop, w1p, w2p, cq, c1, q_scr, acc_scr, p_scr, l_scr, o_scr, c_scr,
               xb_scr, hb_scr, ob_scr, vtf, pf_scr, pa_scr, z_scr, osems):
        row8 = lax.broadcasted_iota(jnp.int32, (8, Dh), 0)
        rowg = lax.broadcasted_iota(jnp.int32, (8, G), 0)
        colg = lax.broadcasted_iota(jnp.int32, (8, G), 1)
        diag_mask = rowg == (colg // Dh)
        eye = (lax.broadcasted_iota(jnp.int32, (Dh, Dh), 0) == lax.broadcasted_iota(jnp.int32, (Dh, Dh), 1))

        def load_v(h, off, n):
            return pltpu.bitcast(vbuf.bitcast(U32)[1, h, off // 2:(off + n) // 2, :], BF16)

        def load_kt(h, off, n):
            return pltpu.bitcast(ktbuf[h, :, off:off + n], BF16)

        def pick_rows(qa):
            qg = jnp.zeros((8, Dh), F32)
            for j in range(rep):
                qg = jnp.where(row8 == j, qa[:, j * Dh:(j + 1) * Dh], qg)
            return qg

        def diag_lhs(o):
            o4 = jnp.concatenate([o] * rep, axis=1)
            return jnp.where(diag_mask, o4, 0.0).astype(BF16)

        def out_proj_fast(o, g):
            return jnp.dot(diag_lhs(o), pltpu.bitcast(wop[mxu_o.index(g)], BF16), preferred_element_type=F32)

        def rowsum(a):
            return jnp.broadcast_to(jnp.sum(a, axis=0, keepdims=True), a.shape)

        def lanesum(a):
            return jnp.broadcast_to(jnp.sum(a, axis=1, keepdims=True), (a.shape[0], Dh))

        def col_bcast(row):
            return lanesum(jnp.where(eye, jnp.broadcast_to(row, (Dh, Dh)), 0.0))

        def cp_vl(i, sem):
            sl = pl.ds(lc_off[i], LAST_CHUNKS[i])
            return pltpu.make_async_copy(v_hbm.at[1, HL, sl], vbuf.at[1, HL, sl], sem)

        def pv_last(i):
            sl = slice(lc_off[i], lc_off[i] + LAST_CHUNKS[i])
            return jnp.dot(p_scr[HL, :, sl], vbuf[1, HL, sl, :], preferred_element_type=F32)

        cps_out = [cp_vl(n_in + i, osems.at[i]) for i in range(N_OUTER)]

        def streaming_part(sems):
            def cp_kv(hbm, buf, b, grp, sem):
                sl = pl.ds(grp[0], grp[1] - grp[0])
                return pltpu.make_async_copy(hbm.at[b, sl], buf.at[b, sl], sems.at[sem])
            cps_w = [pltpu.make_async_copy(s_, d_, sems.at[SEM_W]) for s_, d_ in
                     ((x_hbm, xbuf), (wq_hbm, wq), (wo_hbm, wo), (w1_hbm, w1), (w2_hbm, w2))]
            cps_0 = [(cp_kv(k_hbm, kbuf, 0, g, SEM_0 + i), cp_kv(v_hbm, vbuf, 0, g, SEM_0 + i))
                     for i, g in enumerate(G0)]
            cps_k1 = [cp_kv(k_hbm, kbuf, 1, g, SEM_K1 + i) for i, g in enumerate(GK1)]
            cps_v1 = [cp_kv(v_hbm, vbuf, 1, g, SEM_V1 + i) for i, g in enumerate(GV1)]
            cps_l = [cp_vl(i, sems.at[SEM_L + i]) for i in range(n_in)]
            for c in cps_w:
                c.start()
            for a, b_ in cps_0:
                a.start()
                b_.start()
            for c in cps_k1 + cps_v1 + cps_l + cps_out:
                c.start()

            def layernorm(x):
                xc = x - jnp.mean(x, axis=-1, keepdims=True)
                return xc * lax.rsqrt(jnp.mean(xc * xc, axis=-1, keepdims=True) + eps)

            def compute_q(x):
                xn = layernorm(x).astype(BF16)
                for g in range(Hkv):
                    qa = jnp.dot(xn, wq[:, g * G:(g + 1) * G], preferred_element_type=F32) * scale
                    q_scr[g] = pick_rows(qa).astype(BF16)

            def softmax_parts(s):
                p = jnp.exp(s - jnp.max(s, axis=1, keepdims=True))
                return p.astype(BF16), jnp.sum(p, axis=1, keepdims=True)

            def out_proj(o, h):
                w = wo[pl.ds(pl.multiple_of(h * G, G), G), :]
                return jnp.dot(diag_lhs(o), w, preferred_element_type=F32)

            def attn_head0(h, c):
                s = lax.dot_general(q_scr[h], kbuf[0, h], NT, preferred_element_type=F32)
                p, l = softmax_parts(s)
                o = jnp.dot(p, vbuf[0, h], preferred_element_type=F32)
                acc_scr[...] += out_proj(o / l, h)
                return c

            def kside1(h, c):
                s = lax.dot_general(q_scr[h], kbuf[1, h], NT, preferred_element_type=F32)
                p, l = softmax_parts(s)
                p_scr[h] = p
                l_scr[h] = jnp.broadcast_to(1.0 / l, (8, Dh))

                def tr(i, carry):
                    off = pl.multiple_of(i * TCHUNK, TCHUNK)
                    ktbuf[h, :, pl.ds(off, TCHUNK)] = pltpu.bitcast(kbuf[1, h, pl.ds(off, TCHUNK), :].T, U32)
                    return carry
                lax.fori_loop(0, S // TCHUNK, tr, 0)
                return c

            def vside1(h, c):
                o = jnp.dot(p_scr[h], vbuf[1, h], preferred_element_type=F32)
                acc_scr[...] += out_proj(o * l_scr[h], h)
                return c

            def vside1t(h, c):
                vside1(h, c)
                for hf in range(2):
                    vtf[h, :, hf * NVP * Dh:(hf + 1) * NVP * Dh] = (
                        vbuf[1, h, hf * SW + VP0:(hf + 1) * SW, :].astype(F32).T)
                return c

            def ffn(x):
                hh = jnp.dot(layernorm(x).astype(BF16), w1[...], preferred_element_type=F32)
                hh = hh * jax.nn.sigmoid(hh)
                return jnp.dot(hh.astype(BF16), w2[...], preferred_element_type=F32)

            for c in cps_w:
                c.wait()

            def prep_q(i, c):
                off = pl.multiple_of(i * 64, 64)
                wqf[pl.ds(off, 64), :] = wq[pl.ds(off, 64), Q0:].astype(F32)
                return c
            lax.fori_loop(0, D // 64, prep_q, 0)

            def prep_o(i, c):
                off = pl.multiple_of(i * G, G)
                wof[pl.ds(off, G), :] = wo[pl.ds(off, G), :].astype(F32)
                return c
            lax.fori_loop(0, len(vpu_o), prep_o, 0)
            for i, g in enumerate(mxu_q):
                wqp[i] = pltpu.bitcast(wq[:, g * G:(g + 1) * G], U32)
            for i, g in enumerate(mxu_o):
                wop[i] = pltpu.bitcast(wo[g * G:(g + 1) * G, :], U32)
            w1p[...] = pltpu.bitcast(w1[:, 0:FM], U32)
            w2p[...] = pltpu.bitcast(w2[N2 * Dh:FM, :], U32)
            for i in range(N2):
                w2f[i * Dh:(i + 1) * Dh, :] = w2[i * Dh:(i + 1) * Dh, :].astype(F32)
            w1t[...] = w1[:, FM:].astype(F32).T
            w2g[...] = w2[FM:, :].astype(F32)
            w1t[...] = w1t[...] - jnp.mean(w1t[...], axis=1, keepdims=True)
            ones8 = jnp.ones((8, D), BF16)
            cq[...] = jnp.dot(ones8, wq[...], preferred_element_type=F32)
            c1[...] = jnp.dot(ones8, w1[:, 0:FM], preferred_element_type=F32)
            z_scr[...] = jnp.zeros_like(z_scr)

            x = jnp.broadcast_to(xbuf[0:1, :].astype(F32), (8, D))
            compute_q(x)
            acc_scr[...] = jnp.zeros_like(acc_scr)
            for i, g in enumerate(G0):
                cps_0[i][0].wait()
                cps_0[i][1].wait()
                lax.fori_loop(g[0], g[1], attn_head0, 0)
            x = x + rowsum(acc_scr[...])
            x = x + ffn(x)
            compute_q(x)
            acc_scr[...] = jnp.zeros_like(acc_scr)
            lax.fori_loop(0, Hkv, attn_head0, 0)
            x = x + rowsum(acc_scr[...])
            x = x + ffn(x)
            o_ref[0:1, :] = x[0:1, :].astype(o_ref.dtype)
            x = jnp.broadcast_to(xbuf[1:2, :].astype(F32), (8, D))
            compute_q(x)
            for i, g in enumerate(GK1):
                cps_k1[i].wait()
                lax.fori_loop(g[0], g[1], kside1, 0)
            c0 = jnp.mean(x, axis=-1, keepdims=True)
            c_scr[...] = jnp.broadcast_to(c0, (8, Dh))
            acc_scr[...] = jnp.where(rowg == 0, x - c0, 0.0)
            for i, g in enumerate(GV1):
                cps_v1[i].wait()
                assert (g[0] in vpu_p) == (g[1] - 1 in vpu_p)
                lax.fori_loop(g[0], g[1], vside1t if g[0] in vpu_p else vside1, 0)
            o_scr[...] = jnp.zeros_like(o_scr)
            for i in range(n_in):
                cps_l[i].wait()
                o_scr[...] += pv_last(i)

        pl.run_scoped(streaming_part, pltpu.SemaphoreType.DMA((NSEM_IN,)))

        for i in range(N_OUTER - 1):
            cps_out[i].wait()
            o_scr[...] += pv_last(n_in + i)
        cps_out[-1].wait()
        o = o_scr[...] + pv_last(NL - 1)

        zero_i = z_scr[...]

        def mk_tok(v):
            return lax.bitcast_convert_type(lax.bitcast_convert_type(v, jnp.int32) & zero_i, F32)

        def sum_all(vs):
            t = vs[0]
            for v in vs[1:]:
                t = t + v
            return t

        def sum_tree(vs):
            vs = list(vs)
            while len(vs) > 1:
                vs = [vs[i] + vs[i + 1] if i + 1 < len(vs) else vs[i] for i in range(0, len(vs), 2)]
            return vs[0]

        def blocks(a):
            return [a[:, c * Dh:(c + 1) * Dh] for c in range(a.shape[1] // Dh)]

        def halves(a):
            return [a[0:8, :], a[8:16, :]]

        def stats(x):
            s1 = sum_all(blocks(x))
            s2 = sum_all(blocks(x * x))
            m = jnp.sum(s1, axis=-1, keepdims=True) * (1.0 / D)
            m2 = jnp.sum(s2, axis=-1, keepdims=True) * (1.0 / D)
            v = jnp.maximum(m2 - m * m, 0.0)
            return m, lax.rsqrt(v + eps), mk_tok(s1 + s2)

        def silu_half(a):
            return a + a * jnp.tanh(a)

        tile_cache = {}

        def tile_rows(tok, n):
            if (id(tok), n) not in tile_cache:
                tile_cache[(id(tok), n)] = (tok, jnp.concatenate([tok] * n, axis=0))
            return tile_cache[(id(tok), n)][1]

        class MatVec:
            def __init__(self, xb_ref, slot, w_ref, row0, col0, nkb=NKB):
                self.xb_ref, self.slot, self.w_ref, self.row0, self.col0 = xb_ref, slot, w_ref, row0, col0
                self.acc = None
                self.kb = 0
                self.nkb = nkb

            def step(self, n, tok):
                xv = self.xb_ref[self.slot, self.kb * 8:(self.kb + n) * 8, :]
                if tok is not None:
                    xv = xv + tile_rows(tok, n)
                self.fma(self.kb, xv)
                self.kb += n

            def fma(self, kb, xv):
                r0, n = self.row0 + kb * 8, xv.shape[0]
                t = jnp.concatenate([xv] * rep, axis=1) * self.w_ref[r0:r0 + n, self.col0:self.col0 + G]
                for i in range(0, n, 8):
                    ti = t[i:i + 8, :] if n > 8 else t
                    self.acc = ti if self.acc is None else self.acc + ti

        def ffn_fast(x):
            m, r, _ = stats(x)
            rh = 0.5 * r
            y = jnp.dot(x.astype(BF16), pltpu.bitcast(w1p[...], BF16), preferred_element_type=F32)
            h1 = silu_half((y - m * c1[...]) * rh)
            out = sum_all([
                jnp.dot(h1[:, k0:k0 + Dh].astype(BF16),
                        pltpu.bitcast(w2p[(k0 - N2 * Dh) // 2:(k0 - N2 * Dh + Dh) // 2, :], BF16),
                        preferred_element_type=F32)
                for k0 in range(N2 * Dh, FM, Dh)])
            ta = MatVec(None, 0, w2g, 0, 0)
            for kb in range(NF * 16):
                yc = lanesum(sum_all(blocks(w1t[kb * 8:kb * 8 + 8, :] * x)))
                ta.fma(kb, silu_half(yc * rh))
            for c in range(N2):
                hb_scr[0, c * Dh:(c + 1) * Dh, :] = col_bcast(h1[0:1, c * Dh:(c + 1) * Dh])
            tb = MatVec(hb_scr, 0, w2f, 0, 0, nkb=N2 * 16)
            while tb.kb < tb.nkb:
                tb.step(4, None)
            return m, out + rowsum(ta.acc + tb.acc)

        x = rowsum(acc_scr[...] + out_proj_fast(o * l_scr[HL], HL))
        m1, y1 = ffn_fast(x)
        x = (x - m1) + y1

        m, r, stok = stats(x)
        rs = r * (scale * LOG2E)

        def fin_q(qa, g):
            return pick_rows((qa - m * cq[:, g * G:(g + 1) * G]) * rs)
        x16 = x.astype(BF16)
        for c, xr in enumerate(blocks(x)):
            if c == D // Dh - 1:
                xr = xr + stok
            xb_scr[0, c * Dh:(c + 1) * Dh, :] = col_bcast(xr[0:1, :])

        qs, os_, linv_, mx_ = {}, {}, {}, {}
        state = {"acc": jnp.where(rowg == 0, x - m, 0.0)}
        shift = c_scr[:, 0:1] + m1 + m
        live, fin = [None], []
        chunk_no = [0]
        k_at, os_at, e_at = {}, {}, {}
        todo = list(QUEUE)
        stack, etasks, due = [], [], []
        credit = [0.0]
        e_started, ep_ok = set(), set()
        last_tok = [None]

        def matvec_gen(mv):
            while mv.kb < NKB:
                tok = yield 36
                mv.step(4, tok)
                live[0] = mv

        def q_gen(g):
            mv = MatVec(xb_scr, 0, wqf, 0, g * G - Q0)
            yield from matvec_gen(mv)
            qs[g] = fin_q(rowsum(mv.acc), g)
            return mk_tok(qs[g])

        def e_gen(g):
            m_ = jnp.broadcast_to(jnp.max(mx_[g], axis=1, keepdims=True), (8, Dh))
            m_ = jnp.maximum(m_, pltpu.roll(m_, 4, 0))
            lp = None
            order_ = list(range(NBLK))
            if g in vpu_p:
                order_ = order_[NBLK - NVP:] + order_[:NBLK - NVP]
            for u in range(0, NBLK, EUNIT):
                tok = yield ECOST * EUNIT
                mm = m_ if tok is None else m_ + tok
                for c in order_[u:u + EUNIT]:
                    pc = jnp.exp2(pf_scr[g, :, c * Dh:(c + 1) * Dh] - mm)
                    pf_scr[g, :, c * Dh:(c + 1) * Dh] = pc
                    lp = pc if lp is None else lp + pc
                fin.append(lp)
                if g in vpu_p and u + EUNIT >= NVP:
                    ep_ok.add(g)
            lp = lp + pltpu.roll(lp, 4, 0)
            linv_[g] = jnp.broadcast_to(1.0 / jnp.sum(lp, axis=1, keepdims=True), (8, Dh))
            e_at[g] = chunk_no[0]

        def p_gen(g):
            slot = g % 3
            for dg in range(Dh // 16):
                accs = [None] * rep
                for blk in range(NVP):
                    for hf in range(2):
                        tok = yield 20
                        col = (hf * NVP + blk) * Dh
                        vt = vtf[g, dg * 16:dg * 16 + 16, col:col + Dh]
                        if tok is not None:
                            vt = vt + tile_rows(tok, 2)
                        for j in range(rep):
                            r_ = hf * 4 + j
                            t = pf_scr[g, r_:r_ + 1, VP0 + blk * Dh:VP0 + (blk + 1) * Dh] * vt
                            accs[j] = t if accs[j] is None else accs[j] + t
                        live[0] = list(accs)
                for j in range(rep):
                    pa_scr[slot, j * Dh + dg * 16:j * Dh + dg * 16 + 16, :] = accs[j]
                fin.extend(halves(sum_tree(accs)))
                live[0] = None

        def o_gen(g):
            slot = g % 2
            linv = linv_[g]
            for j in range(rep):
                tok = yield 48
                orow = os_[g] if tok is None else os_[g] + tok
                z = jnp.where(eye, jnp.broadcast_to(orow[j:j + 1, :], (Dh, Dh)), 0.0)
                if g in vpu_p:
                    z = z + pa_scr[g % 3, j * Dh:(j + 1) * Dh, :]
                ob_scr[slot, j * Dh:(j + 1) * Dh, :] = lanesum(z) * jnp.broadcast_to(linv[j:j + 1, :], (Dh, Dh))
            mv = MatVec(ob_scr, slot, wof, g * G, 0)
            yield from matvec_gen(mv)
            state["acc"] = state["acc"] + mv.acc
            return mk_tok(sum_tree(blocks(mv.acc)))

        def ready(t):
            k_, g_ = t[0], int(t[1])
            if k_ == "p":
                return g_ in ep_ok
            if k_ == "o":
                return g_ in os_ and chunk_no[0] >= os_at[g_] + OLAG
            return True

        def run_vpu(tok, budget, force_e=None, flush=False):
            live[0] = None
            for g_, a_ in k_at.items():
                if g_ not in e_started and (chunk_no[0] >= a_ + ELAG or g_ == force_e):
                    e_started.add(g_)
                    gen = e_gen(g_)
                    etasks.append([gen, next(gen)])
            credit[0] = 1e12 if flush else min(credit[0] + budget, 2 * RATE)
            while etasks:
                credit[0] -= etasks[0][1]
                try:
                    etasks[0][1] = etasks[0][0].send(tok)
                except StopIteration:
                    etasks.pop(0)
                if not flush:
                    break
            while True:
                if not stack:
                    if not todo or (not flush and not ready(todo[0])):
                        break
                    t = todo.pop(0)
                    gen = {"q": q_gen, "p": p_gen, "o": o_gen}[t[0]](int(t[1]))
                    stack.append([gen, next(gen)])
                cur = stack[-1]
                if credit[0] < cur[1]:
                    break
                credit[0] -= cur[1]
                try:
                    cur[1] = cur[0].send(tok)
                except StopIteration as e:
                    if e.value is not None:
                        due.append((chunk_no[0] + LAG, e.value))
                    live[0] = None
                    stack.pop()
            cov = list(fin)
            if isinstance(live[0], MatVec):
                cov += blocks(live[0].acc)
            elif live[0]:
                cov += halves(sum_tree(live[0]))
            del fin[:]
            if cov and not flush:
                due.append((chunk_no[0] + LAG, mk_tok(sum_tree(cov))))

        def take_due():
            toks = [t for c_, t in due if c_ <= chunk_no[0]]
            due[:] = [(c_, t) for c_, t in due if c_ > chunk_no[0]]
            return sum_all(toks) if toks else None

        def qk2(g):
            while g not in qs:
                run_vpu(last_tok[0], RATE)
            qq = qs[g]
            mx = None
            n = CB * Dh
            for c0 in range(0, NBLK, CB):
                dtok = take_due()
                if c0 == 0 or dtok is not None:
                    if dtok is not None:
                        qq = qq + dtok
                    qa = qq.astype(BF16)
                    qb = pltpu.roll(qq, 4, 0).astype(BF16)
                sc = (jnp.dot(qa, load_kt(g, c0 * Dh, n), preferred_element_type=F32)
                      + jnp.dot(qb, load_kt(g, SW + c0 * Dh, n), preferred_element_type=F32))
                pf_scr[g, :, c0 * Dh:c0 * Dh + n] = sc
                for v in blocks(sc):
                    mx = v if mx is None else jnp.maximum(mx, v)
                chunk_no[0] += 1
                last_tok[0] = mk_tok(sc[:, 0:Dh])
                run_vpu(last_tok[0], RATE)
            mx_[g] = mx

        def pv2(g):
            while g not in e_at:
                run_vpu(last_tok[0], RATE, force_e=g)
            nb = NBLK - (NVP if g in vpu_p else 0)
            o1 = None
            o2 = None
            n = CB * Dh
            for c0 in range(0, nb, CB):
                pc = pf_scr[g, :, c0 * Dh:c0 * Dh + n]
                dtok = take_due()
                if dtok is not None:
                    pc = jnp.concatenate([pc[:, 0:Dh] + dtok, pc[:, Dh:]], axis=1)
                pc = pc.astype(BF16)
                oc = jnp.dot(pc, load_v(g, c0 * Dh, n), preferred_element_type=F32)
                o1 = oc if o1 is None else o1 + oc
                oc2 = jnp.dot(pc, load_v(g, SW + c0 * Dh, n), preferred_element_type=F32)
                o2 = oc2 if o2 is None else o2 + oc2
                chunk_no[0] += 1
                last_tok[0] = mk_tok(oc)
                run_vpu(last_tok[0], RATE)
            return o1 + pltpu.roll(o2, 4, 0)

        for g in mxu_q:
            qs[g] = fin_q(jnp.dot(x16, pltpu.bitcast(wqp[mxu_q.index(g)], BF16), preferred_element_type=F32), g)
        for _ in range(PRE):
            run_vpu(None, RATE)
        pending_o = []
        for ph in ORDER:
            kind, g = ph[0], int(ph[1])
            if kind == "K":
                qk2(g)
                k_at[g] = chunk_no[0]
            else:
                os_[g] = pv2(g)
                os_at[g] = chunk_no[0]
            for og in pending_o:
                state["acc"] = state["acc"] + out_proj_fast(os_[og] * linv_[og], og)
            pending_o = [g] if (kind == "V" and g in mxu_o) else []
        run_vpu(last_tok[0], 0, flush=True)
        for og in pending_o:
            state["acc"] = state["acc"] + out_proj_fast(os_[og] * linv_[og], og)
        x = rowsum(state["acc"])
        x = (x + shift) + ffn_fast(x)[1]
        o_ref[1:2, :] = x[0:1, :].astype(o_ref.dtype)

    assert NBLK % CB == 0 and (NBLK - NVP) % CB == 0 and CB >= 2
    out = pl.pallas_call(
        kernel,
        out_shape=jax.ShapeDtypeStruct((B, D), A_x.dtype),
        in_specs=[pl.BlockSpec(memory_space=pl.ANY)] * 7,
        out_specs=pl.BlockSpec(memory_space=pltpu.VMEM),
        scratch_shapes=[
            pltpu.VMEM((B, D), BF16),
            pltpu.VMEM((B, Hkv, S, Dh), BF16),
            pltpu.VMEM((B, Hkv, S, Dh), BF16),
            pltpu.VMEM((Hkv, Dh // 2, S), U32),
            pltpu.VMEM((D, Hq * Dh), BF16),
            pltpu.VMEM((Hq * Dh, D), BF16),
            pltpu.VMEM((D, Fdim), BF16),
            pltpu.VMEM((Fdim, D), BF16),
            pltpu.VMEM((D, Hq * Dh - Q0), F32),
            pltpu.VMEM((len(vpu_o) * G, D), F32),
            pltpu.VMEM((N2 * Dh, D), F32),
            pltpu.VMEM((NF * Dh, D), F32),
            pltpu.VMEM((NF * Dh, D), F32),
            pltpu.VMEM((len(mxu_q), D // 2, G), U32),
            pltpu.VMEM((len(mxu_o), G // 2, D), U32),
            pltpu.VMEM((D // 2, FM), U32),
            pltpu.VMEM(((FM - N2 * Dh) // 2, D), U32),
            pltpu.VMEM((8, Hq * Dh), F32),
            pltpu.VMEM((8, FM), F32),
            pltpu.VMEM((Hkv, 8, Dh), BF16),
            pltpu.VMEM((8, D), F32),
            pltpu.VMEM((Hkv, 8, S), BF16),
            pltpu.VMEM((Hkv, 8, Dh), F32),
            pltpu.VMEM((8, Dh), F32),
            pltpu.VMEM((8, Dh), F32),
            pltpu.VMEM((1, D, Dh), F32),
            pltpu.VMEM((1, N2 * Dh, Dh), F32),
            pltpu.VMEM((2, G, Dh), F32),
            pltpu.VMEM((len(vpu_p), Dh, 2 * NVP * Dh), F32),
            pltpu.VMEM((Hkv, 8, SW), F32),
            pltpu.VMEM((3, G, Dh), F32),
            pltpu.VMEM((8, Dh), jnp.int32),
            pltpu.SemaphoreType.DMA((N_OUTER,)),
        ],
        compiler_params=pltpu.CompilerParams(vmem_limit_bytes=126 * 1024 * 1024),
    )(A_x.reshape(B, D), A_k_cache, A_v_cache, A_wq, A_wo, B_w1, B_w2)
    return out.reshape(B, Sq, D)
```

```python
import jax
import jax.numpy as jnp
from jax import lax
import jax.experimental.pallas as pl
import jax.experimental.pallas.tpu as pltpu

F32 = jnp.float32
BF16 = jnp.bfloat16
U32 = jnp.uint32
NT = (((1,), (1,)), ((), ()))
LOG2E = 1.4426950408889634

G0 = ((0, 4), (4, 6), (6, 7), (7, 8))
GK1 = ((0, 4), (4, 8))
GV1 = ((0, 4), (4, 6), (6, 7))
LAST_CHUNKS = (6144, 1536, 512)
N_OUTER = 2
TCHUNK = 2048

ORDER = "K0 K1 K2 K3 V0 K4 V1 K5 V2 K6 V3 K7 V4 V5 V6 V7".split()
QUEUE = "q2 q3 q4 q5 q6 q7 p0 p1 p2 o0 p3 o1 p4 o2 p5 o3 o4 o5".split()
NVP = 8
CB = 2
RATE = 102.3
LAG = 8
ELAG = 7
EUNIT = 4
ECOST = 5
OLAG = 6
PRE = 8
N2 = 2
NF = 6


@jax.jit
def pallas_interleave_layers__gqa_block_cached__dense_activation_silu__decode_kernel(
    A_x: jax.Array,
    A_k_cache: jax.Array,
    A_v_cache: jax.Array,
    A_wq: jax.Array,
    A_wo: jax.Array,
    B_x: jax.Array,
    B_w1: jax.Array,
    B_w2: jax.Array,
):
    B, Sq, D = A_x.shape
    _, Hkv, S, Dh = A_k_cache.shape
    Hq = A_wq.shape[1] // Dh
    rep = Hq // Hkv
    Fdim = B_w1.shape[1]
    assert (B, Sq, rep, Dh, Hkv) == (2, 1, 4, 128, 8) and D == rep * Dh and sum(LAST_CHUNKS) == S
    G = rep * Dh
    scale = Dh ** -0.5
    eps = 1e-5
    SEM_W = 0
    SEM_0 = 1
    SEM_K1 = SEM_0 + len(G0)
    SEM_V1 = SEM_K1 + len(GK1)
    SEM_L = SEM_V1 + len(GV1)
    NL = len(LAST_CHUNKS)
    n_in = NL - N_OUTER
    NSEM_IN = SEM_L + n_in
    lc_off = [sum(LAST_CHUNKS[:i]) for i in range(NL)]
    HL = Hkv - 1
    vpu_q = [g for g in range(Hkv) if "q%d" % g in QUEUE]
    vpu_o = [g for g in range(Hkv) if "o%d" % g in QUEUE]
    vpu_p = [g for g in range(Hkv) if "p%d" % g in QUEUE]
    mxu_q = [g for g in range(Hkv) if g not in vpu_q]
    mxu_o = [g for g in range(Hkv) if g not in vpu_o]
    assert vpu_q == list(range(vpu_q[0], Hkv)) and vpu_o == list(range(len(vpu_o)))
    assert vpu_p == list(range(len(vpu_p))) and set(vpu_p) <= set(vpu_o) and HL in mxu_o
    Q0 = vpu_q[0] * G
    SW = S // 2
    NBLK = SW // Dh
    VP0 = SW - NVP * Dh
    NKB = D // 8
    FM = Fdim - NF * Dh

    def kernel(x_hbm, k_hbm, v_hbm, wq_hbm, wo_hbm, w1_hbm, w2_hbm, o_ref,
               xbuf, kbuf, vbuf, ktbuf, wq, wo, w1, w2, wqf, wof, w2f, w1t, w2g,
               wqp, wop, w1p, w2p, cq, c1, q_scr, acc_scr, p_scr, l_scr, o_scr, c_scr,
               xb_scr, hb_scr, ob_scr, vtf, pf_scr, pa_scr, z_scr, osems):
        row8 = lax.broadcasted_iota(jnp.int32, (8, Dh), 0)
        rowg = lax.broadcasted_iota(jnp.int32, (8, G), 0)
        colg = lax.broadcasted_iota(jnp.int32, (8, G), 1)
        diag_mask = rowg == (colg // Dh)
        eye = (lax.broadcasted_iota(jnp.int32, (Dh, Dh), 0) == lax.broadcasted_iota(jnp.int32, (Dh, Dh), 1))

        def load_v(h, off, n):
            return pltpu.bitcast(vbuf.bitcast(U32)[1, h, off // 2:(off + n) // 2, :], BF16)

        def load_kt(h, off, n):
            return pltpu.bitcast(ktbuf[h, :, off:off + n], BF16)

        def pick_rows(qa):
            qg = jnp.zeros((8, Dh), F32)
            for j in range(rep):
                qg = jnp.where(row8 == j, qa[:, j * Dh:(j + 1) * Dh], qg)
            return qg

        def diag_lhs(o):
            o4 = jnp.concatenate([o] * rep, axis=1)
            return jnp.where(diag_mask, o4, 0.0).astype(BF16)

        def out_proj_fast(o, g):
            return jnp.dot(diag_lhs(o), pltpu.bitcast(wop[mxu_o.index(g)], BF16), preferred_element_type=F32)

        def rowsum(a):
            return jnp.broadcast_to(jnp.sum(a, axis=0, keepdims=True), a.shape)

        def lanesum(a):
            return jnp.broadcast_to(jnp.sum(a, axis=1, keepdims=True), (a.shape[0], Dh))

        def col_bcast(row):
            return lanesum(jnp.where(eye, jnp.broadcast_to(row, (Dh, Dh)), 0.0))

        def cp_vl(i, sem):
            sl = pl.ds(lc_off[i], LAST_CHUNKS[i])
            return pltpu.make_async_copy(v_hbm.at[1, HL, sl], vbuf.at[1, HL, sl], sem)

        def pv_last(i):
            sl = slice(lc_off[i], lc_off[i] + LAST_CHUNKS[i])
            return jnp.dot(p_scr[HL, :, sl], vbuf[1, HL, sl, :], preferred_element_type=F32)

        cps_out = [cp_vl(n_in + i, osems.at[i]) for i in range(N_OUTER)]

        def streaming_part(sems):
            def cp_kv(hbm, buf, b, grp, sem):
                sl = pl.ds(grp[0], grp[1] - grp[0])
                return pltpu.make_async_copy(hbm.at[b, sl], buf.at[b, sl], sems.at[sem])
            cps_w = [pltpu.make_async_copy(s_, d_, sems.at[SEM_W]) for s_, d_ in
                     ((x_hbm, xbuf), (wq_hbm, wq), (wo_hbm, wo), (w1_hbm, w1), (w2_hbm, w2))]
            cps_0 = [(cp_kv(k_hbm, kbuf, 0, g, SEM_0 + i), cp_kv(v_hbm, vbuf, 0, g, SEM_0 + i))
                     for i, g in enumerate(G0)]
            cps_k1 = [cp_kv(k_hbm, kbuf, 1, g, SEM_K1 + i) for i, g in enumerate(GK1)]
            cps_v1 = [cp_kv(v_hbm, vbuf, 1, g, SEM_V1 + i) for i, g in enumerate(GV1)]
            cps_l = [cp_vl(i, sems.at[SEM_L + i]) for i in range(n_in)]
            for c in cps_w:
                c.start()
            for a, b_ in cps_0:
                a.start()
                b_.start()
            for c in cps_k1 + cps_v1 + cps_l + cps_out:
                c.start()

            def layernorm(x):
                xc = x - jnp.mean(x, axis=-1, keepdims=True)
                return xc * lax.rsqrt(jnp.mean(xc * xc, axis=-1, keepdims=True) + eps)

            def compute_q(x):
                xn = layernorm(x).astype(BF16)
                for g in range(Hkv):
                    qa = jnp.dot(xn, wq[:, g * G:(g + 1) * G], preferred_element_type=F32) * scale
                    q_scr[g] = pick_rows(qa).astype(BF16)

            def softmax_parts(s):
                p = jnp.exp(s - jnp.max(s, axis=1, keepdims=True))
                return p.astype(BF16), jnp.sum(p, axis=1, keepdims=True)

            def out_proj(o, h):
                w = wo[pl.ds(pl.multiple_of(h * G, G), G), :]
                return jnp.dot(diag_lhs(o), w, preferred_element_type=F32)

            def attn_head0(h, c):
                s = lax.dot_general(q_scr[h], kbuf[0, h], NT, preferred_element_type=F32)
                p, l = softmax_parts(s)
                o = jnp.dot(p, vbuf[0, h], preferred_element_type=F32)
                acc_scr[...] += out_proj(o / l, h)
                return c

            def kside1(h, c):
                s = lax.dot_general(q_scr[h], kbuf[1, h], NT, preferred_element_type=F32)
                p, l = softmax_parts(s)
                p_scr[h] = p
                l_scr[h] = jnp.broadcast_to(1.0 / l, (8, Dh))

                def tr(i, carry):
                    off = pl.multiple_of(i * TCHUNK, TCHUNK)
                    ktbuf[h, :, pl.ds(off, TCHUNK)] = pltpu.bitcast(kbuf[1, h, pl.ds(off, TCHUNK), :].T, U32)
                    return carry
                lax.fori_loop(0, S // TCHUNK, tr, 0)
                return c

            def vside1(h, c):
                o = jnp.dot(p_scr[h], vbuf[1, h], preferred_element_type=F32)
                acc_scr[...] += out_proj(o * l_scr[h], h)
                return c

            def vside1t(h, c):
                vside1(h, c)
                for hf in range(2):
                    vtf[h, :, hf * NVP * Dh:(hf + 1) * NVP * Dh] = (
                        vbuf[1, h, hf * SW + VP0:(hf + 1) * SW, :].astype(F32).T)
                return c

            def ffn(x):
                hh = jnp.dot(layernorm(x).astype(BF16), w1[...], preferred_element_type=F32)
                hh = hh * jax.nn.sigmoid(hh)
                return jnp.dot(hh.astype(BF16), w2[...], preferred_element_type=F32)

            for c in cps_w:
                c.wait()

            def prep_q(i, c):
                off = pl.multiple_of(i * 64, 64)
                wqf[pl.ds(off, 64), :] = wq[pl.ds(off, 64), Q0:].astype(F32)
                return c
            lax.fori_loop(0, D // 64, prep_q, 0)

            def prep_o(i, c):
                off = pl.multiple_of(i * G, G)
                wof[pl.ds(off, G), :] = wo[pl.ds(off, G), :].astype(F32)
                return c
            lax.fori_loop(0, len(vpu_o), prep_o, 0)
            for i, g in enumerate(mxu_q):
                wqp[i] = pltpu.bitcast(wq[:, g * G:(g + 1) * G], U32)
            for i, g in enumerate(mxu_o):
                wop[i] = pltpu.bitcast(wo[g * G:(g + 1) * G, :], U32)
            w1p[...] = pltpu.bitcast(w1[:, 0:FM], U32)
            w2p[...] = pltpu.bitcast(w2[N2 * Dh:FM, :], U32)
            for i in range(N2):
                w2f[i * Dh:(i + 1) * Dh, :] = w2[i * Dh:(i + 1) * Dh, :].astype(F32)
            w1t[...] = w1[:, FM:].astype(F32).T
            w2g[...] = w2[FM:, :].astype(F32)
            w1t[...] = w1t[...] - jnp.mean(w1t[...], axis=1, keepdims=True)
            ones8 = jnp.ones((8, D), BF16)
            cq[...] = jnp.dot(ones8, wq[...], preferred_element_type=F32)
            c1[...] = jnp.dot(ones8, w1[:, 0:FM], preferred_element_type=F32)
            z_scr[...] = jnp.zeros_like(z_scr)

            x = jnp.broadcast_to(xbuf[0:1, :].astype(F32), (8, D))
            compute_q(x)
            acc_scr[...] = jnp.zeros_like(acc_scr)
            for i, g in enumerate(G0):
                cps_0[i][0].wait()
                cps_0[i][1].wait()
                lax.fori_loop(g[0], g[1], attn_head0, 0)
            x = x + rowsum(acc_scr[...])
            x = x + ffn(x)
            compute_q(x)
            acc_scr[...] = jnp.zeros_like(acc_scr)
            lax.fori_loop(0, Hkv, attn_head0, 0)
            x = x + rowsum(acc_scr[...])
            x = x + ffn(x)
            o_ref[0:1, :] = x[0:1, :].astype(o_ref.dtype)
            x = jnp.broadcast_to(xbuf[1:2, :].astype(F32), (8, D))
            compute_q(x)
            for i, g in enumerate(GK1):
                cps_k1[i].wait()
                lax.fori_loop(g[0], g[1], kside1, 0)
            c0 = jnp.mean(x, axis=-1, keepdims=True)
            c_scr[...] = jnp.broadcast_to(c0, (8, Dh))
            acc_scr[...] = jnp.where(rowg == 0, x - c0, 0.0)
            for i, g in enumerate(GV1):
                cps_v1[i].wait()
                assert (g[0] in vpu_p) == (g[1] - 1 in vpu_p)
                lax.fori_loop(g[0], g[1], vside1t if g[0] in vpu_p else vside1, 0)
            o_scr[...] = jnp.zeros_like(o_scr)
            for i in range(n_in):
                cps_l[i].wait()
                o_scr[...] += pv_last(i)

        pl.run_scoped(streaming_part, pltpu.SemaphoreType.DMA((NSEM_IN,)))

        for i in range(N_OUTER - 1):
            cps_out[i].wait()
            o_scr[...] += pv_last(n_in + i)
        cps_out[-1].wait()
        o = o_scr[...] + pv_last(NL - 1)

        zero_i = z_scr[...]

        def mk_tok(v):
            return lax.bitcast_convert_type(lax.bitcast_convert_type(v, jnp.int32) & zero_i, F32)

        def sum_all(vs):
            t = vs[0]
            for v in vs[1:]:
                t = t + v
            return t

        def blocks(a):
            return [a[:, c * Dh:(c + 1) * Dh] for c in range(a.shape[1] // Dh)]

        def halves(a):
            return [a[0:8, :], a[8:16, :]]

        def stats(x):
            s1 = sum_all(blocks(x))
            s2 = sum_all(blocks(x * x))
            m = jnp.sum(s1, axis=-1, keepdims=True) * (1.0 / D)
            m2 = jnp.sum(s2, axis=-1, keepdims=True) * (1.0 / D)
            v = jnp.maximum(m2 - m * m, 0.0)
            return m, lax.rsqrt(v + eps), mk_tok(s1 + s2)

        def silu_half(a):
            return a + a * jnp.tanh(a)

        tile_cache = {}

        def tile_rows(tok, n):
            if (id(tok), n) not in tile_cache:
                tile_cache[(id(tok), n)] = (tok, jnp.concatenate([tok] * n, axis=0))
            return tile_cache[(id(tok), n)][1]

        class MatVec:
            def __init__(self, xb_ref, slot, w_ref, row0, col0, nkb=NKB):
                self.xb_ref, self.slot, self.w_ref, self.row0, self.col0 = xb_ref, slot, w_ref, row0, col0
                self.acc = None
                self.kb = 0
                self.nkb = nkb

            def step(self, n, tok):
                xv = self.xb_ref[self.slot, self.kb * 8:(self.kb + n) * 8, :]
                if tok is not None:
                    xv = xv + tile_rows(tok, n)
                self.fma(self.kb, xv)
                self.kb += n

            def fma(self, kb, xv):
                r0, n = self.row0 + kb * 8, xv.shape[0]
                t = jnp.concatenate([xv] * rep, axis=1) * self.w_ref[r0:r0 + n, self.col0:self.col0 + G]
                for i in range(0, n, 8):
                    ti = t[i:i + 8, :] if n > 8 else t
                    self.acc = ti if self.acc is None else self.acc + ti

        def ffn_fast(x):
            m, r, _ = stats(x)
            rh = 0.5 * r
            y = jnp.dot(x.astype(BF16), pltpu.bitcast(w1p[...], BF16), preferred_element_type=F32)
            h1 = silu_half((y - m * c1[...]) * rh)
            out = sum_all([
                jnp.dot(h1[:, k0:k0 + Dh].astype(BF16),
                        pltpu.bitcast(w2p[(k0 - N2 * Dh) // 2:(k0 - N2 * Dh + Dh) // 2, :], BF16),
                        preferred_element_type=F32)
                for k0 in range(N2 * Dh, FM, Dh)])
            ta = MatVec(None, 0, w2g, 0, 0)
            for kb in range(NF * 16):
                yc = lanesum(sum_all(blocks(w1t[kb * 8:kb * 8 + 8, :] * x)))
                ta.fma(kb, silu_half(yc * rh))
            for c in range(N2):
                hb_scr[0, c * Dh:(c + 1) * Dh, :] = col_bcast(h1[0:1, c * Dh:(c + 1) * Dh])
            tb = MatVec(hb_scr, 0, w2f, 0, 0, nkb=N2 * 16)
            while tb.kb < tb.nkb:
                tb.step(4, None)
            return m, out + rowsum(ta.acc + tb.acc)

        x = rowsum(acc_scr[...] + out_proj_fast(o * l_scr[HL], HL))
        m1, y1 = ffn_fast(x)
        x = (x - m1) + y1

        m, r, stok = stats(x)
        rs = r * (scale * LOG2E)

        def fin_q(qa, g):
            return pick_rows((qa - m * cq[:, g * G:(g + 1) * G]) * rs)
        x16 = x.astype(BF16)
        for c, xr in enumerate(blocks(x)):
            if c == D // Dh - 1:
                xr = xr + stok
            xb_scr[0, c * Dh:(c + 1) * Dh, :] = col_bcast(xr[0:1, :])

        qs, os_, linv_, mx_ = {}, {}, {}, {}
        state = {"acc": jnp.where(rowg == 0, x - m, 0.0)}
        shift = c_scr[:, 0:1] + m1 + m
        live, fin = [None], []
        chunk_no = [0]
        k_at, os_at, e_at = {}, {}, {}
        todo = list(QUEUE)
        stack, etasks, due = [], [], []
        credit = [0.0]
        e_started, ep_ok = set(), set()
        last_tok = [None]

        def matvec_gen(mv):
            while mv.kb < NKB:
                tok = yield 36
                mv.step(4, tok)
                live[0] = mv

        def q_gen(g):
            mv = MatVec(xb_scr, 0, wqf, 0, g * G - Q0)
            yield from matvec_gen(mv)
            qs[g] = fin_q(rowsum(mv.acc), g)
            return mk_tok(qs[g])

        def e_gen(g):
            m_ = jnp.broadcast_to(jnp.max(mx_[g], axis=1, keepdims=True), (8, Dh))
            m_ = jnp.maximum(m_, pltpu.roll(m_, 4, 0))
            lp = None
            order_ = list(range(NBLK))
            if g in vpu_p:
                order_ = order_[NBLK - NVP:] + order_[:NBLK - NVP]
            for u in range(0, NBLK, EUNIT):
                tok = yield ECOST * EUNIT
                mm = m_ if tok is None else m_ + tok
                for c in order_[u:u + EUNIT]:
                    pc = jnp.exp2(pf_scr[g, :, c * Dh:(c + 1) * Dh] - mm)
                    pf_scr[g, :, c * Dh:(c + 1) * Dh] = pc
                    lp = pc if lp is None else lp + pc
                fin.append(lp)
                if g in vpu_p and u + EUNIT >= NVP:
                    ep_ok.add(g)
            lp = lp + pltpu.roll(lp, 4, 0)
            linv_[g] = jnp.broadcast_to(1.0 / jnp.sum(lp, axis=1, keepdims=True), (8, Dh))
            e_at[g] = chunk_no[0]

        def p_gen(g):
            slot = g % 3
            for dg in range(Dh // 16):
                accs = [None] * rep
                for blk in range(NVP):
                    for hf in range(2):
                        tok = yield 20
                        col = (hf * NVP + blk) * Dh
                        vt = vtf[g, dg * 16:dg * 16 + 16, col:col + Dh]
                        if tok is not None:
                            vt = vt + tile_rows(tok, 2)
                        for j in range(rep):
                            r_ = hf * 4 + j
                            t = pf_scr[g, r_:r_ + 1, VP0 + blk * Dh:VP0 + (blk + 1) * Dh] * vt
                            accs[j] = t if accs[j] is None else accs[j] + t
                        live[0] = list(accs)
                for j in range(rep):
                    pa_scr[slot, j * Dh + dg * 16:j * Dh + dg * 16 + 16, :] = accs[j]
                fin.extend(halves(sum_all(accs)))
                live[0] = None

        def o_gen(g):
            slot = g % 2
            linv = linv_[g]
            for j in range(rep):
                tok = yield 48
                orow = os_[g] if tok is None else os_[g] + tok
                z = jnp.where(eye, jnp.broadcast_to(orow[j:j + 1, :], (Dh, Dh)), 0.0)
                if g in vpu_p:
                    z = z + pa_scr[g % 3, j * Dh:(j + 1) * Dh, :]
                ob_scr[slot, j * Dh:(j + 1) * Dh, :] = lanesum(z) * jnp.broadcast_to(linv[j:j + 1, :], (Dh, Dh))
            mv = MatVec(ob_scr, slot, wof, g * G, 0)
            yield from matvec_gen(mv)
            state["acc"] = state["acc"] + mv.acc
            return mk_tok(sum_all(blocks(mv.acc)))

        def ready(t):
            k_, g_ = t[0], int(t[1])
            if k_ == "p":
                return g_ in ep_ok
            if k_ == "o":
                return g_ in os_ and chunk_no[0] >= os_at[g_] + OLAG
            return True

        def run_vpu(tok, budget, force_e=None, flush=False):
            live[0] = None
            for g_, a_ in k_at.items():
                if g_ not in e_started and (chunk_no[0] >= a_ + ELAG or g_ == force_e):
                    e_started.add(g_)
                    gen = e_gen(g_)
                    etasks.append([gen, next(gen)])
            credit[0] = 1e12 if flush else min(credit[0] + budget, 2 * RATE)
            while etasks:
                credit[0] -= etasks[0][1]
                try:
                    etasks[0][1] = etasks[0][0].send(tok)
                except StopIteration:
                    etasks.pop(0)
                if not flush:
                    break
            while True:
                if not stack:
                    if not todo or (not flush and not ready(todo[0])):
                        break
                    t = todo.pop(0)
                    gen = {"q": q_gen, "p": p_gen, "o": o_gen}[t[0]](int(t[1]))
                    stack.append([gen, next(gen)])
                cur = stack[-1]
                if credit[0] < cur[1]:
                    break
                credit[0] -= cur[1]
                try:
                    cur[1] = cur[0].send(tok)
                except StopIteration as e:
                    if e.value is not None:
                        due.append((chunk_no[0] + LAG, e.value))
                    live[0] = None
                    stack.pop()
            cov = list(fin)
            if isinstance(live[0], MatVec):
                cov += blocks(live[0].acc)
            elif live[0]:
                cov += halves(sum_all(live[0]))
            del fin[:]
            if cov and not flush:
                due.append((chunk_no[0] + LAG, mk_tok(sum_all(cov))))

        def take_due():
            toks = [t for c_, t in due if c_ <= chunk_no[0]]
            due[:] = [(c_, t) for c_, t in due if c_ > chunk_no[0]]
            return sum_all(toks) if toks else None

        def qk2(g):
            while g not in qs:
                run_vpu(last_tok[0], RATE)
            qq = qs[g]
            mx = None
            n = CB * Dh
            for c0 in range(0, NBLK, CB):
                dtok = take_due()
                if c0 == 0 or dtok is not None:
                    if dtok is not None:
                        qq = qq + dtok
                    qa = qq.astype(BF16)
                    qb = pltpu.roll(qq, 4, 0).astype(BF16)
                sc = (jnp.dot(qa, load_kt(g, c0 * Dh, n), preferred_element_type=F32)
                      + jnp.dot(qb, load_kt(g, SW + c0 * Dh, n), preferred_element_type=F32))
                pf_scr[g, :, c0 * Dh:c0 * Dh + n] = sc
                for v in blocks(sc):
                    mx = v if mx is None else jnp.maximum(mx, v)
                chunk_no[0] += 1
                last_tok[0] = mk_tok(sc[:, 0:Dh])
                run_vpu(last_tok[0], RATE)
            mx_[g] = mx

        def pv2(g):
            while g not in e_at:
                run_vpu(last_tok[0], RATE, force_e=g)
            nb = NBLK - (NVP if g in vpu_p else 0)
            o1 = None
            o2 = None
            n = CB * Dh
            for c0 in range(0, nb, CB):
                pc = pf_scr[g, :, c0 * Dh:c0 * Dh + n]
                dtok = take_due()
                if dtok is not None:
                    pc = jnp.concatenate([pc[:, 0:Dh] + dtok, pc[:, Dh:]], axis=1)
                pc = pc.astype(BF16)
                oc = jnp.dot(pc, load_v(g, c0 * Dh, n), preferred_element_type=F32)
                o1 = oc if o1 is None else o1 + oc
                oc2 = jnp.dot(pc, load_v(g, SW + c0 * Dh, n), preferred_element_type=F32)
                o2 = oc2 if o2 is None else o2 + oc2
                chunk_no[0] += 1
                last_tok[0] = mk_tok(oc)
                run_vpu(last_tok[0], RATE)
            return o1 + pltpu.roll(o2, 4, 0)

        for g in mxu_q:
            qs[g] = fin_q(jnp.dot(x16, pltpu.bitcast(wqp[mxu_q.index(g)], BF16), preferred_element_type=F32), g)
        for _ in range(PRE):
            run_vpu(None, RATE)
        pending_o = []
        for ph in ORDER:
            kind, g = ph[0], int(ph[1])
            if kind == "K":
                qk2(g)
                k_at[g] = chunk_no[0]
            else:
                os_[g] = pv2(g)
                os_at[g] = chunk_no[0]
            for og in pending_o:
                state["acc"] = state["acc"] + out_proj_fast(os_[og] * linv_[og], og)
            pending_o = [g] if (kind == "V" and g in mxu_o) else []
        run_vpu(last_tok[0], 0, flush=True)
        for og in pending_o:
            state["acc"] = state["acc"] + out_proj_fast(os_[og] * linv_[og], og)
        x = rowsum(state["acc"])
        x = (x + shift) + ffn_fast(x)[1]
        o_ref[1:2, :] = x[0:1, :].astype(o_ref.dtype)

    assert NBLK % CB == 0 and (NBLK - NVP) % CB == 0 and CB >= 2
    out = pl.pallas_call(
        kernel,
        out_shape=jax.ShapeDtypeStruct((B, D), A_x.dtype),
        in_specs=[pl.BlockSpec(memory_space=pl.ANY)] * 7,
        out_specs=pl.BlockSpec(memory_space=pltpu.VMEM),
        scratch_shapes=[
            pltpu.VMEM((B, D), BF16),
            pltpu.VMEM((B, Hkv, S, Dh), BF16),
            pltpu.VMEM((B, Hkv, S, Dh), BF16),
            pltpu.VMEM((Hkv, Dh // 2, S), U32),
            pltpu.VMEM((D, Hq * Dh), BF16),
            pltpu.VMEM((Hq * Dh, D), BF16),
            pltpu.VMEM((D, Fdim), BF16),
            pltpu.VMEM((Fdim, D), BF16),
            pltpu.VMEM((D, Hq * Dh - Q0), F32),
            pltpu.VMEM((len(vpu_o) * G, D), F32),
            pltpu.VMEM((N2 * Dh, D), F32),
            pltpu.VMEM((NF * Dh, D), F32),
            pltpu.VMEM((NF * Dh, D), F32),
            pltpu.VMEM((len(mxu_q), D // 2, G), U32),
            pltpu.VMEM((len(mxu_o), G // 2, D), U32),
            pltpu.VMEM((D // 2, FM), U32),
            pltpu.VMEM(((FM - N2 * Dh) // 2, D), U32),
            pltpu.VMEM((8, Hq * Dh), F32),
            pltpu.VMEM((8, FM), F32),
            pltpu.VMEM((Hkv, 8, Dh), BF16),
            pltpu.VMEM((8, D), F32),
            pltpu.VMEM((Hkv, 8, S), BF16),
            pltpu.VMEM((Hkv, 8, Dh), F32),
            pltpu.VMEM((8, Dh), F32),
            pltpu.VMEM((8, Dh), F32),
            pltpu.VMEM((1, D, Dh), F32),
            pltpu.VMEM((1, N2 * Dh, Dh), F32),
            pltpu.VMEM((2, G, Dh), F32),
            pltpu.VMEM((len(vpu_p), Dh, 2 * NVP * Dh), F32),
            pltpu.VMEM((Hkv, 8, SW), F32),
            pltpu.VMEM((3, G, Dh), F32),
            pltpu.VMEM((8, Dh), jnp.int32),
            pltpu.SemaphoreType.DMA((N_OUTER,)),
        ],
        compiler_params=pltpu.CompilerParams(vmem_limit_bytes=126 * 1024 * 1024),
    )(A_x.reshape(B, D), A_k_cache, A_v_cache, A_wq, A_wo, B_w1, B_w2)
    return out.reshape(B, Sq, D)
```

```python
import jax
import jax.numpy as jnp
from jax import lax
import jax.experimental.pallas as pl
import jax.experimental.pallas.tpu as pltpu

F32 = jnp.float32
BF16 = jnp.bfloat16
U32 = jnp.uint32
NT = (((1,), (1,)), ((), ()))
LOG2E = 1.4426950408889634

G0 = ((0, 4), (4, 6), (6, 7), (7, 8))
GK1 = ((0, 4), (4, 8))
GV1 = ((0, 4), (4, 6), (6, 7))
LAST_CHUNKS = (6144, 1536, 512)
TCHUNK = 2048

ORDER = "K0 K1 K2 K3 V0 K4 V1 K5 V2 K6 V3 K7 V4 V5 V6 V7".split()
QUEUE = "q2 q3 q4 q5 q6 q7 p0 p1 p2 o0 p3 o1 p4 o2 p5 o3 o4 o5".split()
NVP = 8
CB = 2
RATE = 102.3
LAG = 8
ELAG = 7
EUNIT = 4
ECOST = 5
OLAG = 6
PRE = 8
N2 = 2
NF = 6


@jax.jit
def pallas_interleave_layers__gqa_block_cached__dense_activation_silu__decode_kernel(
    A_x: jax.Array,
    A_k_cache: jax.Array,
    A_v_cache: jax.Array,
    A_wq: jax.Array,
    A_wo: jax.Array,
    B_x: jax.Array,
    B_w1: jax.Array,
    B_w2: jax.Array,
):
    B, Sq, D = A_x.shape
    _, Hkv, S, Dh = A_k_cache.shape
    Hq = A_wq.shape[1] // Dh
    rep = Hq // Hkv
    Fdim = B_w1.shape[1]
    assert (B, Sq, rep, Dh, Hkv) == (2, 1, 4, 128, 8) and D == rep * Dh and sum(LAST_CHUNKS) == S
    G = rep * Dh
    scale = Dh ** -0.5
    eps = 1e-5
    SEM_W = 0
    SEM_0 = 1
    SEM_K1 = SEM_0 + len(G0)
    SEM_V1 = SEM_K1 + len(GK1)
    SEM_L = SEM_V1 + len(GV1)
    NL = len(LAST_CHUNKS)
    NSEM = SEM_L + NL
    lc_off = [sum(LAST_CHUNKS[:i]) for i in range(NL)]
    HL = Hkv - 1
    vpu_q = [g for g in range(Hkv) if "q%d" % g in QUEUE]
    vpu_o = [g for g in range(Hkv) if "o%d" % g in QUEUE]
    vpu_p = [g for g in range(Hkv) if "p%d" % g in QUEUE]
    mxu_q = [g for g in range(Hkv) if g not in vpu_q]
    mxu_o = [g for g in range(Hkv) if g not in vpu_o]
    assert vpu_q == list(range(vpu_q[0], Hkv)) and vpu_o == list(range(len(vpu_o)))
    assert vpu_p == list(range(len(vpu_p))) and set(vpu_p) <= set(vpu_o) and HL in mxu_o
    Q0 = vpu_q[0] * G
    SW = S // 2
    NBLK = SW // Dh
    VP0 = SW - NVP * Dh
    NKB = D // 8
    FM = Fdim - NF * Dh

    def body(x_hbm, k_hbm, v_hbm, wq_hbm, wo_hbm, w1_hbm, w2_hbm, o_ref,
             xbuf, k1buf, v1buf, wq, wo, w1, w2, wqf, wof, w2f, w1t, w2g,
             wqp, wop, w1p, w2p, cq, c1, q_scr, acc_scr, p_scr, l_scr, o_scr, c_scr,
             xb_scr, hb_scr, ob_scr, pf_scr, pa_scr, z_scr, sems):
        def cp_kv(hbm, buf, b, grp, sem):
            sl = pl.ds(grp[0], grp[1] - grp[0])
            return pltpu.make_async_copy(hbm.at[b, sl], buf.at[sl], sems.at[sem])

        def cp_vl(i):
            sl = pl.ds(lc_off[i], LAST_CHUNKS[i])
            return pltpu.make_async_copy(v_hbm.at[1, HL, sl], v1buf.at[HL, sl], sems.at[SEM_L + i])

        cps_w = [pltpu.make_async_copy(s_, d_, sems.at[SEM_W]) for s_, d_ in
                 ((x_hbm, xbuf), (wq_hbm, wq), (wo_hbm, wo), (w1_hbm, w1), (w2_hbm, w2))]
        cps_k1 = [cp_kv(k_hbm, k1buf, 1, g, SEM_K1 + i) for i, g in enumerate(GK1)]
        cps_v1 = [cp_kv(v_hbm, v1buf, 1, g, SEM_V1 + i) for i, g in enumerate(GV1)]
        cps_l = [cp_vl(i) for i in range(NL)]
        for c in cps_w:
            c.start()

        row8 = lax.broadcasted_iota(jnp.int32, (8, Dh), 0)
        rowg = lax.broadcasted_iota(jnp.int32, (8, G), 0)
        colg = lax.broadcasted_iota(jnp.int32, (8, G), 1)
        diag_mask = rowg == (colg // Dh)
        eye = (lax.broadcasted_iota(jnp.int32, (Dh, Dh), 0) == lax.broadcasted_iota(jnp.int32, (Dh, Dh), 1))

        def pick_rows(qa):
            qg = jnp.zeros((8, Dh), F32)
            for j in range(rep):
                qg = jnp.where(row8 == j, qa[:, j * Dh:(j + 1) * Dh], qg)
            return qg

        def diag_lhs(o):
            o4 = jnp.concatenate([o] * rep, axis=1)
            return jnp.where(diag_mask, o4, 0.0).astype(BF16)

        def out_proj_fast(o, g):
            return jnp.dot(diag_lhs(o), pltpu.bitcast(wop[mxu_o.index(g)], BF16), preferred_element_type=F32)

        def rowsum(a):
            return jnp.broadcast_to(jnp.sum(a, axis=0, keepdims=True), a.shape)

        def lanesum(a):
            return jnp.broadcast_to(jnp.sum(a, axis=1, keepdims=True), (a.shape[0], Dh))

        def col_bcast(row):
            return lanesum(jnp.where(eye, jnp.broadcast_to(row, (Dh, Dh)), 0.0))

        def layernorm(x):
            xc = x - jnp.mean(x, axis=-1, keepdims=True)
            return xc * lax.rsqrt(jnp.mean(xc * xc, axis=-1, keepdims=True) + eps)

        def compute_q(x):
            xn = layernorm(x).astype(BF16)
            for g in range(Hkv):
                qa = jnp.dot(xn, wq[:, g * G:(g + 1) * G], preferred_element_type=F32) * scale
                q_scr[g] = pick_rows(qa).astype(BF16)

        def softmax_parts(s):
            p = jnp.exp(s - jnp.max(s, axis=1, keepdims=True))
            return p.astype(BF16), jnp.sum(p, axis=1, keepdims=True)

        def out_proj(o, h):
            w = wo[pl.ds(pl.multiple_of(h * G, G), G), :]
            return jnp.dot(diag_lhs(o), w, preferred_element_type=F32)

        def ffn(x):
            hh = jnp.dot(layernorm(x).astype(BF16), w1[...], preferred_element_type=F32)
            hh = hh * jax.nn.sigmoid(hh)
            return jnp.dot(hh.astype(BF16), w2[...], preferred_element_type=F32)

        def part_a(k0buf, v0buf):
            cps_0 = [(cp_kv(k_hbm, k0buf, 0, g, SEM_0 + i), cp_kv(v_hbm, v0buf, 0, g, SEM_0 + i))
                     for i, g in enumerate(G0)]
            for a, b_ in cps_0:
                a.start()
                b_.start()
            for c in cps_k1 + cps_v1 + cps_l:
                c.start()

            def attn_head0(h, c):
                s = lax.dot_general(q_scr[h], k0buf[h], NT, preferred_element_type=F32)
                p, l = softmax_parts(s)
                o = jnp.dot(p, v0buf[h], preferred_element_type=F32)
                acc_scr[...] += out_proj(o / l, h)
                return c

            for c in cps_w:
                c.wait()

            def prep_q(i, c):
                off = pl.multiple_of(i * 64, 64)
                wqf[pl.ds(off, 64), :] = wq[pl.ds(off, 64), Q0:].astype(F32)
                return c
            lax.fori_loop(0, D // 64, prep_q, 0)

            def prep_o(i, c):
                off = pl.multiple_of(i * G, G)
                wof[pl.ds(off, G), :] = wo[pl.ds(off, G), :].astype(F32)
                return c
            lax.fori_loop(0, len(vpu_o), prep_o, 0)
            for i, g in enumerate(mxu_q):
                wqp[i] = pltpu.bitcast(wq[:, g * G:(g + 1) * G], U32)
            for i, g in enumerate(mxu_o):
                wop[i] = pltpu.bitcast(wo[g * G:(g + 1) * G, :], U32)
            w1p[...] = pltpu.bitcast(w1[:, 0:FM], U32)
            w2p[...] = pltpu.bitcast(w2[N2 * Dh:FM, :], U32)
            for i in range(N2):
                w2f[i * Dh:(i + 1) * Dh, :] = w2[i * Dh:(i + 1) * Dh, :].astype(F32)
            w1t[...] = w1[:, FM:].astype(F32).T
            w2g[...] = w2[FM:, :].astype(F32)
            w1t[...] = w1t[...] - jnp.mean(w1t[...], axis=1, keepdims=True)
            ones8 = jnp.ones((8, D), BF16)
            cq[...] = jnp.dot(ones8, wq[...], preferred_element_type=F32)
            c1[...] = jnp.dot(ones8, w1[:, 0:FM], preferred_element_type=F32)
            z_scr[...] = jnp.zeros_like(z_scr)

            x = jnp.broadcast_to(xbuf[0:1, :].astype(F32), (8, D))
            compute_q(x)
            acc_scr[...] = jnp.zeros_like(acc_scr)
            for i, g in enumerate(G0):
                cps_0[i][0].wait()
                cps_0[i][1].wait()
                lax.fori_loop(g[0], g[1], attn_head0, 0)
            x = x + rowsum(acc_scr[...])
            x = x + ffn(x)
            compute_q(x)
            acc_scr[...] = jnp.zeros_like(acc_scr)
            lax.fori_loop(0, Hkv, attn_head0, 0)
            x = x + rowsum(acc_scr[...])
            x = x + ffn(x)
            o_ref[0:1, :] = x[0:1, :].astype(o_ref.dtype)

        pl.run_scoped(part_a, pltpu.VMEM((Hkv, S, Dh), BF16), pltpu.VMEM((Hkv, S, Dh), BF16))

        def part_b(ktbuf, vpk, vtf):
            def load_v(h, off, n):
                return pltpu.bitcast(vpk[h, off // 2:(off + n) // 2, :], BF16)

            def load_kt(h, off, n):
                return pltpu.bitcast(ktbuf[h, :, off:off + n], BF16)

            def pv_last(i):
                o_, n = lc_off[i], LAST_CHUNKS[i]
                v = v1buf[HL, o_:o_ + n, :]
                vpk[HL, o_ // 2:(o_ + n) // 2, :] = pltpu.bitcast(v, U32)
                return jnp.dot(p_scr[HL, :, o_:o_ + n], v, preferred_element_type=F32)

            def kside1(h, c):
                s = lax.dot_general(q_scr[h], k1buf[h], NT, preferred_element_type=F32)
                p, l = softmax_parts(s)
                p_scr[h] = p
                l_scr[h] = jnp.broadcast_to(1.0 / l, (8, Dh))

                def tr(i, carry):
                    off = pl.multiple_of(i * TCHUNK, TCHUNK)
                    ktbuf[h, :, pl.ds(off, TCHUNK)] = pltpu.bitcast(k1buf[h, pl.ds(off, TCHUNK), :].T, U32)
                    return carry
                lax.fori_loop(0, S // TCHUNK, tr, 0)
                return c

            def vside1(h, c):
                v = v1buf[h]
                vpk[h] = pltpu.bitcast(v, U32)
                o = jnp.dot(p_scr[h], v, preferred_element_type=F32)
                acc_scr[...] += out_proj(o * l_scr[h], h)
                return c

            def vside1t(h, c):
                vside1(h, c)
                for hf in range(2):
                    vtf[h, :, hf * NVP * Dh:(hf + 1) * NVP * Dh] = (
                        v1buf[h, hf * SW + VP0:(hf + 1) * SW, :].astype(F32).T)
                return c

            x = jnp.broadcast_to(xbuf[1:2, :].astype(F32), (8, D))
            compute_q(x)
            for i, g in enumerate(GK1):
                cps_k1[i].wait()
                lax.fori_loop(g[0], g[1], kside1, 0)
            c0 = jnp.mean(x, axis=-1, keepdims=True)
            c_scr[...] = jnp.broadcast_to(c0, (8, Dh))
            acc_scr[...] = jnp.where(rowg == 0, x - c0, 0.0)
            for i, g in enumerate(GV1):
                cps_v1[i].wait()
                assert (g[0] in vpu_p) == (g[1] - 1 in vpu_p)
                lax.fori_loop(g[0], g[1], vside1t if g[0] in vpu_p else vside1, 0)
            o_scr[...] = jnp.zeros_like(o_scr)
            for i in range(NL - 1):
                cps_l[i].wait()
                o_scr[...] += pv_last(i)
            cps_l[NL - 1].wait()
            o = o_scr[...] + pv_last(NL - 1)


            zero_i = z_scr[...]

            def mk_tok(v):
                return lax.bitcast_convert_type(lax.bitcast_convert_type(v, jnp.int32) & zero_i, F32)

            def sum_all(vs):
                t = vs[0]
                for v in vs[1:]:
                    t = t + v
                return t

            def blocks(a):
                return [a[:, c * Dh:(c + 1) * Dh] for c in range(a.shape[1] // Dh)]

            def halves(a):
                return [a[0:8, :], a[8:16, :]]

            def stats(x):
                s1 = sum_all(blocks(x))
                s2 = sum_all(blocks(x * x))
                m = jnp.sum(s1, axis=-1, keepdims=True) * (1.0 / D)
                m2 = jnp.sum(s2, axis=-1, keepdims=True) * (1.0 / D)
                v = jnp.maximum(m2 - m * m, 0.0)
                return m, lax.rsqrt(v + eps), mk_tok(s1 + s2)

            def silu_half(a):
                return a + a * jnp.tanh(a)

            tile_cache = {}

            def tile_rows(tok, n):
                if (id(tok), n) not in tile_cache:
                    tile_cache[(id(tok), n)] = (tok, jnp.concatenate([tok] * n, axis=0))
                return tile_cache[(id(tok), n)][1]

            class MatVec:
                def __init__(self, xb_ref, slot, w_ref, row0, col0, nkb=NKB):
                    self.xb_ref, self.slot, self.w_ref, self.row0, self.col0 = xb_ref, slot, w_ref, row0, col0
                    self.acc = None
                    self.kb = 0
                    self.nkb = nkb

                def step(self, n, tok):
                    xv = self.xb_ref[self.slot, self.kb * 8:(self.kb + n) * 8, :]
                    if tok is not None:
                        xv = xv + tile_rows(tok, n)
                    self.fma(self.kb, xv)
                    self.kb += n

                def fma(self, kb, xv):
                    r0, n = self.row0 + kb * 8, xv.shape[0]
                    t = jnp.concatenate([xv] * rep, axis=1) * self.w_ref[r0:r0 + n, self.col0:self.col0 + G]
                    for i in range(0, n, 8):
                        ti = t[i:i + 8, :] if n > 8 else t
                        self.acc = ti if self.acc is None else self.acc + ti

            def ffn_fast(x):
                m, r, _ = stats(x)
                rh = 0.5 * r
                y = jnp.dot(x.astype(BF16), pltpu.bitcast(w1p[...], BF16), preferred_element_type=F32)
                h1 = silu_half((y - m * c1[...]) * rh)
                out = sum_all([
                    jnp.dot(h1[:, k0:k0 + Dh].astype(BF16),
                            pltpu.bitcast(w2p[(k0 - N2 * Dh) // 2:(k0 - N2 * Dh + Dh) // 2, :], BF16),
                            preferred_element_type=F32)
                    for k0 in range(N2 * Dh, FM, Dh)])
                ta = MatVec(None, 0, w2g, 0, 0)
                for kb in range(NF * 16):
                    yc = lanesum(sum_all(blocks(w1t[kb * 8:kb * 8 + 8, :] * x)))
                    ta.fma(kb, silu_half(yc * rh))
                for c in range(N2):
                    hb_scr[0, c * Dh:(c + 1) * Dh, :] = col_bcast(h1[0:1, c * Dh:(c + 1) * Dh])
                tb = MatVec(hb_scr, 0, w2f, 0, 0, nkb=N2 * 16)
                while tb.kb < tb.nkb:
                    tb.step(4, None)
                return m, out + rowsum(ta.acc + tb.acc)

            x = rowsum(acc_scr[...] + out_proj_fast(o * l_scr[HL], HL))
            m1, y1 = ffn_fast(x)
            x = (x - m1) + y1

            m, r, stok = stats(x)
            rs = r * (scale * LOG2E)

            def fin_q(qa, g):
                return pick_rows((qa - m * cq[:, g * G:(g + 1) * G]) * rs)
            x16 = x.astype(BF16)
            for c, xr in enumerate(blocks(x)):
                if c == D // Dh - 1:
                    xr = xr + stok
                xb_scr[0, c * Dh:(c + 1) * Dh, :] = col_bcast(xr[0:1, :])

            qs, os_, linv_, mx_ = {}, {}, {}, {}
            state = {"acc": jnp.where(rowg == 0, x - m, 0.0)}
            shift = c_scr[:, 0:1] + m1 + m
            live, fin = [None], []
            chunk_no = [0]
            k_at, os_at, e_at = {}, {}, {}
            todo = list(QUEUE)
            stack, etasks, due = [], [], []
            credit = [0.0]
            e_started, ep_ok = set(), set()
            last_tok = [None]

            def matvec_gen(mv):
                while mv.kb < NKB:
                    tok = yield 36
                    mv.step(4, tok)
                    live[0] = mv

            def q_gen(g):
                mv = MatVec(xb_scr, 0, wqf, 0, g * G - Q0)
                yield from matvec_gen(mv)
                qs[g] = fin_q(rowsum(mv.acc), g)
                return mk_tok(qs[g])

            def e_gen(g):
                m_ = jnp.broadcast_to(jnp.max(mx_[g], axis=1, keepdims=True), (8, Dh))
                m_ = jnp.maximum(m_, pltpu.roll(m_, 4, 0))
                lp = None
                order_ = list(range(NBLK))
                if g in vpu_p:
                    order_ = order_[NBLK - NVP:] + order_[:NBLK - NVP]
                for u in range(0, NBLK, EUNIT):
                    tok = yield ECOST * EUNIT
                    mm = m_ if tok is None else m_ + tok
                    for c in order_[u:u + EUNIT]:
                        pc = jnp.exp2(pf_scr[g, :, c * Dh:(c + 1) * Dh] - mm)
                        pf_scr[g, :, c * Dh:(c + 1) * Dh] = pc
                        lp = pc if lp is None else lp + pc
                    fin.append(lp)
                    if g in vpu_p and u + EUNIT >= NVP:
                        ep_ok.add(g)
                lp = lp + pltpu.roll(lp, 4, 0)
                linv_[g] = jnp.broadcast_to(1.0 / jnp.sum(lp, axis=1, keepdims=True), (8, Dh))
                e_at[g] = chunk_no[0]

            def p_gen(g):
                slot = g % 3
                for dg in range(Dh // 16):
                    accs = [None] * rep
                    for blk in range(NVP):
                        for hf in range(2):
                            tok = yield 20
                            col = (hf * NVP + blk) * Dh
                            vt = vtf[g, dg * 16:dg * 16 + 16, col:col + Dh]
                            if tok is not None:
                                vt = vt + tile_rows(tok, 2)
                            for j in range(rep):
                                r_ = hf * 4 + j
                                t = pf_scr[g, r_:r_ + 1, VP0 + blk * Dh:VP0 + (blk + 1) * Dh] * vt
                                accs[j] = t if accs[j] is None else accs[j] + t
                            live[0] = list(accs)
                    for j in range(rep):
                        pa_scr[slot, j * Dh + dg * 16:j * Dh + dg * 16 + 16, :] = accs[j]
                    fin.extend(halves(sum_all(accs)))
                    live[0] = None

            def o_gen(g):
                slot = g % 2
                linv = linv_[g]
                for j in range(rep):
                    tok = yield 48
                    orow = os_[g] if tok is None else os_[g] + tok
                    z = jnp.where(eye, jnp.broadcast_to(orow[j:j + 1, :], (Dh, Dh)), 0.0)
                    if g in vpu_p:
                        z = z + pa_scr[g % 3, j * Dh:(j + 1) * Dh, :]
                    ob_scr[slot, j * Dh:(j + 1) * Dh, :] = lanesum(z) * jnp.broadcast_to(linv[j:j + 1, :], (Dh, Dh))
                mv = MatVec(ob_scr, slot, wof, g * G, 0)
                yield from matvec_gen(mv)
                state["acc"] = state["acc"] + mv.acc
                return mk_tok(sum_all(blocks(mv.acc)))

            def ready(t):
                k_, g_ = t[0], int(t[1])
                if k_ == "p":
                    return g_ in ep_ok
                if k_ == "o":
                    return g_ in os_ and chunk_no[0] >= os_at[g_] + OLAG
                return True

            def run_vpu(tok, budget, force_e=None, flush=False):
                live[0] = None
                for g_, a_ in k_at.items():
                    if g_ not in e_started and (chunk_no[0] >= a_ + ELAG or g_ == force_e):
                        e_started.add(g_)
                        gen = e_gen(g_)
                        etasks.append([gen, next(gen)])
                credit[0] = 1e12 if flush else min(credit[0] + budget, 2 * RATE)
                while etasks:
                    credit[0] -= etasks[0][1]
                    try:
                        etasks[0][1] = etasks[0][0].send(tok)
                    except StopIteration:
                        etasks.pop(0)
                    if not flush:
                        break
                while True:
                    if not stack:
                        if not todo or (not flush and not ready(todo[0])):
                            break
                        t = todo.pop(0)
                        gen = {"q": q_gen, "p": p_gen, "o": o_gen}[t[0]](int(t[1]))
                        stack.append([gen, next(gen)])
                    cur = stack[-1]
                    if credit[0] < cur[1]:
                        break
                    credit[0] -= cur[1]
                    try:
                        cur[1] = cur[0].send(tok)
                    except StopIteration as e:
                        if e.value is not None:
                            due.append((chunk_no[0] + LAG, e.value))
                        live[0] = None
                        stack.pop()
                cov = list(fin)
                if isinstance(live[0], MatVec):
                    cov += blocks(live[0].acc)
                elif live[0]:
                    cov += halves(sum_all(live[0]))
                del fin[:]
                if cov and not flush:
                    due.append((chunk_no[0] + LAG, mk_tok(sum_all(cov))))

            def take_due():
                toks = [t for c_, t in due if c_ <= chunk_no[0]]
                due[:] = [(c_, t) for c_, t in due if c_ > chunk_no[0]]
                return sum_all(toks) if toks else None

            def qk2(g):
                while g not in qs:
                    run_vpu(last_tok[0], RATE)
                qq = qs[g]
                mx = None
                n = CB * Dh
                for c0 in range(0, NBLK, CB):
                    dtok = take_due()
                    if c0 == 0 or dtok is not None:
                        if dtok is not None:
                            qq = qq + dtok
                        qa = qq.astype(BF16)
                        qb = pltpu.roll(qq, 4, 0).astype(BF16)
                    sc = (jnp.dot(qa, load_kt(g, c0 * Dh, n), preferred_element_type=F32)
                          + jnp.dot(qb, load_kt(g, SW + c0 * Dh, n), preferred_element_type=F32))
                    pf_scr[g, :, c0 * Dh:c0 * Dh + n] = sc
                    for v in blocks(sc):
                        mx = v if mx is None else jnp.maximum(mx, v)
                    chunk_no[0] += 1
                    last_tok[0] = mk_tok(sc[:, 0:Dh])
                    run_vpu(last_tok[0], RATE)
                mx_[g] = mx

            def pv2(g):
                while g not in e_at:
                    run_vpu(last_tok[0], RATE, force_e=g)
                nb = NBLK - (NVP if g in vpu_p else 0)
                o1 = None
                o2 = None
                n = CB * Dh
                for c0 in range(0, nb, CB):
                    pc = pf_scr[g, :, c0 * Dh:c0 * Dh + n]
                    dtok = take_due()
                    if dtok is not None:
                        pc = jnp.concatenate([pc[:, 0:Dh] + dtok, pc[:, Dh:]], axis=1)
                    pc = pc.astype(BF16)
                    oc = jnp.dot(pc, load_v(g, c0 * Dh, n), preferred_element_type=F32)
                    o1 = oc if o1 is None else o1 + oc
                    oc2 = jnp.dot(pc, load_v(g, SW + c0 * Dh, n), preferred_element_type=F32)
                    o2 = oc2 if o2 is None else o2 + oc2
                    chunk_no[0] += 1
                    last_tok[0] = mk_tok(oc)
                    run_vpu(last_tok[0], RATE)
                return o1 + pltpu.roll(o2, 4, 0)

            for g in mxu_q:
                qs[g] = fin_q(jnp.dot(x16, pltpu.bitcast(wqp[mxu_q.index(g)], BF16), preferred_element_type=F32), g)
            for _ in range(PRE):
                run_vpu(None, RATE)
            pending_o = []
            for ph in ORDER:
                kind, g = ph[0], int(ph[1])
                if kind == "K":
                    qk2(g)
                    k_at[g] = chunk_no[0]
                else:
                    os_[g] = pv2(g)
                    os_at[g] = chunk_no[0]
                for og in pending_o:
                    state["acc"] = state["acc"] + out_proj_fast(os_[og] * linv_[og], og)
                pending_o = [g] if (kind == "V" and g in mxu_o) else []
            run_vpu(last_tok[0], 0, flush=True)
            for og in pending_o:
                state["acc"] = state["acc"] + out_proj_fast(os_[og] * linv_[og], og)
            x = rowsum(state["acc"])
            x = (x + shift) + ffn_fast(x)[1]
            o_ref[1:2, :] = x[0:1, :].astype(o_ref.dtype)

        pl.run_scoped(
            part_b,
            pltpu.VMEM((Hkv, Dh // 2, S), U32),
            pltpu.VMEM((Hkv, S // 2, Dh), U32),
            pltpu.VMEM((len(vpu_p), Dh, 2 * NVP * Dh), F32),
        )

    def kernel(*refs):
        pl.run_scoped(lambda sems: body(*refs, sems), pltpu.SemaphoreType.DMA((NSEM,)))

    assert NBLK % CB == 0 and (NBLK - NVP) % CB == 0 and CB >= 2
    out = pl.pallas_call(
        kernel,
        out_shape=jax.ShapeDtypeStruct((B, D), A_x.dtype),
        in_specs=[pl.BlockSpec(memory_space=pl.ANY)] * 7,
        out_specs=pl.BlockSpec(memory_space=pltpu.VMEM),
        scratch_shapes=[
            pltpu.VMEM((B, D), BF16),
            pltpu.VMEM((Hkv, S, Dh), BF16),
            pltpu.VMEM((Hkv, S, Dh), BF16),
            pltpu.VMEM((D, Hq * Dh), BF16),
            pltpu.VMEM((Hq * Dh, D), BF16),
            pltpu.VMEM((D, Fdim), BF16),
            pltpu.VMEM((Fdim, D), BF16),
            pltpu.VMEM((D, Hq * Dh - Q0), F32),
            pltpu.VMEM((len(vpu_o) * G, D), F32),
            pltpu.VMEM((N2 * Dh, D), F32),
            pltpu.VMEM((NF * Dh, D), F32),
            pltpu.VMEM((NF * Dh, D), F32),
            pltpu.VMEM((len(mxu_q), D // 2, G), U32),
            pltpu.VMEM((len(mxu_o), G // 2, D), U32),
            pltpu.VMEM((D // 2, FM), U32),
            pltpu.VMEM(((FM - N2 * Dh) // 2, D), U32),
            pltpu.VMEM((8, Hq * Dh), F32),
            pltpu.VMEM((8, FM), F32),
            pltpu.VMEM((Hkv, 8, Dh), BF16),
            pltpu.VMEM((8, D), F32),
            pltpu.VMEM((Hkv, 8, S), BF16),
            pltpu.VMEM((Hkv, 8, Dh), F32),
            pltpu.VMEM((8, Dh), F32),
            pltpu.VMEM((8, Dh), F32),
            pltpu.VMEM((1, D, Dh), F32),
            pltpu.VMEM((1, N2 * Dh, Dh), F32),
            pltpu.VMEM((2, G, Dh), F32),
            pltpu.VMEM((Hkv, 8, SW), F32),
            pltpu.VMEM((3, G, Dh), F32),
            pltpu.VMEM((8, Dh), jnp.int32),
        ],
        compiler_params=pltpu.CompilerParams(vmem_limit_bytes=120 * 1024 * 1024),
    )(A_x.reshape(B, D), A_k_cache, A_v_cache, A_wq, A_wo, B_w1, B_w2)
    return out.reshape(B, Sq, D)
```

```python
import jax
import jax.numpy as jnp
from jax import lax
import jax.experimental.pallas as pl
import jax.experimental.pallas.tpu as pltpu

F32 = jnp.float32
BF16 = jnp.bfloat16
U32 = jnp.uint32
NT = (((1,), (1,)), ((), ()))
LOG2E = 1.4426950408889634

G0 = ((0, 4), (4, 6), (6, 7), (7, 8))
GK1 = ((0, 4), (4, 8))
GV1 = ((0, 4), (4, 6), (6, 7))
LAST_CHUNKS = (6144, 1536, 512)
TCHUNK = 2048

ORDER = "K0 K1 K2 K3 V0 K4 V1 K5 V2 K6 V3 K7 V4 V5 V6 V7".split()
QUEUE = "q2 q3 q4 q5 q6 q7 p0 p1 p2 o0 p3 o1 p4 o2 p5 o3 o4 o5".split()
NVP = 8
CB = 2
RATE = 102.3
LAG = 8
ELAG = 7
EUNIT = 4
ECOST = 5
OLAG = 6
PRE = 8
N2 = 2
NF = 6


@jax.jit
def pallas_interleave_layers__gqa_block_cached__dense_activation_silu__decode_kernel(
    A_x: jax.Array,
    A_k_cache: jax.Array,
    A_v_cache: jax.Array,
    A_wq: jax.Array,
    A_wo: jax.Array,
    B_x: jax.Array,
    B_w1: jax.Array,
    B_w2: jax.Array,
):
    B, Sq, D = A_x.shape
    _, Hkv, S, Dh = A_k_cache.shape
    Hq = A_wq.shape[1] // Dh
    rep = Hq // Hkv
    Fdim = B_w1.shape[1]
    assert (B, Sq, rep, Dh, Hkv) == (2, 1, 4, 128, 8) and D == rep * Dh and sum(LAST_CHUNKS) == S
    G = rep * Dh
    scale = Dh ** -0.5
    eps = 1e-5
    SEM_W = 0
    SEM_0 = 5
    SEM_K1 = SEM_0 + 2 * len(G0)
    SEM_V1 = SEM_K1 + len(GK1)
    SEM_L = SEM_V1 + len(GV1)
    NL = len(LAST_CHUNKS)
    NSEM = SEM_L + NL
    lc_off = [sum(LAST_CHUNKS[:i]) for i in range(NL)]
    HL = Hkv - 1
    vpu_q = [g for g in range(Hkv) if "q%d" % g in QUEUE]
    vpu_o = [g for g in range(Hkv) if "o%d" % g in QUEUE]
    vpu_p = [g for g in range(Hkv) if "p%d" % g in QUEUE]
    mxu_q = [g for g in range(Hkv) if g not in vpu_q]
    mxu_o = [g for g in range(Hkv) if g not in vpu_o]
    assert vpu_q == list(range(vpu_q[0], Hkv)) and vpu_o == list(range(len(vpu_o)))
    assert vpu_p == list(range(len(vpu_p))) and set(vpu_p) <= set(vpu_o) and HL in mxu_o
    Q0 = vpu_q[0] * G
    SW = S // 2
    NBLK = SW // Dh
    VP0 = SW - NVP * Dh
    NKB = D // 8
    FM = Fdim - NF * Dh

    def body(x_hbm, k_hbm, v_hbm, wq_hbm, wo_hbm, w1_hbm, w2_hbm, o_ref,
             xbuf, k1buf, v1buf, wq, wo, w1, w2, wqf, wof, w2f, w1t, w2g,
             wqp, wop, w1p, w2p, cq, c1, q_scr, acc_scr, p_scr, l_scr, o_scr, c_scr,
             xb_scr, hb_scr, ob_scr, pf_scr, pa_scr, z_scr, sems):
        def cp_kv(hbm, buf, b, grp, sem):
            sl = pl.ds(grp[0], grp[1] - grp[0])
            return pltpu.make_async_copy(hbm.at[b, sl], buf.at[sl], sems.at[sem])

        def cp_vl(i):
            sl = pl.ds(lc_off[i], LAST_CHUNKS[i])
            return pltpu.make_async_copy(v_hbm.at[1, HL, sl], v1buf.at[HL, sl], sems.at[SEM_L + i])

        cps_w = [pltpu.make_async_copy(s_, d_, sems.at[SEM_W + i]) for i, (s_, d_) in enumerate(
            ((x_hbm, xbuf), (wq_hbm, wq), (wo_hbm, wo), (w1_hbm, w1), (w2_hbm, w2)))]
        cps_k1 = [cp_kv(k_hbm, k1buf, 1, g, SEM_K1 + i) for i, g in enumerate(GK1)]
        cps_v1 = [cp_kv(v_hbm, v1buf, 1, g, SEM_V1 + i) for i, g in enumerate(GV1)]
        cps_l = [cp_vl(i) for i in range(NL)]
        for c in cps_w:
            c.start()

        row8 = lax.broadcasted_iota(jnp.int32, (8, Dh), 0)
        rowg = lax.broadcasted_iota(jnp.int32, (8, G), 0)
        colg = lax.broadcasted_iota(jnp.int32, (8, G), 1)
        diag_mask = rowg == (colg // Dh)
        eye = (lax.broadcasted_iota(jnp.int32, (Dh, Dh), 0) == lax.broadcasted_iota(jnp.int32, (Dh, Dh), 1))

        def pick_rows(qa):
            qg = jnp.zeros((8, Dh), F32)
            for j in range(rep):
                qg = jnp.where(row8 == j, qa[:, j * Dh:(j + 1) * Dh], qg)
            return qg

        def diag_lhs(o):
            o4 = jnp.concatenate([o] * rep, axis=1)
            return jnp.where(diag_mask, o4, 0.0).astype(BF16)

        def out_proj_fast(o, g):
            return jnp.dot(diag_lhs(o), pltpu.bitcast(wop[mxu_o.index(g)], BF16), preferred_element_type=F32)

        def rowsum(a):
            return jnp.broadcast_to(jnp.sum(a, axis=0, keepdims=True), a.shape)

        def lanesum(a):
            return jnp.broadcast_to(jnp.sum(a, axis=1, keepdims=True), (a.shape[0], Dh))

        def col_bcast(row):
            return lanesum(jnp.where(eye, jnp.broadcast_to(row, (Dh, Dh)), 0.0))

        def layernorm(x):
            xc = x - jnp.mean(x, axis=-1, keepdims=True)
            return xc * lax.rsqrt(jnp.mean(xc * xc, axis=-1, keepdims=True) + eps)

        def compute_q(x):
            xn = layernorm(x).astype(BF16)
            for g in range(Hkv):
                qa = jnp.dot(xn, wq[:, g * G:(g + 1) * G], preferred_element_type=F32) * scale
                q_scr[g] = pick_rows(qa).astype(BF16)

        def softmax_parts(s):
            p = jnp.exp(s - jnp.max(s, axis=1, keepdims=True))
            return p.astype(BF16), jnp.sum(p, axis=1, keepdims=True)

        def out_proj(o, h):
            w = wo[pl.ds(pl.multiple_of(h * G, G), G), :]
            return jnp.dot(diag_lhs(o), w, preferred_element_type=F32)

        def ffn(x):
            hh = jnp.dot(layernorm(x).astype(BF16), w1[...], preferred_element_type=F32)
            hh = hh * jax.nn.sigmoid(hh)
            return jnp.dot(hh.astype(BF16), w2[...], preferred_element_type=F32)

        def part_a(k0buf, v0buf):
            cps_0 = [(cp_kv(k_hbm, k0buf, 0, g, SEM_0 + 2 * i), cp_kv(v_hbm, v0buf, 0, g, SEM_0 + 2 * i + 1))
                     for i, g in enumerate(G0)]
            for a, b_ in cps_0:
                a.start()
                b_.start()
            for c in cps_k1 + cps_v1 + cps_l:
                c.start()

            def attn_head0(h, c):
                s = lax.dot_general(q_scr[h], k0buf[h], NT, preferred_element_type=F32)
                p, l = softmax_parts(s)
                o = jnp.dot(p, v0buf[h], preferred_element_type=F32)
                acc_scr[...] += out_proj(o / l, h)
                return c

            for c in cps_w:
                c.wait()

            def prep_q(i, c):
                off = pl.multiple_of(i * 64, 64)
                wqf[pl.ds(off, 64), :] = wq[pl.ds(off, 64), Q0:].astype(F32)
                return c
            lax.fori_loop(0, D // 64, prep_q, 0)

            def prep_o(i, c):
                off = pl.multiple_of(i * G, G)
                wof[pl.ds(off, G), :] = wo[pl.ds(off, G), :].astype(F32)
                return c
            lax.fori_loop(0, len(vpu_o), prep_o, 0)
            for i, g in enumerate(mxu_q):
                wqp[i] = pltpu.bitcast(wq[:, g * G:(g + 1) * G], U32)
            for i, g in enumerate(mxu_o):
                wop[i] = pltpu.bitcast(wo[g * G:(g + 1) * G, :], U32)
            w1p[...] = pltpu.bitcast(w1[:, 0:FM], U32)
            w2p[...] = pltpu.bitcast(w2[N2 * Dh:FM, :], U32)
            for i in range(N2):
                w2f[i * Dh:(i + 1) * Dh, :] = w2[i * Dh:(i + 1) * Dh, :].astype(F32)
            w1t[...] = w1[:, FM:].astype(F32).T
            w2g[...] = w2[FM:, :].astype(F32)
            w1t[...] = w1t[...] - jnp.mean(w1t[...], axis=1, keepdims=True)
            ones8 = jnp.ones((8, D), BF16)
            cq[...] = jnp.dot(ones8, wq[...], preferred_element_type=F32)
            c1[...] = jnp.dot(ones8, w1[:, 0:FM], preferred_element_type=F32)
            z_scr[...] = jnp.zeros_like(z_scr)

            x = jnp.broadcast_to(xbuf[0:1, :].astype(F32), (8, D))
            compute_q(x)
            acc_scr[...] = jnp.zeros_like(acc_scr)
            for i, g in enumerate(G0):
                cps_0[i][0].wait()
                cps_0[i][1].wait()
                lax.fori_loop(g[0], g[1], attn_head0, 0)
            x = x + rowsum(acc_scr[...])
            x = x + ffn(x)
            compute_q(x)
            acc_scr[...] = jnp.zeros_like(acc_scr)
            lax.fori_loop(0, Hkv, attn_head0, 0)
            x = x + rowsum(acc_scr[...])
            x = x + ffn(x)
            o_ref[0:1, :] = x[0:1, :].astype(o_ref.dtype)

        pl.run_scoped(part_a, pltpu.VMEM((Hkv, S, Dh), BF16), pltpu.VMEM((Hkv, S, Dh), BF16))

        def part_b(ktbuf, vpk, vtf):
            def load_v(h, off, n):
                return pltpu.bitcast(vpk[h, off // 2:(off + n) // 2, :], BF16)

            def load_kt(h, off, n):
                return pltpu.bitcast(ktbuf[h, :, off:off + n], BF16)

            def pv_last(i):
                o_, n = lc_off[i], LAST_CHUNKS[i]
                v = v1buf[HL, o_:o_ + n, :]
                vpk[HL, o_ // 2:(o_ + n) // 2, :] = pltpu.bitcast(v, U32)
                return jnp.dot(p_scr[HL, :, o_:o_ + n], v, preferred_element_type=F32)

            def kside1(h, c):
                s = lax.dot_general(q_scr[h], k1buf[h], NT, preferred_element_type=F32)
                p, l = softmax_parts(s)
                p_scr[h] = p
                l_scr[h] = jnp.broadcast_to(1.0 / l, (8, Dh))

                def tr(i, carry):
                    off = pl.multiple_of(i * TCHUNK, TCHUNK)
                    ktbuf[h, :, pl.ds(off, TCHUNK)] = pltpu.bitcast(k1buf[h, pl.ds(off, TCHUNK), :].T, U32)
                    return carry
                lax.fori_loop(0, S // TCHUNK, tr, 0)
                return c

            def vside1(h, c):
                v = v1buf[h]
                vpk[h] = pltpu.bitcast(v, U32)
                o = jnp.dot(p_scr[h], v, preferred_element_type=F32)
                acc_scr[...] += out_proj(o * l_scr[h], h)
                return c

            def vside1t(h, c):
                vside1(h, c)
                for hf in range(2):
                    vtf[h, :, hf * NVP * Dh:(hf + 1) * NVP * Dh] = (
                        v1buf[h, hf * SW + VP0:(hf + 1) * SW, :].astype(F32).T)
                return c

            x = jnp.broadcast_to(xbuf[1:2, :].astype(F32), (8, D))
            compute_q(x)
            for i, g in enumerate(GK1):
                cps_k1[i].wait()
                lax.fori_loop(g[0], g[1], kside1, 0)
            c0 = jnp.mean(x, axis=-1, keepdims=True)
            c_scr[...] = jnp.broadcast_to(c0, (8, Dh))
            acc_scr[...] = jnp.where(rowg == 0, x - c0, 0.0)
            for i, g in enumerate(GV1):
                cps_v1[i].wait()
                assert (g[0] in vpu_p) == (g[1] - 1 in vpu_p)
                lax.fori_loop(g[0], g[1], vside1t if g[0] in vpu_p else vside1, 0)
            o_scr[...] = jnp.zeros_like(o_scr)
            for i in range(NL - 1):
                cps_l[i].wait()
                o_scr[...] += pv_last(i)
            cps_l[NL - 1].wait()
            o = o_scr[...] + pv_last(NL - 1)

            zero_i = z_scr[...]

            def mk_tok(v):
                return lax.bitcast_convert_type(lax.bitcast_convert_type(v, jnp.int32) & zero_i, F32)

            def sum_all(vs):
                t = vs[0]
                for v in vs[1:]:
                    t = t + v
                return t

            def blocks(a):
                return [a[:, c * Dh:(c + 1) * Dh] for c in range(a.shape[1] // Dh)]

            def halves(a):
                return [a[0:8, :], a[8:16, :]]

            def stats(x):
                s1 = sum_all(blocks(x))
                s2 = sum_all(blocks(x * x))
                m = jnp.sum(s1, axis=-1, keepdims=True) * (1.0 / D)
                m2 = jnp.sum(s2, axis=-1, keepdims=True) * (1.0 / D)
                v = jnp.maximum(m2 - m * m, 0.0)
                return m, lax.rsqrt(v + eps), mk_tok(s1 + s2)

            def silu_half(a):
                return a + a * jnp.tanh(a)

            tile_cache = {}

            def tile_rows(tok, n):
                if (id(tok), n) not in tile_cache:
                    tile_cache[(id(tok), n)] = (tok, jnp.concatenate([tok] * n, axis=0))
                return tile_cache[(id(tok), n)][1]

            class MatVec:
                def __init__(self, xb_ref, slot, w_ref, row0, col0, nkb=NKB):
                    self.xb_ref, self.slot, self.w_ref, self.row0, self.col0 = xb_ref, slot, w_ref, row0, col0
                    self.acc = None
                    self.kb = 0
                    self.nkb = nkb

                def step(self, n, tok):
                    xv = self.xb_ref[self.slot, self.kb * 8:(self.kb + n) * 8, :]
                    if tok is not None:
                        xv = xv + tile_rows(tok, n)
                    self.fma(self.kb, xv)
                    self.kb += n

                def fma(self, kb, xv):
                    r0, n = self.row0 + kb * 8, xv.shape[0]
                    t = jnp.concatenate([xv] * rep, axis=1) * self.w_ref[r0:r0 + n, self.col0:self.col0 + G]
                    for i in range(0, n, 8):
                        ti = t[i:i + 8, :] if n > 8 else t
                        self.acc = ti if self.acc is None else self.acc + ti

            def ffn_fast(x):
                m, r, _ = stats(x)
                rh = 0.5 * r
                y = jnp.dot(x.astype(BF16), pltpu.bitcast(w1p[...], BF16), preferred_element_type=F32)
                h1 = silu_half((y - m * c1[...]) * rh)
                out = sum_all([
                    jnp.dot(h1[:, k0:k0 + Dh].astype(BF16),
                            pltpu.bitcast(w2p[(k0 - N2 * Dh) // 2:(k0 - N2 * Dh + Dh) // 2, :], BF16),
                            preferred_element_type=F32)
                    for k0 in range(N2 * Dh, FM, Dh)])
                ta = MatVec(None, 0, w2g, 0, 0)
                for kb in range(NF * 16):
                    yc = lanesum(sum_all(blocks(w1t[kb * 8:kb * 8 + 8, :] * x)))
                    ta.fma(kb, silu_half(yc * rh))
                for c in range(N2):
                    hb_scr[0, c * Dh:(c + 1) * Dh, :] = col_bcast(h1[0:1, c * Dh:(c + 1) * Dh])
                tb = MatVec(hb_scr, 0, w2f, 0, 0, nkb=N2 * 16)
                while tb.kb < tb.nkb:
                    tb.step(4, None)
                return m, out + rowsum(ta.acc + tb.acc)

            x = rowsum(acc_scr[...] + out_proj_fast(o * l_scr[HL], HL))
            m1, y1 = ffn_fast(x)
            x = (x - m1) + y1

            m, r, stok = stats(x)
            rs = r * (scale * LOG2E)

            def fin_q(qa, g):
                return pick_rows((qa - m * cq[:, g * G:(g + 1) * G]) * rs)
            x16 = x.astype(BF16)
            for c, xr in enumerate(blocks(x)):
                if c == D // Dh - 1:
                    xr = xr + stok
                xb_scr[0, c * Dh:(c + 1) * Dh, :] = col_bcast(xr[0:1, :])

            qs, os_, linv_, mx_ = {}, {}, {}, {}
            state = {"acc": jnp.where(rowg == 0, x - m, 0.0)}
            shift = c_scr[:, 0:1] + m1 + m
            live, fin = [None], []
            chunk_no = [0]
            k_at, os_at, e_at = {}, {}, {}
            todo = list(QUEUE)
            stack, etasks, due = [], [], []
            credit = [0.0]
            e_started, ep_ok = set(), set()
            last_tok = [None]

            def matvec_gen(mv):
                while mv.kb < NKB:
                    tok = yield 36
                    mv.step(4, tok)
                    live[0] = mv

            def q_gen(g):
                mv = MatVec(xb_scr, 0, wqf, 0, g * G - Q0)
                yield from matvec_gen(mv)
                qs[g] = fin_q(rowsum(mv.acc), g)
                return mk_tok(qs[g])

            def e_gen(g):
                m_ = jnp.broadcast_to(jnp.max(mx_[g], axis=1, keepdims=True), (8, Dh))
                m_ = jnp.maximum(m_, pltpu.roll(m_, 4, 0))
                lp = None
                order_ = list(range(NBLK))
                if g in vpu_p:
                    order_ = order_[NBLK - NVP:] + order_[:NBLK - NVP]
                for u in range(0, NBLK, EUNIT):
                    tok = yield ECOST * EUNIT
                    mm = m_ if tok is None else m_ + tok
                    for c in order_[u:u + EUNIT]:
                        pc = jnp.exp2(pf_scr[g, :, c * Dh:(c + 1) * Dh] - mm)
                        pf_scr[g, :, c * Dh:(c + 1) * Dh] = pc
                        lp = pc if lp is None else lp + pc
                    fin.append(lp)
                    if g in vpu_p and u + EUNIT >= NVP:
                        ep_ok.add(g)
                lp = lp + pltpu.roll(lp, 4, 0)
                linv_[g] = jnp.broadcast_to(1.0 / jnp.sum(lp, axis=1, keepdims=True), (8, Dh))
                e_at[g] = chunk_no[0]

            def p_gen(g):
                slot = g % 3
                for dg in range(Dh // 16):
                    accs = [None] * rep
                    for blk in range(NVP):
                        for hf in range(2):
                            tok = yield 20
                            col = (hf * NVP + blk) * Dh
                            vt = vtf[g, dg * 16:dg * 16 + 16, col:col + Dh]
                            if tok is not None:
                                vt = vt + tile_rows(tok, 2)
                            for j in range(rep):
                                r_ = hf * 4 + j
                                t = pf_scr[g, r_:r_ + 1, VP0 + blk * Dh:VP0 + (blk + 1) * Dh] * vt
                                accs[j] = t if accs[j] is None else accs[j] + t
                            live[0] = list(accs)
                    for j in range(rep):
                        pa_scr[slot, j * Dh + dg * 16:j * Dh + dg * 16 + 16, :] = accs[j]
                    fin.extend(halves(sum_all(accs)))
                    live[0] = None

            def o_gen(g):
                slot = g % 2
                linv = linv_[g]
                for j in range(rep):
                    tok = yield 48
                    orow = os_[g] if tok is None else os_[g] + tok
                    z = jnp.where(eye, jnp.broadcast_to(orow[j:j + 1, :], (Dh, Dh)), 0.0)
                    if g in vpu_p:
                        z = z + pa_scr[g % 3, j * Dh:(j + 1) * Dh, :]
                    ob_scr[slot, j * Dh:(j + 1) * Dh, :] = lanesum(z) * jnp.broadcast_to(linv[j:j + 1, :], (Dh, Dh))
                mv = MatVec(ob_scr, slot, wof, g * G, 0)
                yield from matvec_gen(mv)
                state["acc"] = state["acc"] + mv.acc
                return mk_tok(sum_all(blocks(mv.acc)))

            def ready(t):
                k_, g_ = t[0], int(t[1])
                if k_ == "p":
                    return g_ in ep_ok
                if k_ == "o":
                    return g_ in os_ and chunk_no[0] >= os_at[g_] + OLAG
                return True

            def run_vpu(tok, budget, force_e=None, flush=False):
                live[0] = None
                for g_, a_ in k_at.items():
                    if g_ not in e_started and (chunk_no[0] >= a_ + ELAG or g_ == force_e):
                        e_started.add(g_)
                        gen = e_gen(g_)
                        etasks.append([gen, next(gen)])
                credit[0] = 1e12 if flush else min(credit[0] + budget, 2 * RATE)
                while etasks:
                    credit[0] -= etasks[0][1]
                    try:
                        etasks[0][1] = etasks[0][0].send(tok)
                    except StopIteration:
                        etasks.pop(0)
                    if not flush:
                        break
                while True:
                    if not stack:
                        if not todo or (not flush and not ready(todo[0])):
                            break
                        t = todo.pop(0)
                        gen = {"q": q_gen, "p": p_gen, "o": o_gen}[t[0]](int(t[1]))
                        stack.append([gen, next(gen)])
                    cur = stack[-1]
                    if credit[0] < cur[1]:
                        break
                    credit[0] -= cur[1]
                    try:
                        cur[1] = cur[0].send(tok)
                    except StopIteration as e:
                        if e.value is not None:
                            due.append((chunk_no[0] + LAG, e.value))
                        live[0] = None
                        stack.pop()
                cov = list(fin)
                if isinstance(live[0], MatVec):
                    cov += blocks(live[0].acc)
                elif live[0]:
                    cov += halves(sum_all(live[0]))
                del fin[:]
                if cov and not flush:
                    due.append((chunk_no[0] + LAG, mk_tok(sum_all(cov))))

            def take_due():
                toks = [t for c_, t in due if c_ <= chunk_no[0]]
                due[:] = [(c_, t) for c_, t in due if c_ > chunk_no[0]]
                return sum_all(toks) if toks else None

            def qk2(g):
                while g not in qs:
                    run_vpu(last_tok[0], RATE)
                qq = qs[g]
                mx = None
                n = CB * Dh
                for c0 in range(0, NBLK, CB):
                    dtok = take_due()
                    if c0 == 0 or dtok is not None:
                        if dtok is not None:
                            qq = qq + dtok
                        qa = qq.astype(BF16)
                        qb = pltpu.roll(qq, 4, 0).astype(BF16)
                    sc = (jnp.dot(qa, load_kt(g, c0 * Dh, n), preferred_element_type=F32)
                          + jnp.dot(qb, load_kt(g, SW + c0 * Dh, n), preferred_element_type=F32))
                    pf_scr[g, :, c0 * Dh:c0 * Dh + n] = sc
                    for v in blocks(sc):
                        mx = v if mx is None else jnp.maximum(mx, v)
                    chunk_no[0] += 1
                    last_tok[0] = mk_tok(sc[:, 0:Dh])
                    run_vpu(last_tok[0], RATE)
                mx_[g] = mx

            def pv2(g):
                while g not in e_at:
                    run_vpu(last_tok[0], RATE, force_e=g)
                nb = NBLK - (NVP if g in vpu_p else 0)
                o1 = None
                o2 = None
                n = CB * Dh
                for c0 in range(0, nb, CB):
                    pc = pf_scr[g, :, c0 * Dh:c0 * Dh + n]
                    dtok = take_due()
                    if dtok is not None:
                        pc = jnp.concatenate([pc[:, 0:Dh] + dtok, pc[:, Dh:]], axis=1)
                    pc = pc.astype(BF16)
                    oc = jnp.dot(pc, load_v(g, c0 * Dh, n), preferred_element_type=F32)
                    o1 = oc if o1 is None else o1 + oc
                    oc2 = jnp.dot(pc, load_v(g, SW + c0 * Dh, n), preferred_element_type=F32)
                    o2 = oc2 if o2 is None else o2 + oc2
                    chunk_no[0] += 1
                    last_tok[0] = mk_tok(oc)
                    run_vpu(last_tok[0], RATE)
                return o1 + pltpu.roll(o2, 4, 0)

            for g in mxu_q:
                qs[g] = fin_q(jnp.dot(x16, pltpu.bitcast(wqp[mxu_q.index(g)], BF16), preferred_element_type=F32), g)
            for _ in range(PRE):
                run_vpu(None, RATE)
            pending_o = []
            for ph in ORDER:
                kind, g = ph[0], int(ph[1])
                if kind == "K":
                    qk2(g)
                    k_at[g] = chunk_no[0]
                else:
                    os_[g] = pv2(g)
                    os_at[g] = chunk_no[0]
                for og in pending_o:
                    state["acc"] = state["acc"] + out_proj_fast(os_[og] * linv_[og], og)
                pending_o = [g] if (kind == "V" and g in mxu_o) else []
            run_vpu(last_tok[0], 0, flush=True)
            for og in pending_o:
                state["acc"] = state["acc"] + out_proj_fast(os_[og] * linv_[og], og)
            x = rowsum(state["acc"])
            x = (x + shift) + ffn_fast(x)[1]
            o_ref[1:2, :] = x[0:1, :].astype(o_ref.dtype)

        pl.run_scoped(
            part_b,
            pltpu.VMEM((Hkv, Dh // 2, S), U32),
            pltpu.VMEM((Hkv, S // 2, Dh), U32),
            pltpu.VMEM((len(vpu_p), Dh, 2 * NVP * Dh), F32),
        )

    def kernel(*refs):
        pl.run_scoped(lambda sems: body(*refs, sems), pltpu.SemaphoreType.DMA((NSEM,)))

    assert NBLK % CB == 0 and (NBLK - NVP) % CB == 0 and CB >= 2
    out = pl.pallas_call(
        kernel,
        out_shape=jax.ShapeDtypeStruct((B, D), A_x.dtype),
        in_specs=[pl.BlockSpec(memory_space=pl.ANY)] * 7,
        out_specs=pl.BlockSpec(memory_space=pltpu.VMEM),
        scratch_shapes=[
            pltpu.VMEM((B, D), BF16),
            pltpu.VMEM((Hkv, S, Dh), BF16),
            pltpu.VMEM((Hkv, S, Dh), BF16),
            pltpu.VMEM((D, Hq * Dh), BF16),
            pltpu.VMEM((Hq * Dh, D), BF16),
            pltpu.VMEM((D, Fdim), BF16),
            pltpu.VMEM((Fdim, D), BF16),
            pltpu.VMEM((D, Hq * Dh - Q0), F32),
            pltpu.VMEM((len(vpu_o) * G, D), F32),
            pltpu.VMEM((N2 * Dh, D), F32),
            pltpu.VMEM((NF * Dh, D), F32),
            pltpu.VMEM((NF * Dh, D), F32),
            pltpu.VMEM((len(mxu_q), D // 2, G), U32),
            pltpu.VMEM((len(mxu_o), G // 2, D), U32),
            pltpu.VMEM((D // 2, FM), U32),
            pltpu.VMEM(((FM - N2 * Dh) // 2, D), U32),
            pltpu.VMEM((8, Hq * Dh), F32),
            pltpu.VMEM((8, FM), F32),
            pltpu.VMEM((Hkv, 8, Dh), BF16),
            pltpu.VMEM((8, D), F32),
            pltpu.VMEM((Hkv, 8, S), BF16),
            pltpu.VMEM((Hkv, 8, Dh), F32),
            pltpu.VMEM((8, Dh), F32),
            pltpu.VMEM((8, Dh), F32),
            pltpu.VMEM((1, D, Dh), F32),
            pltpu.VMEM((1, N2 * Dh, Dh), F32),
            pltpu.VMEM((2, G, Dh), F32),
            pltpu.VMEM((Hkv, 8, SW), F32),
            pltpu.VMEM((3, G, Dh), F32),
            pltpu.VMEM((8, Dh), jnp.int32),
        ],
        compiler_params=pltpu.CompilerParams(vmem_limit_bytes=120 * 1024 * 1024),
    )(A_x.reshape(B, D), A_k_cache, A_v_cache, A_wq, A_wo, B_w1, B_w2)
    return out.reshape(B, Sq, D)
```

```python
import jax
import jax.numpy as jnp
from jax import lax
import jax.experimental.pallas as pl
import jax.experimental.pallas.tpu as pltpu

F32 = jnp.float32
BF16 = jnp.bfloat16
U32 = jnp.uint32
NT = (((1,), (1,)), ((), ()))
LOG2E = 1.4426950408889634

HROWS = 64
LAST_CHUNKS = (6144, 1536, 512)
TCHUNK = 2048
GAP = 38
I1 = 250
IDLE_A = (60, 60, 50)
EMB0 = 12
EMB2 = 16
EMBK = 4
CUT = 0

ORDER = "K0 K1 K2 K3 V0 K4 V1 K5 V2 K6 V3 K7 V4 V5 V6 V7".split()
QUEUE = "q2 q3 q4 q5 q6 q7 p0 p1 p2 o0 p3 o1 p4 o2 p5 o3 o4 o5".split()
NVP = 8
CB = 2
RATE = 102.3
LAG = 8
ELAG = 7
EUNIT = 4
ECOST = 5
OLAG = 6
PRE = 8
N2 = 2
NF = 6


@jax.jit
def pallas_interleave_layers__gqa_block_cached__dense_activation_silu__decode_kernel(
    A_x: jax.Array,
    A_k_cache: jax.Array,
    A_v_cache: jax.Array,
    A_wq: jax.Array,
    A_wo: jax.Array,
    B_x: jax.Array,
    B_w1: jax.Array,
    B_w2: jax.Array,
):
    B, Sq, D = A_x.shape
    _, Hkv, S, Dh = A_k_cache.shape
    Hq = A_wq.shape[1] // Dh
    rep = Hq // Hkv
    Fdim = B_w1.shape[1]
    assert (B, Sq, rep, Dh, Hkv) == (2, 1, 4, 128, 8) and D == rep * Dh and sum(LAST_CHUNKS) == S
    G = rep * Dh
    scale = Dh ** -0.5
    eps = 1e-5
    NPC = S // HROWS
    SEM_W = 0
    SEM_K0 = 5
    SEM_V0 = SEM_K0 + 4
    SEM_K1 = SEM_V0 + 4
    SEM_V1 = SEM_K1 + 4
    SEM_L = SEM_V1 + 4
    NL = len(LAST_CHUNKS)
    NSEM = SEM_L + NL
    lc_off = [sum(LAST_CHUNKS[:i]) for i in range(NL)]
    HL = Hkv - 1
    vpu_q = [g for g in range(Hkv) if "q%d" % g in QUEUE]
    vpu_o = [g for g in range(Hkv) if "o%d" % g in QUEUE]
    vpu_p = [g for g in range(Hkv) if "p%d" % g in QUEUE]
    mxu_q = [g for g in range(Hkv) if g not in vpu_q]
    mxu_o = [g for g in range(Hkv) if g not in vpu_o]
    assert vpu_q == list(range(vpu_q[0], Hkv)) and vpu_o == list(range(len(vpu_o)))
    assert vpu_p == list(range(len(vpu_p))) and set(vpu_p) <= set(vpu_o) and HL in mxu_o
    Q0 = vpu_q[0] * G
    SW = S // 2
    NBLK = SW // Dh
    VP0 = SW - NVP * Dh
    NKB = D // 8
    FM = Fdim - NF * Dh

    def body(x_hbm, k_hbm, v_hbm, wq_hbm, wo_hbm, w1_hbm, w2_hbm, o_ref,
             xbuf, kv1, wq, wo, w1, w2, wqf, wof, w2f, w1t, w2g,
             wqp, wop, w1p, w2p, cq, c1, s_scr, d_scr, acc_scr, p_scr, l_scr, o_scr, c_scr,
             xb_scr, hb_scr, ob_scr, pf_scr, pa_scr, z_scr, sems):
        hbm = (k_hbm, v_hbm)

        def cp_big(buf, t, b, h0, nh, sem):
            return pltpu.make_async_copy(hbm[t].at[b, pl.ds(h0, nh)], buf.at[t, pl.ds(h0, nh), pl.ds(0, S)],
                                         sems.at[sem])

        def hi_start(buf, t, b, pair0, sem0, p):
            pr = p // NPC
            hs = pl.ds(2 * (pair0 + pr), 2)
            rs_ = pl.ds(pl.multiple_of((p % NPC) * HROWS, HROWS), HROWS)
            pltpu.make_async_copy(hbm[t].at[b, hs, rs_], buf.at[t, hs, rs_], sems.at[sem0 + pr]).start(priority=0)

        def cp_vl(i):
            sl = pl.ds(lc_off[i], LAST_CHUNKS[i])
            return pltpu.make_async_copy(v_hbm.at[1, HL, sl], kv1.at[1, HL, sl], sems.at[SEM_L + i])

        cps_w = [pltpu.make_async_copy(s_, d_, sems.at[SEM_W + i]) for i, (s_, d_) in enumerate(
            ((x_hbm, xbuf), (wq_hbm, wq), (wo_hbm, wo), (w1_hbm, w1), (w2_hbm, w2)))]
        cps_k1 = [cp_big(kv1, 0, 1, 2 * i, 2, SEM_K1 + i) for i in range(4)]
        cps_v1 = [cp_big(kv1, 1, 1, 2 * i, 2 if i < 3 else 1, SEM_V1 + i) for i in range(4)]
        cps_l = [cp_vl(i) for i in range(NL)]
        for c in cps_w:
            c.start(priority=1)

        row8 = lax.broadcasted_iota(jnp.int32, (8, Dh), 0)
        rowg = lax.broadcasted_iota(jnp.int32, (8, G), 0)
        colg = lax.broadcasted_iota(jnp.int32, (8, G), 1)
        diag_mask = rowg == (colg // Dh)
        eye = (lax.broadcasted_iota(jnp.int32, (Dh, Dh), 0) == lax.broadcasted_iota(jnp.int32, (Dh, Dh), 1))

        def pick_rows(qa):
            qg = jnp.zeros((8, Dh), F32)
            for j in range(rep):
                qg = jnp.where(row8 == j, qa[:, j * Dh:(j + 1) * Dh], qg)
            return qg

        def diag_lhs(o):
            o4 = jnp.concatenate([o] * rep, axis=1)
            return jnp.where(diag_mask, o4, 0.0).astype(BF16)

        def out_proj_fast(o, g):
            return jnp.dot(diag_lhs(o), pltpu.bitcast(wop[mxu_o.index(g)], BF16), preferred_element_type=F32)

        def rowsum(a):
            return jnp.broadcast_to(jnp.sum(a, axis=0, keepdims=True), a.shape)

        def lanesum(a):
            return jnp.broadcast_to(jnp.sum(a, axis=1, keepdims=True), (a.shape[0], Dh))

        def col_bcast(row):
            return lanesum(jnp.where(eye, jnp.broadcast_to(row, (Dh, Dh)), 0.0))

        def layernorm(x):
            xc = x - jnp.mean(x, axis=-1, keepdims=True)
            return xc * lax.rsqrt(jnp.mean(xc * xc, axis=-1, keepdims=True) + eps)

        def compute_q(x):
            xn = layernorm(x).astype(BF16)
            for g in range(Hkv):
                qa = jnp.dot(xn, wq[:, g * G:(g + 1) * G], preferred_element_type=F32) * scale
                kv1[0, g, S:S + 8, :] = pick_rows(qa).astype(BF16)

        def softmax_parts(s):
            p = jnp.exp(s - jnp.max(s, axis=1, keepdims=True))
            return p.astype(BF16), jnp.sum(p, axis=1, keepdims=True)

        def out_proj(o, h):
            w = wo[pl.ds(pl.multiple_of(h * G, G), G), :]
            return jnp.dot(diag_lhs(o), w, preferred_element_type=F32)

        def ffn(x):
            hh = jnp.dot(layernorm(x).astype(BF16), w1[...], preferred_element_type=F32)
            hh = hh * jax.nn.sigmoid(hh)
            return jnp.dot(hh.astype(BF16), w2[...], preferred_element_type=F32)

        def part_a(kv0):
            cps_k0 = [cp_big(kv0, 0, 0, 2 * i, 2, SEM_K0 + i) for i in range(4)]
            cps_v0 = [cp_big(kv0, 1, 0, 2 * i, 2, SEM_V0 + i) for i in range(4)]
            for c in cps_k0 + cps_k1[0:3] + [cps_v1[0], cps_v1[2], cps_v1[3]] + cps_l:
                c.start(priority=1)
            issued = [0]

            def idle_v0(n):
                p0 = issued[0]
                n = max(min(n, 4 * NPC - p0), 0)

                def it(i, y):
                    hi_start(kv0, 1, 0, 0, SEM_V0, p0 + i)
                    for _ in range(GAP):
                        y = y * 0.5 + 1.0
                    return y
                if n > 0:
                    d_scr[...] = lax.fori_loop(0, n, it, d_scr[...])
                issued[0] += n

            def attn_head0(h, emb, start):
                nq = (2 * emb + 2) // 3 if emb else 1
                nv = emb - nq if emb else 1
                ss = []
                for c in range(nq):
                    r0, r1 = (c * (S // Dh) // nq) * Dh, ((c + 1) * (S // Dh) // nq) * Dh
                    ss.append(lax.dot_general(kv1[0, h, S:S + 8, :], kv0[0, h, r0:r1, :], NT,
                                              preferred_element_type=F32))
                    if emb:
                        start(c)
                p, l = softmax_parts(jnp.concatenate(ss, axis=1))
                o = None
                for c in range(nv):
                    r0, r1 = (c * (S // Dh) // nv) * Dh, ((c + 1) * (S // Dh) // nv) * Dh
                    pc = p[:, r0:r1]
                    if emb:
                        z = kv1[1, h, S:S + 8, :]
                        pc = jnp.concatenate([pc[:, 0:Dh] + z, pc[:, Dh:]], axis=1)
                    oc = jnp.dot(pc, kv0[1, h, r0:r1, :], preferred_element_type=F32)
                    o = oc if o is None else o + oc
                    if emb:
                        start(nq + c)
                acc_scr[...] += out_proj(o / l, h)

            d_scr[...] = jnp.zeros_like(d_scr)
            for h in range(Hkv):
                kv1[1, h, S:S + 16, :] = jnp.zeros((16, Dh), BF16)
            idle_v0(I1)
            for c in cps_w:
                c.wait()

            def prep_q(i, c):
                off = pl.multiple_of(i * 64, 64)
                wqf[pl.ds(off, 64), :] = wq[pl.ds(off, 64), Q0:].astype(F32)
                return c
            lax.fori_loop(0, D // 64, prep_q, 0)

            def prep_o(i, c):
                off = pl.multiple_of(i * G, G)
                wof[pl.ds(off, G), :] = wo[pl.ds(off, G), :].astype(F32)
                return c
            lax.fori_loop(0, len(vpu_o), prep_o, 0)
            for i, g in enumerate(mxu_q):
                wqp[i] = pltpu.bitcast(wq[:, g * G:(g + 1) * G], U32)
            for i, g in enumerate(mxu_o):
                wop[i] = pltpu.bitcast(wo[g * G:(g + 1) * G, :], U32)
            w1p[...] = pltpu.bitcast(w1[:, 0:FM], U32)
            w2p[...] = pltpu.bitcast(w2[N2 * Dh:FM, :], U32)
            for i in range(N2):
                w2f[i * Dh:(i + 1) * Dh, :] = w2[i * Dh:(i + 1) * Dh, :].astype(F32)
            w1t[...] = w1[:, FM:].astype(F32).T
            w2g[...] = w2[FM:, :].astype(F32)
            w1t[...] = w1t[...] - jnp.mean(w1t[...], axis=1, keepdims=True)
            ones8 = jnp.ones((8, D), BF16)
            cq[...] = jnp.dot(ones8, wq[...], preferred_element_type=F32)
            c1[...] = jnp.dot(ones8, w1[:, 0:FM], preferred_element_type=F32)
            z_scr[...] = jnp.zeros_like(z_scr)

            x = jnp.broadcast_to(xbuf[0:1, :].astype(F32), (8, D))
            compute_q(x)
            acc_scr[...] = jnp.zeros_like(acc_scr)
            for i in range(4):
                if i:
                    idle_v0(IDLE_A[i - 1])
                idle_v0((i + 1) * NPC - issued[0])
                cps_k0[i].wait()
                cps_v0[i].wait()
                p0 = issued[0]
                emb = EMB0 if p0 + 2 * EMB0 <= 4 * NPC else 0

                def body1(h, c, p0=p0, emb=emb, i=i):
                    attn_head0(h, emb, lambda j: hi_start(kv0, 1, 0, 0, SEM_V0, p0 + (h - 2 * i) * emb + j))
                    return c
                lax.fori_loop(2 * i, 2 * i + 2, body1, 0)
                issued[0] += 2 * emb
            x = x + rowsum(acc_scr[...])
            x = x + ffn(x)
            compute_q(x)
            acc_scr[...] = jnp.zeros_like(acc_scr)

            def body2(h, c):
                attn_head0(h, EMB2, lambda j: hi_start(kv1, 0, 1, 3, SEM_K1 + 3, h * EMB2 + j))
                return c
            lax.fori_loop(0, Hkv, body2, 0)
            x = x + rowsum(acc_scr[...])
            x = x + ffn(x)
            o_ref[0:1, :] = x[0:1, :].astype(o_ref.dtype)

        assert Hkv * EMB2 == NPC and Hkv * (S // TCHUNK) * EMBK == NPC
        pl.run_scoped(part_a, pltpu.VMEM((2, Hkv, S, Dh), BF16))

        def part_b(ktbuf, vpk, vtf):
            def load_v(h, off, n):
                return pltpu.bitcast(vpk[h, off // 2:(off + n) // 2, :], BF16)

            def load_kt(h, off, n):
                return pltpu.bitcast(ktbuf[h, :, off:off + n], BF16)

            def pv_last(i):
                o_, n = lc_off[i], LAST_CHUNKS[i]
                v = kv1[1, HL, o_:o_ + n, :]
                vpk[HL, o_ // 2:(o_ + n) // 2, :] = pltpu.bitcast(v, U32)
                return jnp.dot(p_scr[HL, :, o_:o_ + n], v, preferred_element_type=F32)

            def kside1(h, c):
                sub = TCHUNK // EMBK

                def tr(i, carry):
                    for u in range(EMBK):
                        off = pl.multiple_of(i * TCHUNK + u * sub, sub)
                        kt = kv1[0, h, pl.ds(off, sub), :].T
                        ktbuf[h, :, pl.ds(off, sub)] = pltpu.bitcast(kt, U32)
                        s_scr[:, pl.ds(off, sub)] = jnp.dot(kv1[0, h, S:S + 8, :], kt, preferred_element_type=F32)
                        hi_start(kv1, 1, 1, 1, SEM_V1 + 1, (h * (S // TCHUNK) + i) * EMBK + u)
                    return carry
                lax.fori_loop(0, S // TCHUNK, tr, 0)
                p, l = softmax_parts(s_scr[...])
                p_scr[h] = p
                l_scr[h] = jnp.broadcast_to(1.0 / l, (8, Dh))
                return c

            def vside1(h, c):
                v = kv1[1, h, 0:S, :]
                vpk[h] = pltpu.bitcast(v, U32)
                o = jnp.dot(p_scr[h], v, preferred_element_type=F32)
                acc_scr[...] += out_proj(o * l_scr[h], h)
                return c

            def vside1t(h, c):
                vside1(h, c)
                for hf in range(2):
                    vtf[h, :, hf * NVP * Dh:(hf + 1) * NVP * Dh] = (
                        kv1[1, h, hf * SW + VP0:(hf + 1) * SW, :].astype(F32).T)
                return c

            x = jnp.broadcast_to(xbuf[1:2, :].astype(F32), (8, D))
            compute_q(x)
            for i in range(4):
                cps_k1[i].wait()
                lax.fori_loop(2 * i, 2 * i + 2, kside1, 0)
            c0 = jnp.mean(x, axis=-1, keepdims=True)
            c_scr[...] = jnp.broadcast_to(c0, (8, Dh))
            acc_scr[...] = jnp.where(rowg == 0, x - c0, 0.0)
            assert vpu_p == list(range(6))
            for i in range(4):
                cps_v1[i].wait()
                lax.fori_loop(2 * i, min(2 * i + 2, HL), vside1t if i < 3 else vside1, 0)
            o_scr[...] = jnp.zeros_like(o_scr)
            for i in range(NL - 1):
                cps_l[i].wait()
                o_scr[...] += pv_last(i)
            cps_l[NL - 1].wait()
            o = o_scr[...] + pv_last(NL - 1)
            if CUT:
                o_ref[1:2, :] = jnp.concatenate([o] * 4, axis=1)[0:1, :].astype(o_ref.dtype)
                return

            zero_i = z_scr[...]

            def mk_tok(v):
                return lax.bitcast_convert_type(lax.bitcast_convert_type(v, jnp.int32) & zero_i, F32)

            def sum_all(vs):
                t = vs[0]
                for v in vs[1:]:
                    t = t + v
                return t

            def blocks(a):
                return [a[:, c * Dh:(c + 1) * Dh] for c in range(a.shape[1] // Dh)]

            def halves(a):
                return [a[0:8, :], a[8:16, :]]

            def stats(x):
                s1 = sum_all(blocks(x))
                s2 = sum_all(blocks(x * x))
                m = jnp.sum(s1, axis=-1, keepdims=True) * (1.0 / D)
                m2 = jnp.sum(s2, axis=-1, keepdims=True) * (1.0 / D)
                v = jnp.maximum(m2 - m * m, 0.0)
                return m, lax.rsqrt(v + eps), mk_tok(s1 + s2)

            def silu_half(a):
                return a + a * jnp.tanh(a)

            tile_cache = {}

            def tile_rows(tok, n):
                if (id(tok), n) not in tile_cache:
                    tile_cache[(id(tok), n)] = (tok, jnp.concatenate([tok] * n, axis=0))
                return tile_cache[(id(tok), n)][1]

            class MatVec:
                def __init__(self, xb_ref, slot, w_ref, row0, col0, nkb=NKB):
                    self.xb_ref, self.slot, self.w_ref, self.row0, self.col0 = xb_ref, slot, w_ref, row0, col0
                    self.acc = None
                    self.kb = 0
                    self.nkb = nkb

                def step(self, n, tok):
                    xv = self.xb_ref[self.slot, self.kb * 8:(self.kb + n) * 8, :]
                    if tok is not None:
                        xv = xv + tile_rows(tok, n)
                    self.fma(self.kb, xv)
                    self.kb += n

                def fma(self, kb, xv):
                    r0, n = self.row0 + kb * 8, xv.shape[0]
                    t = jnp.concatenate([xv] * rep, axis=1) * self.w_ref[r0:r0 + n, self.col0:self.col0 + G]
                    for i in range(0, n, 8):
                        ti = t[i:i + 8, :] if n > 8 else t
                        self.acc = ti if self.acc is None else self.acc + ti

            def ffn_fast(x):
                m, r, _ = stats(x)
                rh = 0.5 * r
                y = jnp.dot(x.astype(BF16), pltpu.bitcast(w1p[...], BF16), preferred_element_type=F32)
                h1 = silu_half((y - m * c1[...]) * rh)
                out = sum_all([
                    jnp.dot(h1[:, k0:k0 + Dh].astype(BF16),
                            pltpu.bitcast(w2p[(k0 - N2 * Dh) // 2:(k0 - N2 * Dh + Dh) // 2, :], BF16),
                            preferred_element_type=F32)
                    for k0 in range(N2 * Dh, FM, Dh)])
                ta = MatVec(None, 0, w2g, 0, 0)
                for kb in range(NF * 16):
                    yc = lanesum(sum_all(blocks(w1t[kb * 8:kb * 8 + 8, :] * x)))
                    ta.fma(kb, silu_half(yc * rh))
                for c in range(N2):
                    hb_scr[0, c * Dh:(c + 1) * Dh, :] = col_bcast(h1[0:1, c * Dh:(c + 1) * Dh])
                tb = MatVec(hb_scr, 0, w2f, 0, 0, nkb=N2 * 16)
                while tb.kb < tb.nkb:
                    tb.step(4, None)
                return m, out + rowsum(ta.acc + tb.acc)

            x = rowsum(acc_scr[...] + out_proj_fast(o * l_scr[HL], HL))
            m1, y1 = ffn_fast(x)
            x = (x - m1) + y1

            m, r, stok = stats(x)
            rs = r * (scale * LOG2E)

            def fin_q(qa, g):
                return pick_rows((qa - m * cq[:, g * G:(g + 1) * G]) * rs)
            x16 = x.astype(BF16)
            for c, xr in enumerate(blocks(x)):
                if c == D // Dh - 1:
                    xr = xr + stok
                xb_scr[0, c * Dh:(c + 1) * Dh, :] = col_bcast(xr[0:1, :])

            qs, os_, linv_, mx_ = {}, {}, {}, {}
            state = {"acc": jnp.where(rowg == 0, x - m, 0.0)}
            shift = c_scr[:, 0:1] + m1 + m
            live, fin = [None], []
            chunk_no = [0]
            k_at, os_at, e_at = {}, {}, {}
            todo = list(QUEUE)
            stack, etasks, due = [], [], []
            credit = [0.0]
            e_started, ep_ok = set(), set()
            last_tok = [None]

            def matvec_gen(mv):
                while mv.kb < NKB:
                    tok = yield 36
                    mv.step(4, tok)
                    live[0] = mv

            def q_gen(g):
                mv = MatVec(xb_scr, 0, wqf, 0, g * G - Q0)
                yield from matvec_gen(mv)
                qs[g] = fin_q(rowsum(mv.acc), g)
                return mk_tok(qs[g])

            def e_gen(g):
                m_ = jnp.broadcast_to(jnp.max(mx_[g], axis=1, keepdims=True), (8, Dh))
                m_ = jnp.maximum(m_, pltpu.roll(m_, 4, 0))
                lp = None
                order_ = list(range(NBLK))
                if g in vpu_p:
                    order_ = order_[NBLK - NVP:] + order_[:NBLK - NVP]
                for u in range(0, NBLK, EUNIT):
                    tok = yield ECOST * EUNIT
                    mm = m_ if tok is None else m_ + tok
                    for c in order_[u:u + EUNIT]:
                        pc = jnp.exp2(pf_scr[g, :, c * Dh:(c + 1) * Dh] - mm)
                        pf_scr[g, :, c * Dh:(c + 1) * Dh] = pc
                        lp = pc if lp is None else lp + pc
                    fin.append(lp)
                    if g in vpu_p and u + EUNIT >= NVP:
                        ep_ok.add(g)
                lp = lp + pltpu.roll(lp, 4, 0)
                linv_[g] = jnp.broadcast_to(1.0 / jnp.sum(lp, axis=1, keepdims=True), (8, Dh))
                e_at[g] = chunk_no[0]

            def p_gen(g):
                slot = g % 3
                for dg in range(Dh // 16):
                    accs = [None] * rep
                    for blk in range(NVP):
                        for hf in range(2):
                            tok = yield 20
                            col = (hf * NVP + blk) * Dh
                            vt = vtf[g, dg * 16:dg * 16 + 16, col:col + Dh]
                            if tok is not None:
                                vt = vt + tile_rows(tok, 2)
                            for j in range(rep):
                                r_ = hf * 4 + j
                                t = pf_scr[g, r_:r_ + 1, VP0 + blk * Dh:VP0 + (blk + 1) * Dh] * vt
                                accs[j] = t if accs[j] is None else accs[j] + t
                            live[0] = list(accs)
                    for j in range(rep):
                        pa_scr[slot, j * Dh + dg * 16:j * Dh + dg * 16 + 16, :] = accs[j]
                    fin.extend(halves(sum_all(accs)))
                    live[0] = None

            def o_gen(g):
                slot = g % 2
                linv = linv_[g]
                for j in range(rep):
                    tok = yield 48
                    orow = os_[g] if tok is None else os_[g] + tok
                    z = jnp.where(eye, jnp.broadcast_to(orow[j:j + 1, :], (Dh, Dh)), 0.0)
                    if g in vpu_p:
                        z = z + pa_scr[g % 3, j * Dh:(j + 1) * Dh, :]
                    ob_scr[slot, j * Dh:(j + 1) * Dh, :] = lanesum(z) * jnp.broadcast_to(linv[j:j + 1, :], (Dh, Dh))
                mv = MatVec(ob_scr, slot, wof, g * G, 0)
                yield from matvec_gen(mv)
                state["acc"] = state["acc"] + mv.acc
                return mk_tok(sum_all(blocks(mv.acc)))

            def ready(t):
                k_, g_ = t[0], int(t[1])
                if k_ == "p":
                    return g_ in ep_ok
                if k_ == "o":
                    return g_ in os_ and chunk_no[0] >= os_at[g_] + OLAG
                return True

            def run_vpu(tok, budget, force_e=None, flush=False):
                live[0] = None
                for g_, a_ in k_at.items():
                    if g_ not in e_started and (chunk_no[0] >= a_ + ELAG or g_ == force_e):
                        e_started.add(g_)
                        gen = e_gen(g_)
                        etasks.append([gen, next(gen)])
                credit[0] = 1e12 if flush else min(credit[0] + budget, 2 * RATE)
                while etasks:
                    credit[0] -= etasks[0][1]
                    try:
                        etasks[0][1] = etasks[0][0].send(tok)
                    except StopIteration:
                        etasks.pop(0)
                    if not flush:
                        break
                while True:
                    if not stack:
                        if not todo or (not flush and not ready(todo[0])):
                            break
                        t = todo.pop(0)
                        gen = {"q": q_gen, "p": p_gen, "o": o_gen}[t[0]](int(t[1]))
                        stack.append([gen, next(gen)])
                    cur = stack[-1]
                    if credit[0] < cur[1]:
                        break
                    credit[0] -= cur[1]
                    try:
                        cur[1] = cur[0].send(tok)
                    except StopIteration as e:
                        if e.value is not None:
                            due.append((chunk_no[0] + LAG, e.value))
                        live[0] = None
                        stack.pop()
                cov = list(fin)
                if isinstance(live[0], MatVec):
                    cov += blocks(live[0].acc)
                elif live[0]:
                    cov += halves(sum_all(live[0]))
                del fin[:]
                if cov and not flush:
                    due.append((chunk_no[0] + LAG, mk_tok(sum_all(cov))))

            def take_due():
                toks = [t for c_, t in due if c_ <= chunk_no[0]]
                due[:] = [(c_, t) for c_, t in due if c_ > chunk_no[0]]
                return sum_all(toks) if toks else None

            def qk2(g):
                while g not in qs:
                    run_vpu(last_tok[0], RATE)
                qq = qs[g]
                mx = None
                n = CB * Dh
                for c0 in range(0, NBLK, CB):
                    dtok = take_due()
                    if c0 == 0 or dtok is not None:
                        if dtok is not None:
                            qq = qq + dtok
                        qa = qq.astype(BF16)
                        qb = pltpu.roll(qq, 4, 0).astype(BF16)
                    sc = (jnp.dot(qa, load_kt(g, c0 * Dh, n), preferred_element_type=F32)
                          + jnp.dot(qb, load_kt(g, SW + c0 * Dh, n), preferred_element_type=F32))
                    pf_scr[g, :, c0 * Dh:c0 * Dh + n] = sc
                    for v in blocks(sc):
                        mx = v if mx is None else jnp.maximum(mx, v)
                    chunk_no[0] += 1
                    last_tok[0] = mk_tok(sc[:, 0:Dh])
                    run_vpu(last_tok[0], RATE)
                mx_[g] = mx

            def pv2(g):
                while g not in e_at:
                    run_vpu(last_tok[0], RATE, force_e=g)
                nb = NBLK - (NVP if g in vpu_p else 0)
                o1 = None
                o2 = None
                n = CB * Dh
                for c0 in range(0, nb, CB):
                    pc = pf_scr[g, :, c0 * Dh:c0 * Dh + n]
                    dtok = take_due()
                    if dtok is not None:
                        pc = jnp.concatenate([pc[:, 0:Dh] + dtok, pc[:, Dh:]], axis=1)
                    pc = pc.astype(BF16)
                    oc = jnp.dot(pc, load_v(g, c0 * Dh, n), preferred_element_type=F32)
                    o1 = oc if o1 is None else o1 + oc
                    oc2 = jnp.dot(pc, load_v(g, SW + c0 * Dh, n), preferred_element_type=F32)
                    o2 = oc2 if o2 is None else o2 + oc2
                    chunk_no[0] += 1
                    last_tok[0] = mk_tok(oc)
                    run_vpu(last_tok[0], RATE)
                return o1 + pltpu.roll(o2, 4, 0)

            for g in mxu_q:
                qs[g] = fin_q(jnp.dot(x16, pltpu.bitcast(wqp[mxu_q.index(g)], BF16), preferred_element_type=F32), g)
            for _ in range(PRE):
                run_vpu(None, RATE)
            pending_o = []
            for ph in ORDER:
                kind, g = ph[0], int(ph[1])
                if kind == "K":
                    qk2(g)
                    k_at[g] = chunk_no[0]
                else:
                    os_[g] = pv2(g)
                    os_at[g] = chunk_no[0]
                for og in pending_o:
                    state["acc"] = state["acc"] + out_proj_fast(os_[og] * linv_[og], og)
                pending_o = [g] if (kind == "V" and g in mxu_o) else []
            run_vpu(last_tok[0], 0, flush=True)
            for og in pending_o:
                state["acc"] = state["acc"] + out_proj_fast(os_[og] * linv_[og], og)
            x = rowsum(state["acc"])
            x = (x + shift) + ffn_fast(x)[1]
            o_ref[1:2, :] = x[0:1, :].astype(o_ref.dtype)

        pl.run_scoped(
            part_b,
            pltpu.VMEM((Hkv, Dh // 2, S), U32),
            pltpu.VMEM((Hkv, S // 2, Dh), U32),
            pltpu.VMEM((len(vpu_p), Dh, 2 * NVP * Dh), F32),
        )

    def kernel(*refs):
        pl.run_scoped(lambda sems: body(*refs, sems), pltpu.SemaphoreType.DMA((NSEM,)))

    assert NBLK % CB == 0 and (NBLK - NVP) % CB == 0 and CB >= 2
    out = pl.pallas_call(
        kernel,
        out_shape=jax.ShapeDtypeStruct((B, D), A_x.dtype),
        in_specs=[pl.BlockSpec(memory_space=pl.ANY)] * 7,
        out_specs=pl.BlockSpec(memory_space=pltpu.VMEM),
        scratch_shapes=[
            pltpu.VMEM((B, D), BF16),
            pltpu.VMEM((2, Hkv, S + 16, Dh), BF16),
            pltpu.VMEM((D, Hq * Dh), BF16),
            pltpu.VMEM((Hq * Dh, D), BF16),
            pltpu.VMEM((D, Fdim), BF16),
            pltpu.VMEM((Fdim, D), BF16),
            pltpu.VMEM((D, Hq * Dh - Q0), F32),
            pltpu.VMEM((len(vpu_o) * G, D), F32),
            pltpu.VMEM((N2 * Dh, D), F32),
            pltpu.VMEM((NF * Dh, D), F32),
            pltpu.VMEM((NF * Dh, D), F32),
            pltpu.VMEM((len(mxu_q), D // 2, G), U32),
            pltpu.VMEM((len(mxu_o), G // 2, D), U32),
            pltpu.VMEM((D // 2, FM), U32),
            pltpu.VMEM(((FM - N2 * Dh) // 2, D), U32),
            pltpu.VMEM((8, Hq * Dh), F32),
            pltpu.VMEM((8, FM), F32),
            pltpu.VMEM((8, S), F32),
            pltpu.VMEM((8, Dh), F32),
            pltpu.VMEM((8, D), F32),
            pltpu.VMEM((Hkv, 8, S), BF16),
            pltpu.VMEM((Hkv, 8, Dh), F32),
            pltpu.VMEM((8, Dh), F32),
            pltpu.VMEM((8, Dh), F32),
            pltpu.VMEM((1, D, Dh), F32),
            pltpu.VMEM((1, N2 * Dh, Dh), F32),
            pltpu.VMEM((2, G, Dh), F32),
            pltpu.VMEM((Hkv, 8, SW), F32),
            pltpu.VMEM((3, G, Dh), F32),
            pltpu.VMEM((8, Dh), jnp.int32),
        ],
        compiler_params=pltpu.CompilerParams(vmem_limit_bytes=120 * 1024 * 1024, disable_bounds_checks=True),
    )(A_x.reshape(B, D), A_k_cache, A_v_cache, A_wq, A_wo, B_w1, B_w2)
    return out.reshape(B, Sq, D)
```

```python
import jax
import jax.numpy as jnp
from jax import lax
import jax.experimental.pallas as pl
import jax.experimental.pallas.tpu as pltpu

F32 = jnp.float32
BF16 = jnp.bfloat16
U32 = jnp.uint32
NT = (((1,), (1,)), ((), ()))
LOG2E = 1.4426950408889634

HROWS = 64
LAST_TWO = (1536, 512)
GAP = 27
I1 = 370
IDLE_A = (60, 80, 50)
EMB0 = 12
EMB2 = 16
EMBK = 16
K0HI = 1
NE = 80
EMBL = 12
N7 = 24
IDLE_E = (26, 4)
EMBV = 6
GAPE = 34
CUT = 0

ORDER = "K0 K1 K2 K3 V0 K4 V1 K5 V2 K6 V3 K7 V4 V5 V6 V7".split()
QUEUE = "q2 q3 q4 q5 q6 q7 p0 p1 p2 o0 p3 o1 p4 o2 p5 o3 o4 o5".split()
NVP = 8
CB = 2
RATE = 102.3
LAG = 8
ELAG = 7
EUNIT = 4
ECOST = 5
OLAG = 6
PRE = 8
N2 = 2
NF = 6


@jax.jit
def pallas_interleave_layers__gqa_block_cached__dense_activation_silu__decode_kernel(
    A_x: jax.Array,
    A_k_cache: jax.Array,
    A_v_cache: jax.Array,
    A_wq: jax.Array,
    A_wo: jax.Array,
    B_x: jax.Array,
    B_w1: jax.Array,
    B_w2: jax.Array,
):
    B, Sq, D = A_x.shape
    _, Hkv, S, Dh = A_k_cache.shape
    Hq = A_wq.shape[1] // Dh
    rep = Hq // Hkv
    Fdim = B_w1.shape[1]
    assert (B, Sq, rep, Dh, Hkv) == (2, 1, 4, 128, 8) and D == rep * Dh
    G = rep * Dh
    scale = Dh ** -0.5
    eps = 1e-5
    R7 = N7 * 2 * HROWS
    LAST_CHUNKS = (S - R7 - sum(LAST_TWO),) + LAST_TWO
    NPC = S // HROWS
    SEM_W = 0
    SEM_K0 = 5
    SEM_V0 = SEM_K0 + 4
    SEM_K1 = SEM_V0 + 4
    SEM_V1 = SEM_K1 + 4
    SEM_L = SEM_V1 + 4
    NL = len(LAST_CHUNKS)
    SEM_K1X = SEM_L + NL
    SEM_X2 = SEM_K1X + 1
    SEM_K07 = SEM_X2 + 1
    SEM_7 = SEM_K07 + 1
    NSEM = SEM_7 + 1
    K1X = 2 * EMBL * HROWS
    lc_off = [R7 + sum(LAST_CHUNKS[:i]) for i in range(NL)]
    HL = Hkv - 1
    vpu_q = [g for g in range(Hkv) if "q%d" % g in QUEUE]
    vpu_o = [g for g in range(Hkv) if "o%d" % g in QUEUE]
    vpu_p = [g for g in range(Hkv) if "p%d" % g in QUEUE]
    mxu_q = [g for g in range(Hkv) if g not in vpu_q]
    mxu_o = [g for g in range(Hkv) if g not in vpu_o]
    assert vpu_q == list(range(vpu_q[0], Hkv)) and vpu_o == list(range(len(vpu_o)))
    assert vpu_p == list(range(len(vpu_p))) and set(vpu_p) <= set(vpu_o) and HL in mxu_o
    Q0 = vpu_q[0] * G
    SW = S // 2
    NBLK = SW // Dh
    VP0 = SW - NVP * Dh
    NKB = D // 8
    FM = Fdim - NF * Dh

    def body(x_hbm, k_hbm, v_hbm, wq_hbm, wo_hbm, w1_hbm, w2_hbm, o_ref,
             xbuf, kv1, wq, wo, w1, w2, wqf, wof, w2f, w1t, w2g,
             wqp, wop, w1p, w2p, cq, c1, d_scr, acc_scr, p_scr, l_scr, o_scr, c_scr,
             xb_scr, hb_scr, ob_scr, pf_scr, pa_scr, z_scr, sems):
        hbm = (k_hbm, v_hbm)

        def cp_big(buf, t, b, h0, nh, sem, r0=0, r1=S):
            hs, rs_ = pl.ds(h0, nh), pl.ds(r0, r1 - r0)
            return pltpu.make_async_copy(hbm[t].at[b, hs, rs_], buf.at[t, hs, rs_], sems.at[sem])

        def hi_start(buf, t, b, pair0, sem0, p):
            pr = p // NPC
            hs = pl.ds(2 * (pair0 + pr), 2)
            rs_ = pl.ds(pl.multiple_of((p % NPC) * HROWS, HROWS), HROWS)
            pltpu.make_async_copy(hbm[t].at[b, hs, rs_], buf.at[t, hs, rs_], sems.at[sem0 + pr]).start(priority=0)

        def hi7_start(p):
            rs_ = pl.ds(pl.multiple_of(p * 2 * HROWS, 2 * HROWS), 2 * HROWS)
            pltpu.make_async_copy(v_hbm.at[1, HL, rs_], kv1.at[1, HL, rs_], sems.at[SEM_7]).start(priority=0)

        def cp_vl(i):
            sl = pl.ds(lc_off[i], LAST_CHUNKS[i])
            return pltpu.make_async_copy(v_hbm.at[1, HL, sl], kv1.at[1, HL, sl], sems.at[SEM_L + i])

        cps_w = [pltpu.make_async_copy(s_, d_, sems.at[SEM_W + i]) for i, (s_, d_) in enumerate(
            ((x_hbm, xbuf), (wq_hbm, wq), (wo_hbm, wo), (w1_hbm, w1), (w2_hbm, w2)))]
        cps_k1 = [cp_big(kv1, 0, 1, 2 * i, 2, SEM_K1 + i, K1X if i == 2 else 0) for i in range(4)]
        cp_k1x = cp_big(kv1, 0, 1, 4, 2, SEM_K1X, 0, K1X)
        cps_v1 = [cp_big(kv1, 1, 1, 2 * i, 2, SEM_V1 + i, 0, NE * HROWS if i == 2 else S) for i in range(3)]
        cp_x2 = cp_big(kv1, 1, 1, 4, 2, SEM_X2, NE * HROWS)
        cps_v1.append(cp_big(kv1, 1, 1, 6, 1, SEM_V1 + 3))

        def idle_loop(n, gap, start):
            def it(i, y):
                start(i)
                for _ in range(gap):
                    y = y * 0.5 + 1.0
                return y
            if n > 0:
                d_scr[...] = lax.fori_loop(0, n, it, d_scr[...])
        cps_l = [cp_vl(i) for i in range(NL)]
        for c in cps_w:
            c.start(priority=1)

        row8 = lax.broadcasted_iota(jnp.int32, (8, Dh), 0)
        rowg = lax.broadcasted_iota(jnp.int32, (8, G), 0)
        colg = lax.broadcasted_iota(jnp.int32, (8, G), 1)
        diag_mask = rowg == (colg // Dh)
        eye = (lax.broadcasted_iota(jnp.int32, (Dh, Dh), 0) == lax.broadcasted_iota(jnp.int32, (Dh, Dh), 1))

        def pick_rows(qa):
            qg = jnp.zeros((8, Dh), F32)
            for j in range(rep):
                qg = jnp.where(row8 == j, qa[:, j * Dh:(j + 1) * Dh], qg)
            return qg

        def diag_lhs(o):
            o4 = jnp.concatenate([o] * rep, axis=1)
            return jnp.where(diag_mask, o4, 0.0).astype(BF16)

        def out_proj_fast(o, g):
            return jnp.dot(diag_lhs(o), pltpu.bitcast(wop[mxu_o.index(g)], BF16), preferred_element_type=F32)

        def rowsum(a):
            return jnp.broadcast_to(jnp.sum(a, axis=0, keepdims=True), a.shape)

        def lanesum(a):
            return jnp.broadcast_to(jnp.sum(a, axis=1, keepdims=True), (a.shape[0], Dh))

        def col_bcast(row):
            return lanesum(jnp.where(eye, jnp.broadcast_to(row, (Dh, Dh)), 0.0))

        def layernorm(x):
            xc = x - jnp.mean(x, axis=-1, keepdims=True)
            return xc * lax.rsqrt(jnp.mean(xc * xc, axis=-1, keepdims=True) + eps)

        def compute_q(x):
            xn = layernorm(x).astype(BF16)
            for g in range(Hkv):
                qa = jnp.dot(xn, wq[:, g * G:(g + 1) * G], preferred_element_type=F32) * scale
                kv1[0, g, S:S + 8, :] = pick_rows(qa).astype(BF16)

        def softmax_parts(s):
            p = jnp.exp(s - jnp.max(s, axis=1, keepdims=True))
            return p.astype(BF16), jnp.sum(p, axis=1, keepdims=True)

        def out_proj(o, h):
            w = wo[pl.ds(pl.multiple_of(h * G, G), G), :]
            return jnp.dot(diag_lhs(o), w, preferred_element_type=F32)

        def ffn(x):
            hh = jnp.dot(layernorm(x).astype(BF16), w1[...], preferred_element_type=F32)
            hh = hh * jax.nn.sigmoid(hh)
            return jnp.dot(hh.astype(BF16), w2[...], preferred_element_type=F32)

        def part_a(kv0):
            cps_k0 = [cp_big(kv0, 0, 0, 2 * i, 2 if i < 3 else 1, SEM_K0 + i) for i in range(4)]
            cp_k07 = cp_big(kv0, 0, 0, HL, 1, SEM_K07)
            cps_v0 = [cp_big(kv0, 1, 0, 2 * i, 2, SEM_V0 + i) for i in range(4)]
            for c in cps_k0[K0HI:] + [cp_k07] + ([] if CUT >= 2 else cps_k1[0:3] + [cps_v1[1], cp_x2, cps_v1[3]] + cps_l):
                c.start(priority=1)
            issued = [0]

            NA = (4 + K0HI) * NPC

            def seg_a(p):
                if p < K0HI * NPC:
                    return 0, K0HI * NPC, lambda q: hi_start(kv0, 0, 0, 0, SEM_K0, q)
                return K0HI * NPC, NA, lambda q: hi_start(kv0, 1, 0, 0, SEM_V0, q)

            def idle_v0(n):
                n = max(min(n, NA - issued[0]), 0)
                while n > 0:
                    s0, s1, st = seg_a(issued[0])
                    k = min(n, s1 - issued[0])
                    idle_loop(k, GAP, lambda i, o_=issued[0] - s0, st=st: st(o_ + i))
                    issued[0] += k
                    n -= k

            def take_a(n):
                s0, s1, st = seg_a(issued[0])
                if issued[0] + n > s1:
                    return None
                o_ = issued[0] - s0
                issued[0] += n
                return lambda q: st(o_ + q)

            def attn_head0(h, emb, start):
                nq = (2 * emb + 2) // 3 if emb else 1
                nv = emb - nq if emb else 1
                ss = []
                for c in range(nq):
                    r0, r1 = (c * (S // Dh) // nq) * Dh, ((c + 1) * (S // Dh) // nq) * Dh
                    ss.append(lax.dot_general(kv1[0, h, S:S + 8, :], kv0[0, h, r0:r1, :], NT,
                                              preferred_element_type=F32))
                    if emb:
                        start(c)
                p, l = softmax_parts(jnp.concatenate(ss, axis=1))
                o = None
                for c in range(nv):
                    r0, r1 = (c * (S // Dh) // nv) * Dh, ((c + 1) * (S // Dh) // nv) * Dh
                    pc = p[:, r0:r1]
                    if emb:
                        z = kv1[1, h, S:S + 8, :]
                        pc = jnp.concatenate([pc[:, 0:Dh] + z, pc[:, Dh:]], axis=1)
                    oc = jnp.dot(pc, kv0[1, h, r0:r1, :], preferred_element_type=F32)
                    o = oc if o is None else o + oc
                    if emb:
                        start(nq + c)
                acc_scr[...] += out_proj(o / l, h)

            d_scr[...] = jnp.zeros_like(d_scr)
            for h in range(Hkv):
                kv1[1, h, S:S + 16, :] = jnp.zeros((16, Dh), BF16)
            idle_v0(I1)
            for c in cps_w:
                c.wait()

            st_q = take_a(D // 64)
            st_o = take_a(len(vpu_o))

            def prep_q(i, c):
                st_q(i)
                off = pl.multiple_of(i * 64, 64)
                wqf[pl.ds(off, 64), :] = wq[pl.ds(off, 64), Q0:].astype(F32)
                return c
            lax.fori_loop(0, D // 64, prep_q, 0)

            def prep_o(i, c):
                st_o(i)
                off = pl.multiple_of(i * G, G)
                wof[pl.ds(off, G), :] = wo[pl.ds(off, G), :].astype(F32)
                return c
            lax.fori_loop(0, len(vpu_o), prep_o, 0)
            for i, g in enumerate(mxu_q):
                wqp[i] = pltpu.bitcast(wq[:, g * G:(g + 1) * G], U32)
            for i, g in enumerate(mxu_o):
                wop[i] = pltpu.bitcast(wo[g * G:(g + 1) * G, :], U32)
            w1p[...] = pltpu.bitcast(w1[:, 0:FM], U32)
            w2p[...] = pltpu.bitcast(w2[N2 * Dh:FM, :], U32)
            for i in range(N2):
                w2f[i * Dh:(i + 1) * Dh, :] = w2[i * Dh:(i + 1) * Dh, :].astype(F32)
            w1t[...] = w1[:, FM:].astype(F32).T
            w2g[...] = w2[FM:, :].astype(F32)
            w1t[...] = w1t[...] - jnp.mean(w1t[...], axis=1, keepdims=True)
            ones8 = jnp.ones((8, D), BF16)
            cq[...] = jnp.dot(ones8, wq[...], preferred_element_type=F32)
            c1[...] = jnp.dot(ones8, w1[:, 0:FM], preferred_element_type=F32)
            z_scr[...] = jnp.zeros_like(z_scr)

            x = jnp.broadcast_to(xbuf[0:1, :].astype(F32), (8, D))
            compute_q(x)
            acc_scr[...] = jnp.zeros_like(acc_scr)
            for i in range(4):
                if i:
                    idle_v0(IDLE_A[i - 1])
                idle_v0((K0HI + i + 1) * NPC - issued[0])
                cps_k0[i].wait()
                cps_v0[i].wait()
                if i < 3:
                    emb, st = EMB0, take_a(2 * EMB0)
                else:
                    emb, st = EMBL, lambda q: hi_start(kv1, 0, 1, 2, SEM_K1X, q)
                if st is None or (CUT >= 2 and i == 3):
                    emb = 0

                def body1(h, c, emb=emb, st=st, i=i):
                    attn_head0(h, emb, lambda j: st((h - 2 * i) * emb + j))
                    return c
                lax.fori_loop(2 * i, min(2 * i + 2, HL), body1, 0)
            cp_k07.wait()
            if CUT >= 2:
                o_ref[...] = xbuf[...]
                return
            lax.fori_loop(HL, Hkv, body1, 0)
            x = x + rowsum(acc_scr[...])
            x = x + ffn(x)
            compute_q(x)
            acc_scr[...] = jnp.zeros_like(acc_scr)

            def body2(h, c):
                attn_head0(h, EMB2, lambda j: hi_start(kv1, 0, 1, 3, SEM_K1 + 3, h * EMB2 + j))
                return c
            lax.fori_loop(0, Hkv, body2, 0)
            x = x + rowsum(acc_scr[...])
            x = x + ffn(x)
            o_ref[0:1, :] = x[0:1, :].astype(o_ref.dtype)

        assert Hkv * EMB2 == NPC and Hkv * EMBK == NPC and K0HI <= 1
        pl.run_scoped(part_a, pltpu.VMEM((2, Hkv, S, Dh), BF16))

        def part_b(ktbuf, vpk, vtf):
            def load_v(h, off, n):
                return pltpu.bitcast(vpk[h, off // 2:(off + n) // 2, :], BF16)

            def load_kt(h, off, n):
                return pltpu.bitcast(ktbuf[h, :, off:off + n], BF16)

            def pv_last(i):
                o_, n = lc_off[i], LAST_CHUNKS[i]
                v = kv1[1, HL, o_:o_ + n, :]
                vpk[HL, o_ // 2:(o_ + n) // 2, :] = pltpu.bitcast(v, U32)
                return jnp.dot(p_scr[HL, :, o_:o_ + n], v, preferred_element_type=F32)

            def kside1(h, c):
                sub = S // EMBK
                ss = []
                for u in range(EMBK):
                    kt = kv1[0, h, u * sub:(u + 1) * sub, :].T
                    ktbuf[h, :, u * sub:(u + 1) * sub] = pltpu.bitcast(kt, U32)
                    ss.append(jnp.dot(kv1[0, h, S:S + 8, :], kt, preferred_element_type=F32))
                    hi_start(kv1, 1, 1, 0, SEM_V1, h * EMBK + u)
                p, l = softmax_parts(jnp.concatenate(ss, axis=1))
                p_scr[h] = p
                l_scr[h] = jnp.broadcast_to(1.0 / l, (8, Dh))
                return c

            def vside1(h, tr, emb, st):
                if tr:
                    for hf in range(2):
                        vtf[h, :, hf * NVP * Dh:(hf + 1) * NVP * Dh] = (
                            kv1[1, h, hf * SW + VP0:(hf + 1) * SW, :].astype(F32).T)
                o = None
                nv = max(emb, 1)
                for c in range(nv):
                    r0, r1 = (c * (S // Dh) // nv) * Dh, ((c + 1) * (S // Dh) // nv) * Dh
                    v = kv1[1, h, r0:r1, :]
                    vpk[h, r0 // 2:r1 // 2, :] = pltpu.bitcast(v, U32)
                    oc = jnp.dot(p_scr[h, :, r0:r1], v, preferred_element_type=F32)
                    o = oc if o is None else o + oc
                    if emb:
                        st(c)
                acc_scr[...] += out_proj(o * l_scr[h], h)

            def st2(p):
                hi_start(kv1, 1, 1, 2, SEM_V1 + 2, p)

            def vloop(h0, h1, tr, emb, st, p0):
                def bd(h, c):
                    vside1(h, tr, emb, lambda j: st(p0 + (h - h0) * emb + j))
                    return c
                lax.fori_loop(h0, h1, bd, 0)
                return p0 + (h1 - h0) * emb

            x = jnp.broadcast_to(xbuf[1:2, :].astype(F32), (8, D))
            compute_q(x)
            for i in (0, 1, 3, 2):
                cps_k1[i].wait()
                if i == 2:
                    cp_k1x.wait()
                lax.fori_loop(2 * i, 2 * i + 2, kside1, 0)
            c0 = jnp.mean(x, axis=-1, keepdims=True)
            c_scr[...] = jnp.broadcast_to(c0, (8, Dh))
            acc_scr[...] = jnp.where(rowg == 0, x - c0, 0.0)
            assert vpu_p == list(range(6))
            cps_v1[0].wait()
            ne = vloop(0, 2, True, EMBV, st2, 0)
            idle_loop(IDLE_E[0], GAPE, lambda i, p0=ne: st2(p0 + i))
            cps_v1[1].wait()
            ne = vloop(2, 4, True, EMBV, st2, ne + IDLE_E[0])
            idle_loop(NE - ne, GAPE, lambda i, p0=ne: st2(p0 + i))
            n7 = min(IDLE_E[1], N7 - 2 * EMBV)
            idle_loop(n7, GAPE, hi7_start)
            cps_v1[2].wait()
            cp_x2.wait()
            n7 = vloop(4, 6, True, EMBV, hi7_start, n7)
            idle_loop(N7 - n7, GAPE, lambda i, p0=n7: hi7_start(p0 + i))
            cps_v1[3].wait()
            vloop(6, 7, False, 0, None, 0)
            cp_big(kv1, 1, 1, HL, 1, SEM_7, 0, R7).wait()
            v7 = kv1[1, HL, 0:R7, :]
            vpk[HL, 0:R7 // 2, :] = pltpu.bitcast(v7, U32)
            o_scr[...] = jnp.dot(p_scr[HL, :, 0:R7], v7, preferred_element_type=F32)
            for i in range(NL - 1):
                cps_l[i].wait()
                o_scr[...] += pv_last(i)
            cps_l[NL - 1].wait()
            o = o_scr[...] + pv_last(NL - 1)
            if CUT:
                o_ref[1:2, :] = jnp.concatenate([o] * 4, axis=1)[0:1, :].astype(o_ref.dtype)
                return

            zero_i = z_scr[...]

            def mk_tok(v):
                return lax.bitcast_convert_type(lax.bitcast_convert_type(v, jnp.int32) & zero_i, F32)

            def sum_all(vs):
                t = vs[0]
                for v in vs[1:]:
                    t = t + v
                return t

            def blocks(a):
                return [a[:, c * Dh:(c + 1) * Dh] for c in range(a.shape[1] // Dh)]

            def halves(a):
                return [a[0:8, :], a[8:16, :]]

            def stats(x):
                s1 = sum_all(blocks(x))
                s2 = sum_all(blocks(x * x))
                m = jnp.sum(s1, axis=-1, keepdims=True) * (1.0 / D)
                m2 = jnp.sum(s2, axis=-1, keepdims=True) * (1.0 / D)
                v = jnp.maximum(m2 - m * m, 0.0)
                return m, lax.rsqrt(v + eps), mk_tok(s1 + s2)

            def silu_half(a):
                return a + a * jnp.tanh(a)

            tile_cache = {}

            def tile_rows(tok, n):
                if (id(tok), n) not in tile_cache:
                    tile_cache[(id(tok), n)] = (tok, jnp.concatenate([tok] * n, axis=0))
                return tile_cache[(id(tok), n)][1]

            class MatVec:
                def __init__(self, xb_ref, slot, w_ref, row0, col0, nkb=NKB):
                    self.xb_ref, self.slot, self.w_ref, self.row0, self.col0 = xb_ref, slot, w_ref, row0, col0
                    self.acc = None
                    self.kb = 0
                    self.nkb = nkb

                def step(self, n, tok):
                    xv = self.xb_ref[self.slot, self.kb * 8:(self.kb + n) * 8, :]
                    if tok is not None:
                        xv = xv + tile_rows(tok, n)
                    self.fma(self.kb, xv)
                    self.kb += n

                def fma(self, kb, xv):
                    r0, n = self.row0 + kb * 8, xv.shape[0]
                    t = jnp.concatenate([xv] * rep, axis=1) * self.w_ref[r0:r0 + n, self.col0:self.col0 + G]
                    for i in range(0, n, 8):
                        ti = t[i:i + 8, :] if n > 8 else t
                        self.acc = ti if self.acc is None else self.acc + ti

            def ffn_fast(x):
                m, r, _ = stats(x)
                rh = 0.5 * r
                y = jnp.dot(x.astype(BF16), pltpu.bitcast(w1p[...], BF16), preferred_element_type=F32)
                h1 = silu_half((y - m * c1[...]) * rh)
                out = sum_all([
                    jnp.dot(h1[:, k0:k0 + Dh].astype(BF16),
                            pltpu.bitcast(w2p[(k0 - N2 * Dh) // 2:(k0 - N2 * Dh + Dh) // 2, :], BF16),
                            preferred_element_type=F32)
                    for k0 in range(N2 * Dh, FM, Dh)])
                ta = MatVec(None, 0, w2g, 0, 0)
                for kb in range(NF * 16):
                    yc = lanesum(sum_all(blocks(w1t[kb * 8:kb * 8 + 8, :] * x)))
                    ta.fma(kb, silu_half(yc * rh))
                for c in range(N2):
                    hb_scr[0, c * Dh:(c + 1) * Dh, :] = col_bcast(h1[0:1, c * Dh:(c + 1) * Dh])
                tb = MatVec(hb_scr, 0, w2f, 0, 0, nkb=N2 * 16)
                while tb.kb < tb.nkb:
                    tb.step(4, None)
                return m, out + rowsum(ta.acc + tb.acc)

            x = rowsum(acc_scr[...] + out_proj_fast(o * l_scr[HL], HL))
            m1, y1 = ffn_fast(x)
            x = (x - m1) + y1

            m, r, stok = stats(x)
            rs = r * (scale * LOG2E)

            def fin_q(qa, g):
                return pick_rows((qa - m * cq[:, g * G:(g + 1) * G]) * rs)
            x16 = x.astype(BF16)
            for c, xr in enumerate(blocks(x)):
                if c == D // Dh - 1:
                    xr = xr + stok
                xb_scr[0, c * Dh:(c + 1) * Dh, :] = col_bcast(xr[0:1, :])

            qs, os_, linv_, mx_ = {}, {}, {}, {}
            state = {"acc": jnp.where(rowg == 0, x - m, 0.0)}
            shift = c_scr[:, 0:1] + m1 + m
            live, fin = [None], []
            chunk_no = [0]
            k_at, os_at, e_at = {}, {}, {}
            todo = list(QUEUE)
            stack, etasks, due = [], [], []
            credit = [0.0]
            e_started, ep_ok = set(), set()
            last_tok = [None]

            def matvec_gen(mv):
                while mv.kb < NKB:
                    tok = yield 36
                    mv.step(4, tok)
                    live[0] = mv

            def q_gen(g):
                mv = MatVec(xb_scr, 0, wqf, 0, g * G - Q0)
                yield from matvec_gen(mv)
                qs[g] = fin_q(rowsum(mv.acc), g)
                return mk_tok(qs[g])

            def e_gen(g):
                m_ = jnp.broadcast_to(jnp.max(mx_[g], axis=1, keepdims=True), (8, Dh))
                m_ = jnp.maximum(m_, pltpu.roll(m_, 4, 0))
                lp = None
                order_ = list(range(NBLK))
                if g in vpu_p:
                    order_ = order_[NBLK - NVP:] + order_[:NBLK - NVP]
                for u in range(0, NBLK, EUNIT):
                    tok = yield ECOST * EUNIT
                    mm = m_ if tok is None else m_ + tok
                    for c in order_[u:u + EUNIT]:
                        pc = jnp.exp2(pf_scr[g, :, c * Dh:(c + 1) * Dh] - mm)
                        pf_scr[g, :, c * Dh:(c + 1) * Dh] = pc
                        lp = pc if lp is None else lp + pc
                    fin.append(lp)
                    if g in vpu_p and u + EUNIT >= NVP:
                        ep_ok.add(g)
                lp = lp + pltpu.roll(lp, 4, 0)
                linv_[g] = jnp.broadcast_to(1.0 / jnp.sum(lp, axis=1, keepdims=True), (8, Dh))
                e_at[g] = chunk_no[0]

            def p_gen(g):
                slot = g % 3
                for dg in range(Dh // 16):
                    accs = [None] * rep
                    for blk in range(NVP):
                        for hf in range(2):
                            tok = yield 20
                            col = (hf * NVP + blk) * Dh
                            vt = vtf[g, dg * 16:dg * 16 + 16, col:col + Dh]
                            if tok is not None:
                                vt = vt + tile_rows(tok, 2)
                            for j in range(rep):
                                r_ = hf * 4 + j
                                t = pf_scr[g, r_:r_ + 1, VP0 + blk * Dh:VP0 + (blk + 1) * Dh] * vt
                                accs[j] = t if accs[j] is None else accs[j] + t
                            live[0] = list(accs)
                    for j in range(rep):
                        pa_scr[slot, j * Dh + dg * 16:j * Dh + dg * 16 + 16, :] = accs[j]
                    fin.extend(halves(sum_all(accs)))
                    live[0] = None

            def o_gen(g):
                slot = g % 2
                linv = linv_[g]
                for j in range(rep):
                    tok = yield 48
                    orow = os_[g] if tok is None else os_[g] + tok
                    z = jnp.where(eye, jnp.broadcast_to(orow[j:j + 1, :], (Dh, Dh)), 0.0)
                    if g in vpu_p:
                        z = z + pa_scr[g % 3, j * Dh:(j + 1) * Dh, :]
                    ob_scr[slot, j * Dh:(j + 1) * Dh, :] = lanesum(z) * jnp.broadcast_to(linv[j:j + 1, :], (Dh, Dh))
                mv = MatVec(ob_scr, slot, wof, g * G, 0)
                yield from matvec_gen(mv)
                state["acc"] = state["acc"] + mv.acc
                return mk_tok(sum_all(blocks(mv.acc)))

            def ready(t):
                k_, g_ = t[0], int(t[1])
                if k_ == "p":
                    return g_ in ep_ok
                if k_ == "o":
                    return g_ in os_ and chunk_no[0] >= os_at[g_] + OLAG
                return True

            def run_vpu(tok, budget, force_e=None, flush=False):
                live[0] = None
                for g_, a_ in k_at.items():
                    if g_ not in e_started and (chunk_no[0] >= a_ + ELAG or g_ == force_e):
                        e_started.add(g_)
                        gen = e_gen(g_)
                        etasks.append([gen, next(gen)])
                credit[0] = 1e12 if flush else min(credit[0] + budget, 2 * RATE)
                while etasks:
                    credit[0] -= etasks[0][1]
                    try:
                        etasks[0][1] = etasks[0][0].send(tok)
                    except StopIteration:
                        etasks.pop(0)
                    if not flush:
                        break
                while True:
                    if not stack:
                        if not todo or (not flush and not ready(todo[0])):
                            break
                        t = todo.pop(0)
                        gen = {"q": q_gen, "p": p_gen, "o": o_gen}[t[0]](int(t[1]))
                        stack.append([gen, next(gen)])
                    cur = stack[-1]
                    if credit[0] < cur[1]:
                        break
                    credit[0] -= cur[1]
                    try:
                        cur[1] = cur[0].send(tok)
                    except StopIteration as e:
                        if e.value is not None:
                            due.append((chunk_no[0] + LAG, e.value))
                        live[0] = None
                        stack.pop()
                cov = list(fin)
                if isinstance(live[0], MatVec):
                    cov += blocks(live[0].acc)
                elif live[0]:
                    cov += halves(sum_all(live[0]))
                del fin[:]
                if cov and not flush:
                    due.append((chunk_no[0] + LAG, mk_tok(sum_all(cov))))

            def take_due():
                toks = [t for c_, t in due if c_ <= chunk_no[0]]
                due[:] = [(c_, t) for c_, t in due if c_ > chunk_no[0]]
                return sum_all(toks) if toks else None

            def qk2(g):
                while g not in qs:
                    run_vpu(last_tok[0], RATE)
                qq = qs[g]
                mx = None
                n = CB * Dh
                for c0 in range(0, NBLK, CB):
                    dtok = take_due()
                    if c0 == 0 or dtok is not None:
                        if dtok is not None:
                            qq = qq + dtok
                        qa = qq.astype(BF16)
                        qb = pltpu.roll(qq, 4, 0).astype(BF16)
                    sc = (jnp.dot(qa, load_kt(g, c0 * Dh, n), preferred_element_type=F32)
                          + jnp.dot(qb, load_kt(g, SW + c0 * Dh, n), preferred_element_type=F32))
                    pf_scr[g, :, c0 * Dh:c0 * Dh + n] = sc
                    for v in blocks(sc):
                        mx = v if mx is None else jnp.maximum(mx, v)
                    chunk_no[0] += 1
                    last_tok[0] = mk_tok(sc[:, 0:Dh])
                    run_vpu(last_tok[0], RATE)
                mx_[g] = mx

            def pv2(g):
                while g not in e_at:
                    run_vpu(last_tok[0], RATE, force_e=g)
                nb = NBLK - (NVP if g in vpu_p else 0)
                o1 = None
                o2 = None
                n = CB * Dh
                for c0 in range(0, nb, CB):
                    pc = pf_scr[g, :, c0 * Dh:c0 * Dh + n]
                    dtok = take_due()
                    if dtok is not None:
                        pc = jnp.concatenate([pc[:, 0:Dh] + dtok, pc[:, Dh:]], axis=1)
                    pc = pc.astype(BF16)
                    oc = jnp.dot(pc, load_v(g, c0 * Dh, n), preferred_element_type=F32)
                    o1 = oc if o1 is None else o1 + oc
                    oc2 = jnp.dot(pc, load_v(g, SW + c0 * Dh, n), preferred_element_type=F32)
                    o2 = oc2 if o2 is None else o2 + oc2
                    chunk_no[0] += 1
                    last_tok[0] = mk_tok(oc)
                    run_vpu(last_tok[0], RATE)
                return o1 + pltpu.roll(o2, 4, 0)

            for g in mxu_q:
                qs[g] = fin_q(jnp.dot(x16, pltpu.bitcast(wqp[mxu_q.index(g)], BF16), preferred_element_type=F32), g)
            for _ in range(PRE):
                run_vpu(None, RATE)
            pending_o = []
            for ph in ORDER:
                kind, g = ph[0], int(ph[1])
                if kind == "K":
                    qk2(g)
                    k_at[g] = chunk_no[0]
                else:
                    os_[g] = pv2(g)
                    os_at[g] = chunk_no[0]
                for og in pending_o:
                    state["acc"] = state["acc"] + out_proj_fast(os_[og] * linv_[og], og)
                pending_o = [g] if (kind == "V" and g in mxu_o) else []
            run_vpu(last_tok[0], 0, flush=True)
            for og in pending_o:
                state["acc"] = state["acc"] + out_proj_fast(os_[og] * linv_[og], og)
            x = rowsum(state["acc"])
            x = (x + shift) + ffn_fast(x)[1]
            o_ref[1:2, :] = x[0:1, :].astype(o_ref.dtype)

        if CUT >= 2:
            return
        pl.run_scoped(
            part_b,
            pltpu.VMEM((Hkv, Dh // 2, S), U32),
            pltpu.VMEM((Hkv, S // 2, Dh), U32),
            pltpu.VMEM((len(vpu_p), Dh, 2 * NVP * Dh), F32),
        )

    def kernel(*refs):
        pl.run_scoped(lambda sems: body(*refs, sems), pltpu.SemaphoreType.DMA((NSEM,)))

    assert NBLK % CB == 0 and (NBLK - NVP) % CB == 0 and CB >= 2
    out = pl.pallas_call(
        kernel,
        out_shape=jax.ShapeDtypeStruct((B, D), A_x.dtype),
        in_specs=[pl.BlockSpec(memory_space=pl.ANY)] * 7,
        out_specs=pl.BlockSpec(memory_space=pltpu.VMEM),
        scratch_shapes=[
            pltpu.VMEM((B, D), BF16),
            pltpu.VMEM((2, Hkv, S + 16, Dh), BF16),
            pltpu.VMEM((D, Hq * Dh), BF16),
            pltpu.VMEM((Hq * Dh, D), BF16),
            pltpu.VMEM((D, Fdim), BF16),
            pltpu.VMEM((Fdim, D), BF16),
            pltpu.VMEM((D, Hq * Dh - Q0), F32),
            pltpu.VMEM((len(vpu_o) * G, D), F32),
            pltpu.VMEM((N2 * Dh, D), F32),
            pltpu.VMEM((NF * Dh, D), F32),
            pltpu.VMEM((NF * Dh, D), F32),
            pltpu.VMEM((len(mxu_q), D // 2, G), U32),
            pltpu.VMEM((len(mxu_o), G // 2, D), U32),
            pltpu.VMEM((D // 2, FM), U32),
            pltpu.VMEM(((FM - N2 * Dh) // 2, D), U32),
            pltpu.VMEM((8, Hq * Dh), F32),
            pltpu.VMEM((8, FM), F32),
            pltpu.VMEM((8, Dh), F32),
            pltpu.VMEM((8, D), F32),
            pltpu.VMEM((Hkv, 8, S), BF16),
            pltpu.VMEM((Hkv, 8, Dh), F32),
            pltpu.VMEM((8, Dh), F32),
            pltpu.VMEM((8, Dh), F32),
            pltpu.VMEM((1, D, Dh), F32),
            pltpu.VMEM((1, N2 * Dh, Dh), F32),
            pltpu.VMEM((2, G, Dh), F32),
            pltpu.VMEM((Hkv, 8, SW), F32),
            pltpu.VMEM((3, G, Dh), F32),
            pltpu.VMEM((8, Dh), jnp.int32),
        ],
        compiler_params=pltpu.CompilerParams(vmem_limit_bytes=120 * 1024 * 1024, disable_bounds_checks=True),
    )(A_x.reshape(B, D), A_k_cache, A_v_cache, A_wq, A_wo, B_w1, B_w2)
    return out.reshape(B, Sq, D)
```

```python
import jax
import jax.numpy as jnp
from jax import lax
import jax.experimental.pallas as pl
import jax.experimental.pallas.tpu as pltpu

F32 = jnp.float32
BF16 = jnp.bfloat16
U32 = jnp.uint32
NT = (((1,), (1,)), ((), ()))
LOG2E = 1.4426950408889634

HROWS = 64
HRB = 32
GAP = 40
IDLE_A = (190, 120, 30)
EMB0 = 13
EMB2 = 16
EMBK = 16
EMBV = 6
NK0 = 64
IDLE_E = (4, 16)
GAPE = 34
LAST_TWO = (1536, 512)

ORDER = "K0 K1 K2 K3 V0 K4 V1 K5 V2 K6 V3 K7 V4 V5 V6 V7".split()
QUEUE = "q2 q3 q4 q5 q6 q7 p0 p1 p2 o0 p3 o1 p4 o2 p5 o3 o4 o5".split()
NVP = 8
CB = 2
RATE = 102.3
LAG = 8
ELAG = 7
EUNIT = 4
ECOST = 5
OLAG = 6
PRE = 8
N2 = 2
NF = 6


@jax.jit
def pallas_interleave_layers__gqa_block_cached__dense_activation_silu__decode_kernel(
    A_x: jax.Array,
    A_k_cache: jax.Array,
    A_v_cache: jax.Array,
    A_wq: jax.Array,
    A_wo: jax.Array,
    B_x: jax.Array,
    B_w1: jax.Array,
    B_w2: jax.Array,
):
    B, Sq, D = A_x.shape
    _, Hkv, S, Dh = A_k_cache.shape
    Hq = A_wq.shape[1] // Dh
    rep = Hq // Hkv
    Fdim = B_w1.shape[1]
    assert (B, Sq, rep, Dh, Hkv) == (2, 1, 4, 128, 8) and D == rep * Dh
    G = rep * Dh
    scale = Dh ** -0.5
    eps = 1e-5
    NPC = S // HROWS
    NK1 = 2 * EMB0 + Hkv * EMB2 + 3 * EMBK - NK0
    NV0 = 5 * EMBK + IDLE_E[0]
    NV1 = 4 * EMBV + IDLE_E[1]
    assert NK0 <= 2 * EMB0 + Hkv * EMB2 and max(NK0, NK1, NV0) * HRB < S
    R7 = NV1 * HRB
    LAST_CHUNKS = (S - R7 - sum(LAST_TWO),) + LAST_TWO
    assert LAST_CHUNKS[0] > 0 and R7 % Dh == 0
    NL = len(LAST_CHUNKS)
    lc_off = [R7 + sum(LAST_CHUNKS[:i]) for i in range(NL)]
    SEM_W = 0
    SEM_K0 = 5
    SEM_V0 = 9
    SEM_HB = 13
    SEM_LB = 17
    SEM_L = 22
    NSEM = SEM_L + NL
    HL = Hkv - 1
    vpu_q = [g for g in range(Hkv) if "q%d" % g in QUEUE]
    vpu_o = [g for g in range(Hkv) if "o%d" % g in QUEUE]
    vpu_p = [g for g in range(Hkv) if "p%d" % g in QUEUE]
    mxu_q = [g for g in range(Hkv) if g not in vpu_q]
    mxu_o = [g for g in range(Hkv) if g not in vpu_o]
    assert vpu_q == list(range(vpu_q[0], Hkv)) and vpu_o == list(range(len(vpu_o)))
    assert vpu_p == list(range(len(vpu_p))) and set(vpu_p) <= set(vpu_o) and HL in mxu_o
    Q0 = vpu_q[0] * G
    SW = S // 2
    NBLK = SW // Dh
    VP0 = SW - NVP * Dh
    NKB = D // 8
    FM = Fdim - NF * Dh

    def body(x_hbm, k_hbm, v_hbm, wq_hbm, wo_hbm, w1_hbm, w2_hbm, o_ref,
             xbuf, kv1, wq, wo, w1, w2, wqf, wof, w2f, w1t, w2g,
             wqp, wop, w1p, w2p, cq, c1, d_scr, acc_scr, p_scr, l_scr, o_scr, c_scr,
             xb_scr, hb_scr, ob_scr, pf_scr, pa_scr, z_scr, sems):
        hbm = (k_hbm, v_hbm)

        def cp_big(buf, t, b, h0, nh, sem, r0=0, r1=S):
            hs, rs_ = pl.ds(h0, nh), pl.ds(r0, r1 - r0)
            return pltpu.make_async_copy(hbm[t].at[b, hs, rs_], buf.at[t, hs, rs_], sems.at[sem])

        def hi_copy(buf, t, b, h0, nh, row, sem, nr=HROWS):
            hs, rs_ = pl.ds(h0, nh), pl.ds(pl.multiple_of(row * nr, nr), nr)
            pltpu.make_async_copy(hbm[t].at[b, hs, rs_], buf.at[t, hs, rs_], sems.at[sem]).start(priority=0)

        def hi_b(t, n0, p):
            hq = (p >= n0).astype(jnp.int32) if not isinstance(p, int) else int(p >= n0)
            hi_copy(kv1, t, 1, 4 * hq, 4, p - n0 * hq, SEM_HB + 2 * t + hq, HRB)

        def cp_vl(i):
            sl = pl.ds(lc_off[i], LAST_CHUNKS[i])
            return pltpu.make_async_copy(v_hbm.at[1, HL, sl], kv1.at[1, HL, sl], sems.at[SEM_L + i])

        cps_w = [pltpu.make_async_copy(s_, d_, sems.at[SEM_W + i]) for i, (s_, d_) in enumerate(
            ((x_hbm, xbuf), (wq_hbm, wq), (wo_hbm, wo), (w1_hbm, w1), (w2_hbm, w2)))]
        nhi = (NK0, NK1, NV0, NV1)
        hi_wait = [cp_big(kv1, i // 2, 1, 4 * (i % 2), 4, SEM_HB + i, 0, nhi[i] * HRB) for i in range(4)]
        cps_lb = [cp_big(kv1, i // 2, 1, 4 * (i % 2), 4, SEM_LB + i, nhi[i] * HRB) for i in range(3)]
        cps_lb += [cp_big(kv1, 1, 1, 4, 2, SEM_LB + 3, R7), cp_big(kv1, 1, 1, 6, 1, SEM_LB + 4, R7)]

        def idle_loop(n, gap, start):
            def it(i, y):
                start(i)
                for _ in range(gap):
                    y = y * 0.5 + 1.0
                return y
            if n > 0:
                d_scr[...] = lax.fori_loop(0, n, it, d_scr[...])
        cps_l = [cp_vl(i) for i in range(NL)]
        for c in cps_w + cps_lb + cps_l:
            c.start(priority=1)

        row8 = lax.broadcasted_iota(jnp.int32, (8, Dh), 0)
        rowg = lax.broadcasted_iota(jnp.int32, (8, G), 0)
        colg = lax.broadcasted_iota(jnp.int32, (8, G), 1)
        diag_mask = rowg == (colg // Dh)
        eye = (lax.broadcasted_iota(jnp.int32, (Dh, Dh), 0) == lax.broadcasted_iota(jnp.int32, (Dh, Dh), 1))

        def pick_rows(qa):
            qg = jnp.zeros((8, Dh), F32)
            for j in range(rep):
                qg = jnp.where(row8 == j, qa[:, j * Dh:(j + 1) * Dh], qg)
            return qg

        def diag_lhs(o):
            o4 = jnp.concatenate([o] * rep, axis=1)
            return jnp.where(diag_mask, o4, 0.0).astype(BF16)

        def out_proj_fast(o, g):
            return jnp.dot(diag_lhs(o), pltpu.bitcast(wop[mxu_o.index(g)], BF16), preferred_element_type=F32)

        def rowsum(a):
            return jnp.broadcast_to(jnp.sum(a, axis=0, keepdims=True), a.shape)

        def lanesum(a):
            return jnp.broadcast_to(jnp.sum(a, axis=1, keepdims=True), (a.shape[0], Dh))

        def col_bcast(row):
            return lanesum(jnp.where(eye, jnp.broadcast_to(row, (Dh, Dh)), 0.0))

        def layernorm(x):
            xc = x - jnp.mean(x, axis=-1, keepdims=True)
            return xc * lax.rsqrt(jnp.mean(xc * xc, axis=-1, keepdims=True) + eps)

        def compute_q(x):
            xn = layernorm(x).astype(BF16)
            for g in range(Hkv):
                qa = jnp.dot(xn, wq[:, g * G:(g + 1) * G], preferred_element_type=F32) * scale
                kv1[0, g, S:S + 8, :] = pick_rows(qa).astype(BF16)

        def softmax_parts(s):
            p = jnp.exp(s - jnp.max(s, axis=1, keepdims=True))
            return p.astype(BF16), jnp.sum(p, axis=1, keepdims=True)

        def out_proj(o, h):
            w = wo[pl.ds(pl.multiple_of(h * G, G), G), :]
            return jnp.dot(diag_lhs(o), w, preferred_element_type=F32)

        def ffn(x):
            hh = jnp.dot(layernorm(x).astype(BF16), w1[...], preferred_element_type=F32)
            hh = hh * jax.nn.sigmoid(hh)
            return jnp.dot(hh.astype(BF16), w2[...], preferred_element_type=F32)

        def part_a(kv0):
            issued = [0]

            def hi_a(p):
                for t, sem in ((0, SEM_K0), (1, SEM_V0)):
                    hi_copy(kv0, t, 0, 2 * (p // NPC), 2, p % NPC, sem + p // NPC)

            def idle_a(n):
                n = max(min(n, 4 * NPC - issued[0]), 0)
                idle_loop(n, GAP, lambda i, p0=issued[0]: hi_a(p0 + i))
                issued[0] += n

            def take_a(n):
                assert issued[0] + n <= 4 * NPC
                p0 = issued[0]
                issued[0] += n
                return lambda q: hi_a(p0 + q)

            def attn_head0(h, emb, start):
                nq = (2 * emb + 2) // 3 if emb else 1
                nv = emb - nq if emb else 1
                ss = []
                for c in range(nq):
                    r0, r1 = (c * (S // Dh) // nq) * Dh, ((c + 1) * (S // Dh) // nq) * Dh
                    ss.append(lax.dot_general(kv1[0, h, S:S + 8, :], kv0[0, h, r0:r1, :], NT,
                                              preferred_element_type=F32))
                    if emb:
                        start(c)
                p, l = softmax_parts(jnp.concatenate(ss, axis=1))
                o = None
                for c in range(nv):
                    r0, r1 = (c * (S // Dh) // nv) * Dh, ((c + 1) * (S // Dh) // nv) * Dh
                    pc = p[:, r0:r1]
                    if emb:
                        z = kv1[1, h, S:S + 8, :]
                        pc = jnp.concatenate([pc[:, 0:Dh] + z, pc[:, Dh:]], axis=1)
                    oc = jnp.dot(pc, kv0[1, h, r0:r1, :], preferred_element_type=F32)
                    o = oc if o is None else o + oc
                    if emb:
                        start(nq + c)
                acc_scr[...] += out_proj(o / l, h)

            d_scr[...] = jnp.zeros_like(d_scr)
            for h in range(Hkv):
                kv1[1, h, S:S + 16, :] = jnp.zeros((16, Dh), BF16)
            z_scr[...] = jnp.zeros_like(z_scr)
            acc_scr[...] = jnp.zeros_like(acc_scr)
            ones8 = jnp.ones((8, D), BF16)

            idle_a(IDLE_A[0])
            cps_w[0].wait()
            cps_w[1].wait()
            st_q = take_a(D // 64)

            def prep_q(i, c):
                st_q(i)
                off = pl.multiple_of(i * 64, 64)
                wqf[pl.ds(off, 64), :] = wq[pl.ds(off, 64), Q0:].astype(F32)
                return c
            lax.fori_loop(0, D // 64, prep_q, 0)
            for i, g in enumerate(mxu_q):
                wqp[i] = pltpu.bitcast(wq[:, g * G:(g + 1) * G], U32)
            cq[...] = jnp.dot(ones8, wq[...], preferred_element_type=F32)
            x = jnp.broadcast_to(xbuf[0:1, :].astype(F32), (8, D))
            compute_q(x)

            idle_a(IDLE_A[1])
            cps_w[2].wait()
            st_o = take_a(len(vpu_o))

            def prep_o(i, c):
                st_o(i)
                off = pl.multiple_of(i * G, G)
                wof[pl.ds(off, G), :] = wo[pl.ds(off, G), :].astype(F32)
                return c
            lax.fori_loop(0, len(vpu_o), prep_o, 0)
            for i, g in enumerate(mxu_o):
                wop[i] = pltpu.bitcast(wo[g * G:(g + 1) * G, :], U32)

            for i in range(4):
                if i == 3:
                    idle_a(IDLE_A[2])
                    cps_w[3].wait()
                    cps_w[4].wait()
                    w1p[...] = pltpu.bitcast(w1[:, 0:FM], U32)
                    w2p[...] = pltpu.bitcast(w2[N2 * Dh:FM, :], U32)
                    w2f[...] = w2[0:N2 * Dh, :].astype(F32)
                    w1t[...] = w1[:, FM:].astype(F32).T
                    w2g[...] = w2[FM:, :].astype(F32)
                    w1t[...] = w1t[...] - jnp.mean(w1t[...], axis=1, keepdims=True)
                    c1[...] = jnp.dot(ones8, w1[:, 0:FM], preferred_element_type=F32)
                idle_a((i + 1) * NPC - issued[0])
                cp_big(kv0, 0, 0, 2 * i, 2, SEM_K0 + i).wait()
                cp_big(kv0, 1, 0, 2 * i, 2, SEM_V0 + i).wait()
                st = take_a(2 * EMB0) if i < 3 else (lambda q: hi_b(0, NK0, q))

                def body1(h, c, st=st, i=i):
                    attn_head0(h, EMB0, lambda j: st((h - 2 * i) * EMB0 + j))
                    return c
                lax.fori_loop(2 * i, 2 * i + 2, body1, 0)
            x = x + rowsum(acc_scr[...])
            x = x + ffn(x)
            compute_q(x)
            acc_scr[...] = jnp.zeros_like(acc_scr)

            def body2(h, c):
                attn_head0(h, EMB2, lambda j: hi_b(0, NK0, 2 * EMB0 + h * EMB2 + j))
                return c
            lax.fori_loop(0, Hkv, body2, 0)
            x = x + rowsum(acc_scr[...])
            x = x + ffn(x)
            o_ref[0:1, :] = x[0:1, :].astype(o_ref.dtype)

        pl.run_scoped(part_a, pltpu.VMEM((2, Hkv, S, Dh), BF16))

        def part_b(ktbuf, vpk, vtf):
            def load_v(h, off, n):
                return pltpu.bitcast(vpk[h, off // 2:(off + n) // 2, :], BF16)

            def load_kt(h, off, n):
                return pltpu.bitcast(ktbuf[h, :, off:off + n], BF16)

            def pv_last(i):
                o_, n = lc_off[i], LAST_CHUNKS[i]
                v = kv1[1, HL, o_:o_ + n, :]
                vpk[HL, o_ // 2:(o_ + n) // 2, :] = pltpu.bitcast(v, U32)
                return jnp.dot(p_scr[HL, :, o_:o_ + n], v, preferred_element_type=F32)

            def kside1(h, st):
                ss = []
                for u in range(EMBK):
                    r0, r1 = (u * (S // Dh) // EMBK) * Dh, ((u + 1) * (S // Dh) // EMBK) * Dh
                    kt = kv1[0, h, r0:r1, :].T
                    ktbuf[h, :, r0:r1] = pltpu.bitcast(kt, U32)
                    ss.append(jnp.dot(kv1[0, h, S:S + 8, :], kt, preferred_element_type=F32))
                    st(u)
                p, l = softmax_parts(jnp.concatenate(ss, axis=1))
                p_scr[h] = p
                l_scr[h] = jnp.broadcast_to(1.0 / l, (8, Dh))

            def kloop(h0, h1, st, p0):
                def bd(h, c):
                    kside1(h, lambda j: st(p0 + (h - h0) * EMBK + j))
                    return c
                lax.fori_loop(h0, h1, bd, 0)

            def vside1(h, tr, emb, st):
                if tr:
                    for hf in range(2):
                        vtf[h, :, hf * NVP * Dh:(hf + 1) * NVP * Dh] = (
                            kv1[1, h, hf * SW + VP0:(hf + 1) * SW, :].astype(F32).T)
                o = None
                nv = max(emb, 1)
                for c in range(nv):
                    r0, r1 = (c * (S // Dh) // nv) * Dh, ((c + 1) * (S // Dh) // nv) * Dh
                    v = kv1[1, h, r0:r1, :]
                    vpk[h, r0 // 2:r1 // 2, :] = pltpu.bitcast(v, U32)
                    oc = jnp.dot(p_scr[h, :, r0:r1], v, preferred_element_type=F32)
                    o = oc if o is None else o + oc
                    if emb:
                        st(c)
                acc_scr[...] += out_proj(o * l_scr[h], h)

            def stv(p):
                hi_b(1, NV0, p)

            def vloop(h0, h1, tr, emb, st, p0):
                def bd(h, c):
                    vside1(h, tr, emb, lambda j: st(p0 + (h - h0) * emb + j))
                    return c
                lax.fori_loop(h0, h1, bd, 0)
                return p0 + (h1 - h0) * emb

            x = jnp.broadcast_to(xbuf[1:2, :].astype(F32), (8, D))
            compute_q(x)
            hi_wait[0].wait()
            cps_lb[0].wait()
            kloop(0, 3, lambda p: hi_b(0, NK0, p), 2 * EMB0 + Hkv * EMB2)
            kloop(3, 4, stv, 0)
            hi_wait[1].wait()
            cps_lb[1].wait()
            kloop(4, 8, stv, EMBK)
            c0 = jnp.mean(x, axis=-1, keepdims=True)
            c_scr[...] = jnp.broadcast_to(c0, (8, Dh))
            acc_scr[...] = jnp.where(rowg == 0, x - c0, 0.0)
            assert vpu_p == list(range(6))
            idle_loop(IDLE_E[0], GAPE, lambda i: stv(5 * EMBK + i))
            hi_wait[2].wait()
            cps_lb[2].wait()
            ne = vloop(0, 4, True, EMBV, stv, NV0)
            idle_loop(IDLE_E[1], GAPE, lambda i: stv(ne + i))
            hi_wait[3].wait()
            cps_lb[3].wait()
            vloop(4, 6, True, 0, None, 0)
            cps_lb[4].wait()
            vloop(6, 7, False, 0, None, 0)
            v7 = kv1[1, HL, 0:R7, :]
            vpk[HL, 0:R7 // 2, :] = pltpu.bitcast(v7, U32)
            o_scr[...] = jnp.dot(p_scr[HL, :, 0:R7], v7, preferred_element_type=F32)
            for i in range(NL - 1):
                cps_l[i].wait()
                o_scr[...] += pv_last(i)
            cps_l[NL - 1].wait()
            o = o_scr[...] + pv_last(NL - 1)

            zero_i = z_scr[...]

            def mk_tok(v):
                return lax.bitcast_convert_type(lax.bitcast_convert_type(v, jnp.int32) & zero_i, F32)

            def sum_all(vs):
                t = vs[0]
                for v in vs[1:]:
                    t = t + v
                return t

            def blocks(a):
                return [a[:, c * Dh:(c + 1) * Dh] for c in range(a.shape[1] // Dh)]

            def halves(a):
                return [a[0:8, :], a[8:16, :]]

            def stats(x):
                s1 = sum_all(blocks(x))
                s2 = sum_all(blocks(x * x))
                m = jnp.sum(s1, axis=-1, keepdims=True) * (1.0 / D)
                m2 = jnp.sum(s2, axis=-1, keepdims=True) * (1.0 / D)
                v = jnp.maximum(m2 - m * m, 0.0)
                return m, lax.rsqrt(v + eps), mk_tok(s1 + s2)

            def silu_half(a):
                return a + a * jnp.tanh(a)

            tile_cache = {}

            def tile_rows(tok, n):
                if (id(tok), n) not in tile_cache:
                    tile_cache[(id(tok), n)] = (tok, jnp.concatenate([tok] * n, axis=0))
                return tile_cache[(id(tok), n)][1]

            class MatVec:
                def __init__(self, xb_ref, slot, w_ref, row0, col0, nkb=NKB):
                    self.xb_ref, self.slot, self.w_ref, self.row0, self.col0 = xb_ref, slot, w_ref, row0, col0
                    self.acc = None
                    self.kb = 0
                    self.nkb = nkb

                def step(self, n, tok):
                    xv = self.xb_ref[self.slot, self.kb * 8:(self.kb + n) * 8, :]
                    if tok is not None:
                        xv = xv + tile_rows(tok, n)
                    self.fma(self.kb, xv)
                    self.kb += n

                def fma(self, kb, xv):
                    r0, n = self.row0 + kb * 8, xv.shape[0]
                    t = jnp.concatenate([xv] * rep, axis=1) * self.w_ref[r0:r0 + n, self.col0:self.col0 + G]
                    for i in range(0, n, 8):
                        ti = t[i:i + 8, :] if n > 8 else t
                        self.acc = ti if self.acc is None else self.acc + ti

            def ffn_fast(x):
                m, r, _ = stats(x)
                rh = 0.5 * r
                y = jnp.dot(x.astype(BF16), pltpu.bitcast(w1p[...], BF16), preferred_element_type=F32)
                h1 = silu_half((y - m * c1[...]) * rh)
                out = sum_all([
                    jnp.dot(h1[:, k0:k0 + Dh].astype(BF16),
                            pltpu.bitcast(w2p[(k0 - N2 * Dh) // 2:(k0 - N2 * Dh + Dh) // 2, :], BF16),
                            preferred_element_type=F32)
                    for k0 in range(N2 * Dh, FM, Dh)])
                ta = MatVec(None, 0, w2g, 0, 0)
                for kb in range(NF * 16):
                    yc = lanesum(sum_all(blocks(w1t[kb * 8:kb * 8 + 8, :] * x)))
                    ta.fma(kb, silu_half(yc * rh))
                for c in range(N2):
                    hb_scr[0, c * Dh:(c + 1) * Dh, :] = col_bcast(h1[0:1, c * Dh:(c + 1) * Dh])
                tb = MatVec(hb_scr, 0, w2f, 0, 0, nkb=N2 * 16)
                while tb.kb < tb.nkb:
                    tb.step(4, None)
                return m, out + rowsum(ta.acc + tb.acc)

            x = rowsum(acc_scr[...] + out_proj_fast(o * l_scr[HL], HL))
            m1, y1 = ffn_fast(x)
            x = (x - m1) + y1

            m, r, stok = stats(x)
            rs = r * (scale * LOG2E)

            def fin_q(qa, g):
                return pick_rows((qa - m * cq[:, g * G:(g + 1) * G]) * rs)
            x16 = x.astype(BF16)
            for c, xr in enumerate(blocks(x)):
                if c == D // Dh - 1:
                    xr = xr + stok
                xb_scr[0, c * Dh:(c + 1) * Dh, :] = col_bcast(xr[0:1, :])

            qs, os_, linv_, mx_ = {}, {}, {}, {}
            state = {"acc": jnp.where(rowg == 0, x - m, 0.0)}
            shift = c_scr[:, 0:1] + m1 + m
            live, fin = [None], []
            chunk_no = [0]
            k_at, os_at, e_at = {}, {}, {}
            todo = list(QUEUE)
            stack, etasks, due = [], [], []
            credit = [0.0]
            e_started, ep_ok = set(), set()
            last_tok = [None]

            def matvec_gen(mv):
                while mv.kb < NKB:
                    tok = yield 36
                    mv.step(4, tok)
                    live[0] = mv

            def q_gen(g):
                mv = MatVec(xb_scr, 0, wqf, 0, g * G - Q0)
                yield from matvec_gen(mv)
                qs[g] = fin_q(rowsum(mv.acc), g)
                return mk_tok(qs[g])

            def e_gen(g):
                m_ = jnp.broadcast_to(jnp.max(mx_[g], axis=1, keepdims=True), (8, Dh))
                m_ = jnp.maximum(m_, pltpu.roll(m_, 4, 0))
                lp = None
                order_ = list(range(NBLK))
                if g in vpu_p:
                    order_ = order_[NBLK - NVP:] + order_[:NBLK - NVP]
                for u in range(0, NBLK, EUNIT):
                    tok = yield ECOST * EUNIT
                    mm = m_ if tok is None else m_ + tok
                    for c in order_[u:u + EUNIT]:
                        pc = jnp.exp2(pf_scr[g, :, c * Dh:(c + 1) * Dh] - mm)
                        pf_scr[g, :, c * Dh:(c + 1) * Dh] = pc
                        lp = pc if lp is None else lp + pc
                    fin.append(lp)
                    if g in vpu_p and u + EUNIT >= NVP:
                        ep_ok.add(g)
                lp = lp + pltpu.roll(lp, 4, 0)
                linv_[g] = jnp.broadcast_to(1.0 / jnp.sum(lp, axis=1, keepdims=True), (8, Dh))
                e_at[g] = chunk_no[0]

            def p_gen(g):
                slot = g % 3
                for dg in range(Dh // 16):
                    accs = [None] * rep
                    for blk in range(NVP):
                        for hf in range(2):
                            tok = yield 20
                            col = (hf * NVP + blk) * Dh
                            vt = vtf[g, dg * 16:dg * 16 + 16, col:col + Dh]
                            if tok is not None:
                                vt = vt + tile_rows(tok, 2)
                            for j in range(rep):
                                r_ = hf * 4 + j
                                t = pf_scr[g, r_:r_ + 1, VP0 + blk * Dh:VP0 + (blk + 1) * Dh] * vt
                                accs[j] = t if accs[j] is None else accs[j] + t
                            live[0] = list(accs)
                    for j in range(rep):
                        pa_scr[slot, j * Dh + dg * 16:j * Dh + dg * 16 + 16, :] = accs[j]
                    fin.extend(halves(sum_all(accs)))
                    live[0] = None

            def o_gen(g):
                slot = g % 2
                linv = linv_[g]
                for j in range(rep):
                    tok = yield 48
                    orow = os_[g] if tok is None else os_[g] + tok
                    z = jnp.where(eye, jnp.broadcast_to(orow[j:j + 1, :], (Dh, Dh)), 0.0)
                    if g in vpu_p:
                        z = z + pa_scr[g % 3, j * Dh:(j + 1) * Dh, :]
                    ob_scr[slot, j * Dh:(j + 1) * Dh, :] = lanesum(z) * jnp.broadcast_to(linv[j:j + 1, :], (Dh, Dh))
                mv = MatVec(ob_scr, slot, wof, g * G, 0)
                yield from matvec_gen(mv)
                state["acc"] = state["acc"] + mv.acc
                return mk_tok(sum_all(blocks(mv.acc)))

            def ready(t):
                k_, g_ = t[0], int(t[1])
                if k_ == "p":
                    return g_ in ep_ok
                if k_ == "o":
                    return g_ in os_ and chunk_no[0] >= os_at[g_] + OLAG
                return True

            def run_vpu(tok, budget, force_e=None, flush=False):
                live[0] = None
                for g_, a_ in k_at.items():
                    if g_ not in e_started and (chunk_no[0] >= a_ + ELAG or g_ == force_e):
                        e_started.add(g_)
                        gen = e_gen(g_)
                        etasks.append([gen, next(gen)])
                credit[0] = 1e12 if flush else min(credit[0] + budget, 2 * RATE)
                while etasks:
                    credit[0] -= etasks[0][1]
                    try:
                        etasks[0][1] = etasks[0][0].send(tok)
                    except StopIteration:
                        etasks.pop(0)
                    if not flush:
                        break
                while True:
                    if not stack:
                        if not todo or (not flush and not ready(todo[0])):
                            break
                        t = todo.pop(0)
                        gen = {"q": q_gen, "p": p_gen, "o": o_gen}[t[0]](int(t[1]))
                        stack.append([gen, next(gen)])
                    cur = stack[-1]
                    if credit[0] < cur[1]:
                        break
                    credit[0] -= cur[1]
                    try:
                        cur[1] = cur[0].send(tok)
                    except StopIteration as e:
                        if e.value is not None:
                            due.append((chunk_no[0] + LAG, e.value))
                        live[0] = None
                        stack.pop()
                cov = list(fin)
                if isinstance(live[0], MatVec):
                    cov += blocks(live[0].acc)
                elif live[0]:
                    cov += halves(sum_all(live[0]))
                del fin[:]
                if cov and not flush:
                    due.append((chunk_no[0] + LAG, mk_tok(sum_all(cov))))

            def take_due():
                toks = [t for c_, t in due if c_ <= chunk_no[0]]
                due[:] = [(c_, t) for c_, t in due if c_ > chunk_no[0]]
                return sum_all(toks) if toks else None

            def qk2(g):
                while g not in qs:
                    run_vpu(last_tok[0], RATE)
                qq = qs[g]
                mx = None
                n = CB * Dh
                for c0 in range(0, NBLK, CB):
                    dtok = take_due()
                    if c0 == 0 or dtok is not None:
                        if dtok is not None:
                            qq = qq + dtok
                        qa = qq.astype(BF16)
                        qb = pltpu.roll(qq, 4, 0).astype(BF16)
                    sc = (jnp.dot(qa, load_kt(g, c0 * Dh, n), preferred_element_type=F32)
                          + jnp.dot(qb, load_kt(g, SW + c0 * Dh, n), preferred_element_type=F32))
                    pf_scr[g, :, c0 * Dh:c0 * Dh + n] = sc
                    for v in blocks(sc):
                        mx = v if mx is None else jnp.maximum(mx, v)
                    chunk_no[0] += 1
                    last_tok[0] = mk_tok(sc[:, 0:Dh])
                    run_vpu(last_tok[0], RATE)
                mx_[g] = mx

            def pv2(g):
                while g not in e_at:
                    run_vpu(last_tok[0], RATE, force_e=g)
                nb = NBLK - (NVP if g in vpu_p else 0)
                o1 = None
                o2 = None
                n = CB * Dh
                for c0 in range(0, nb, CB):
                    pc = pf_scr[g, :, c0 * Dh:c0 * Dh + n]
                    dtok = take_due()
                    if dtok is not None:
                        pc = jnp.concatenate([pc[:, 0:Dh] + dtok, pc[:, Dh:]], axis=1)
                    pc = pc.astype(BF16)
                    oc = jnp.dot(pc, load_v(g, c0 * Dh, n), preferred_element_type=F32)
                    o1 = oc if o1 is None else o1 + oc
                    oc2 = jnp.dot(pc, load_v(g, SW + c0 * Dh, n), preferred_element_type=F32)
                    o2 = oc2 if o2 is None else o2 + oc2
                    chunk_no[0] += 1
                    last_tok[0] = mk_tok(oc)
                    run_vpu(last_tok[0], RATE)
                return o1 + pltpu.roll(o2, 4, 0)

            for g in mxu_q:
                qs[g] = fin_q(jnp.dot(x16, pltpu.bitcast(wqp[mxu_q.index(g)], BF16), preferred_element_type=F32), g)
            for _ in range(PRE):
                run_vpu(None, RATE)
            pending_o = []
            for ph in ORDER:
                kind, g = ph[0], int(ph[1])
                if kind == "K":
                    qk2(g)
                    k_at[g] = chunk_no[0]
                else:
                    os_[g] = pv2(g)
                    os_at[g] = chunk_no[0]
                for og in pending_o:
                    state["acc"] = state["acc"] + out_proj_fast(os_[og] * linv_[og], og)
                pending_o = [g] if (kind == "V" and g in mxu_o) else []
            run_vpu(last_tok[0], 0, flush=True)
            for og in pending_o:
                state["acc"] = state["acc"] + out_proj_fast(os_[og] * linv_[og], og)
            x = rowsum(state["acc"])
            x = (x + shift) + ffn_fast(x)[1]
            o_ref[1:2, :] = x[0:1, :].astype(o_ref.dtype)

        pl.run_scoped(
            part_b,
            pltpu.VMEM((Hkv, Dh // 2, S), U32),
            pltpu.VMEM((Hkv, S // 2, Dh), U32),
            pltpu.VMEM((len(vpu_p), Dh, 2 * NVP * Dh), F32),
        )

    def kernel(*refs):
        pl.run_scoped(lambda sems: body(*refs, sems), pltpu.SemaphoreType.DMA((NSEM,)))

    assert NBLK % CB == 0 and (NBLK - NVP) % CB == 0 and CB >= 2
    out = pl.pallas_call(
        kernel,
        out_shape=jax.ShapeDtypeStruct((B, D), A_x.dtype),
        in_specs=[pl.BlockSpec(memory_space=pl.ANY)] * 7,
        out_specs=pl.BlockSpec(memory_space=pltpu.VMEM),
        scratch_shapes=[
            pltpu.VMEM((B, D), BF16),
            pltpu.VMEM((2, Hkv, S + 16, Dh), BF16),
            pltpu.VMEM((D, Hq * Dh), BF16),
            pltpu.VMEM((Hq * Dh, D), BF16),
            pltpu.VMEM((D, Fdim), BF16),
            pltpu.VMEM((Fdim, D), BF16),
            pltpu.VMEM((D, Hq * Dh - Q0), F32),
            pltpu.VMEM((len(vpu_o) * G, D), F32),
            pltpu.VMEM((N2 * Dh, D), F32),
            pltpu.VMEM((NF * Dh, D), F32),
            pltpu.VMEM((NF * Dh, D), F32),
            pltpu.VMEM((len(mxu_q), D // 2, G), U32),
            pltpu.VMEM((len(mxu_o), G // 2, D), U32),
            pltpu.VMEM((D // 2, FM), U32),
            pltpu.VMEM(((FM - N2 * Dh) // 2, D), U32),
            pltpu.VMEM((8, Hq * Dh), F32),
            pltpu.VMEM((8, FM), F32),
            pltpu.VMEM((8, Dh), F32),
            pltpu.VMEM((8, D), F32),
            pltpu.VMEM((Hkv, 8, S), BF16),
            pltpu.VMEM((Hkv, 8, Dh), F32),
            pltpu.VMEM((8, Dh), F32),
            pltpu.VMEM((8, Dh), F32),
            pltpu.VMEM((1, D, Dh), F32),
            pltpu.VMEM((1, N2 * Dh, Dh), F32),
            pltpu.VMEM((2, G, Dh), F32),
            pltpu.VMEM((Hkv, 8, SW), F32),
            pltpu.VMEM((3, G, Dh), F32),
            pltpu.VMEM((8, Dh), jnp.int32),
        ],
        compiler_params=pltpu.CompilerParams(vmem_limit_bytes=120 * 1024 * 1024, disable_bounds_checks=True),
    )(A_x.reshape(B, D), A_k_cache, A_v_cache, A_wq, A_wo, B_w1, B_w2)
    return out.reshape(B, Sq, D)
```

```python
import jax
import jax.numpy as jnp
from jax import lax
import jax.experimental.pallas as pl
import jax.experimental.pallas.tpu as pltpu

F32 = jnp.float32
BF16 = jnp.bfloat16
U32 = jnp.uint32
NT = (((1,), (1,)), ((), ()))
LOG2E = 1.4426950408889634

HRB = 32
GAP = 22
NA = (200, 190, 200, 200)
IDLE_A = (250, 30, 140)
EMBQ = 12
EMB2 = 18
EMBK = 20
EMBV = 8
NK0 = 64
IDLE_E = (28, 48)
GAPE = 24
LAST_TWO = (1536, 512)

ORDER = "K0 K1 K2 K3 V0 K4 V1 K5 V2 K6 V3 K7 V4 V5 V6 V7".split()
QUEUE = "q2 q3 q4 q5 q6 q7 p0 p1 p2 o0 p3 o1 p4 o2 p5 o3 o4 o5".split()
NVP = 8
CB = 2
RATE = 102.3
LAG = 8
ELAG = 7
EUNIT = 4
ECOST = 5
OLAG = 6
PRE = 8
N2 = 2
NF = 6


@jax.jit
def pallas_interleave_layers__gqa_block_cached__dense_activation_silu__decode_kernel(
    A_x: jax.Array,
    A_k_cache: jax.Array,
    A_v_cache: jax.Array,
    A_wq: jax.Array,
    A_wo: jax.Array,
    B_x: jax.Array,
    B_w1: jax.Array,
    B_w2: jax.Array,
):
    B, Sq, D = A_x.shape
    _, Hkv, S, Dh = A_k_cache.shape
    Hq = A_wq.shape[1] // Dh
    rep = Hq // Hkv
    Fdim = B_w1.shape[1]
    assert (B, Sq, rep, Dh, Hkv) == (2, 1, 4, 128, 8) and D == rep * Dh
    G = rep * Dh
    scale = Dh ** -0.5
    eps = 1e-5
    NK1 = 4 * EMBV + Hkv * EMB2 + 3 * EMBK - NK0
    NV0 = 5 * EMBK + IDLE_E[0]
    NV1 = 4 * EMBV + IDLE_E[1]
    assert NK0 <= 4 * EMBV + Hkv * EMB2 and max(NK0, NK1, NV0, *NA) * HRB < S
    R7 = NV1 * HRB
    LAST_CHUNKS = (S - R7 - sum(LAST_TWO),) + LAST_TWO
    assert LAST_CHUNKS[0] > 0 and R7 % Dh == 0
    NL = len(LAST_CHUNKS)
    lc_off = [R7 + sum(LAST_CHUNKS[:i]) for i in range(NL)]
    SEM_W = 0
    SEM_HA = 5
    SEM_LA = 9
    SEM_HB = 13
    SEM_LB = 17
    SEM_L = 22
    NSEM = SEM_L + NL
    HL = Hkv - 1
    vpu_q = [g for g in range(Hkv) if "q%d" % g in QUEUE]
    vpu_o = [g for g in range(Hkv) if "o%d" % g in QUEUE]
    vpu_p = [g for g in range(Hkv) if "p%d" % g in QUEUE]
    mxu_q = [g for g in range(Hkv) if g not in vpu_q]
    mxu_o = [g for g in range(Hkv) if g not in vpu_o]
    assert vpu_q == list(range(vpu_q[0], Hkv)) and vpu_o == list(range(len(vpu_o)))
    assert vpu_p == list(range(len(vpu_p))) and set(vpu_p) <= set(vpu_o) and HL in mxu_o
    Q0 = vpu_q[0] * G
    SW = S // 2
    NBLK = SW // Dh
    VP0 = SW - NVP * Dh
    NKB = D // 8
    FM = Fdim - NF * Dh

    def body(x_hbm, k_hbm, v_hbm, wq_hbm, wo_hbm, w1_hbm, w2_hbm, o_ref,
             xbuf, kv1, wq, wo, w1, w2, wqf, wof, w2f, w1t, w2g,
             wqp, wop, w1p, w2p, cq, c1, d_scr, acc_scr, p_scr, l_scr, o_scr, c_scr,
             xb_scr, hb_scr, ob_scr, pf_scr, pa_scr, z_scr, sems):
        hbm = (k_hbm, v_hbm)

        def cp_big(buf, t, b, h0, nh, sem, r0=0, r1=S):
            hs, rs_ = pl.ds(h0, nh), pl.ds(r0, r1 - r0)
            return pltpu.make_async_copy(hbm[t].at[b, hs, rs_], buf.at[t, hs, rs_], sems.at[sem])

        def hi_slot(buf, b, sem0, t, n0, p):
            hq = (p >= n0).astype(jnp.int32) if not isinstance(p, int) else int(p >= n0)
            hs, rs_ = pl.ds(4 * hq, 4), pl.ds(pl.multiple_of((p - n0 * hq) * HRB, HRB), HRB)
            pltpu.make_async_copy(hbm[t].at[b, hs, rs_], buf.at[t, hs, rs_],
                                  sems.at[sem0 + 2 * t + hq]).start(priority=0)

        def hi_b(t, n0, p):
            hi_slot(kv1, 1, SEM_HB, t, n0, p)

        def cp_vl(i):
            sl = pl.ds(lc_off[i], LAST_CHUNKS[i])
            return pltpu.make_async_copy(v_hbm.at[1, HL, sl], kv1.at[1, HL, sl], sems.at[SEM_L + i])

        cps_w = [pltpu.make_async_copy(s_, d_, sems.at[SEM_W + i]) for i, (s_, d_) in enumerate(
            ((x_hbm, xbuf), (wq_hbm, wq), (wo_hbm, wo), (w1_hbm, w1), (w2_hbm, w2)))]
        nhi = (NK0, NK1, NV0, NV1)
        hi_wait = [cp_big(kv1, i // 2, 1, 4 * (i % 2), 4, SEM_HB + i, 0, nhi[i] * HRB) for i in range(4)]
        cps_lb = [cp_big(kv1, i // 2, 1, 4 * (i % 2), 4, SEM_LB + i, nhi[i] * HRB) for i in range(3)]
        cps_lb += [cp_big(kv1, 1, 1, 4, 2, SEM_LB + 3, R7), cp_big(kv1, 1, 1, 6, 1, SEM_LB + 4, R7)]

        def idle_loop(n, gap, start):
            def it(i, y):
                start(i)
                for _ in range(gap):
                    y = y * 0.5 + 1.0
                return y
            if n > 0:
                d_scr[...] = lax.fori_loop(0, n, it, d_scr[...])
        cps_l = [cp_vl(i) for i in range(NL)]
        cps_w[0].start(priority=1)
        cps_w[1].start(priority=1)

        row8 = lax.broadcasted_iota(jnp.int32, (8, Dh), 0)
        rowg = lax.broadcasted_iota(jnp.int32, (8, G), 0)
        colg = lax.broadcasted_iota(jnp.int32, (8, G), 1)
        diag_mask = rowg == (colg // Dh)
        eye = (lax.broadcasted_iota(jnp.int32, (Dh, Dh), 0) == lax.broadcasted_iota(jnp.int32, (Dh, Dh), 1))

        def pick_rows(qa):
            qg = jnp.zeros((8, Dh), F32)
            for j in range(rep):
                qg = jnp.where(row8 == j, qa[:, j * Dh:(j + 1) * Dh], qg)
            return qg

        def diag_lhs(o):
            o4 = jnp.concatenate([o] * rep, axis=1)
            return jnp.where(diag_mask, o4, 0.0).astype(BF16)

        def out_proj_fast(o, g):
            return jnp.dot(diag_lhs(o), pltpu.bitcast(wop[mxu_o.index(g)], BF16), preferred_element_type=F32)

        def rowsum(a):
            return jnp.broadcast_to(jnp.sum(a, axis=0, keepdims=True), a.shape)

        def lanesum(a):
            return jnp.broadcast_to(jnp.sum(a, axis=1, keepdims=True), (a.shape[0], Dh))

        def col_bcast(row):
            return lanesum(jnp.where(eye, jnp.broadcast_to(row, (Dh, Dh)), 0.0))

        def layernorm(x):
            xc = x - jnp.mean(x, axis=-1, keepdims=True)
            return xc * lax.rsqrt(jnp.mean(xc * xc, axis=-1, keepdims=True) + eps)

        def compute_q(x):
            xn = layernorm(x).astype(BF16)
            for g in range(Hkv):
                qa = jnp.dot(xn, wq[:, g * G:(g + 1) * G], preferred_element_type=F32) * scale
                kv1[0, g, S:S + 8, :] = pick_rows(qa).astype(BF16)

        def softmax_parts(s):
            p = jnp.exp(s - jnp.max(s, axis=1, keepdims=True))
            return p.astype(BF16), jnp.sum(p, axis=1, keepdims=True)

        def out_proj(o, h):
            w = wo[pl.ds(pl.multiple_of(h * G, G), G), :]
            return jnp.dot(diag_lhs(o), w, preferred_element_type=F32)

        def ffn(x):
            hh = jnp.dot(layernorm(x).astype(BF16), w1[...], preferred_element_type=F32)
            hh = hh * jax.nn.sigmoid(hh)
            return jnp.dot(hh.astype(BF16), w2[...], preferred_element_type=F32)

        def part_a(kv0):
            ha_wait = [cp_big(kv0, i // 2, 0, 4 * (i % 2), 4, SEM_HA + i, 0, NA[i] * HRB) for i in range(4)]
            cps_la = [cp_big(kv0, i // 2, 0, 4 * (i % 2), 4, SEM_LA + i, NA[i] * HRB) for i in range(4)]
            for c in ([cps_la[0], cps_la[1], cps_w[2], cps_la[2], cps_w[3], cps_w[4], cps_la[3]]
                      + cps_lb + cps_l):
                c.start(priority=1)
            issued = [0, 0]

            def take_a(t, n):
                assert issued[t] + n <= NA[2 * t] + NA[2 * t + 1], (t, issued, n)
                p0 = issued[t]
                issued[t] += n
                return lambda q: hi_slot(kv0, 0, SEM_HA, t, NA[2 * t], p0 + q)

            def idle_a(t, n):
                n = max(min(n, NA[2 * t] + NA[2 * t + 1] - issued[t]), 0)
                idle_loop(n, GAP, take_a(t, n))

            def k0loop(h0, h1):
                st = take_a(1, (h1 - h0) * EMBQ)

                def bd(h, c):
                    ss = []
                    for u in range(EMBQ):
                        r0, r1 = (u * (S // Dh) // EMBQ) * Dh, ((u + 1) * (S // Dh) // EMBQ) * Dh
                        ss.append(lax.dot_general(kv1[0, h, S:S + 8, :], kv0[0, h, r0:r1, :], NT,
                                                  preferred_element_type=F32))
                        st((h - h0) * EMBQ + u)
                    p, l = softmax_parts(jnp.concatenate(ss, axis=1))
                    p_scr[h] = p
                    l_scr[h] = jnp.broadcast_to(1.0 / l, (8, Dh))
                    return c
                lax.fori_loop(h0, h1, bd, 0)

            def v0loop(h0, h1, st):
                def bd(h, c):
                    o = None
                    for u in range(EMBV):
                        r0, r1 = (u * (S // Dh) // EMBV) * Dh, ((u + 1) * (S // Dh) // EMBV) * Dh
                        pc = p_scr[h, :, r0:r1]
                        pc = jnp.concatenate([pc[:, 0:Dh] + kv1[1, h, S:S + 8, :], pc[:, Dh:]], axis=1)
                        oc = jnp.dot(pc, kv0[1, h, r0:r1, :], preferred_element_type=F32)
                        o = oc if o is None else o + oc
                        st((h - h0) * EMBV + u)
                    acc_scr[...] += out_proj(o * l_scr[h], h)
                    return c
                lax.fori_loop(h0, h1, bd, 0)

            def attn_head0(h, emb, start):
                nq = (2 * emb + 2) // 3 if emb else 1
                nv = emb - nq if emb else 1
                ss = []
                for c in range(nq):
                    r0, r1 = (c * (S // Dh) // nq) * Dh, ((c + 1) * (S // Dh) // nq) * Dh
                    ss.append(lax.dot_general(kv1[0, h, S:S + 8, :], kv0[0, h, r0:r1, :], NT,
                                              preferred_element_type=F32))
                    if emb:
                        start(c)
                p, l = softmax_parts(jnp.concatenate(ss, axis=1))
                o = None
                for c in range(nv):
                    r0, r1 = (c * (S // Dh) // nv) * Dh, ((c + 1) * (S // Dh) // nv) * Dh
                    pc = p[:, r0:r1]
                    if emb:
                        z = kv1[1, h, S:S + 8, :]
                        pc = jnp.concatenate([pc[:, 0:Dh] + z, pc[:, Dh:]], axis=1)
                    oc = jnp.dot(pc, kv0[1, h, r0:r1, :], preferred_element_type=F32)
                    o = oc if o is None else o + oc
                    if emb:
                        start(nq + c)
                acc_scr[...] += out_proj(o / l, h)

            d_scr[...] = jnp.zeros_like(d_scr)
            for h in range(Hkv):
                kv1[1, h, S:S + 16, :] = jnp.zeros((16, Dh), BF16)
            z_scr[...] = jnp.zeros_like(z_scr)
            acc_scr[...] = jnp.zeros_like(acc_scr)
            ones8 = jnp.ones((8, D), BF16)

            idle_a(0, IDLE_A[0])
            cps_w[0].wait()
            cps_w[1].wait()
            st_q = take_a(0, D // 64)

            def prep_q(i, c):
                st_q(i)
                off = pl.multiple_of(i * 64, 64)
                wqf[pl.ds(off, 64), :] = wq[pl.ds(off, 64), Q0:].astype(F32)
                return c
            lax.fori_loop(0, D // 64, prep_q, 0)
            for i, g in enumerate(mxu_q):
                wqp[i] = pltpu.bitcast(wq[:, g * G:(g + 1) * G], U32)
            cq[...] = jnp.dot(ones8, wq[...], preferred_element_type=F32)
            x = jnp.broadcast_to(xbuf[0:1, :].astype(F32), (8, D))
            compute_q(x)

            idle_a(0, S)
            for i in range(2):
                ha_wait[i].wait()
                cps_la[i].wait()
                k0loop(4 * i, 4 * i + 4)
            idle_a(1, IDLE_A[1])
            cps_w[2].wait()
            st_o = take_a(1, len(vpu_o))

            def prep_o(i, c):
                st_o(i)
                off = pl.multiple_of(i * G, G)
                wof[pl.ds(off, G), :] = wo[pl.ds(off, G), :].astype(F32)
                return c
            lax.fori_loop(0, len(vpu_o), prep_o, 0)
            for i, g in enumerate(mxu_o):
                wop[i] = pltpu.bitcast(wo[g * G:(g + 1) * G, :], U32)

            idle_a(1, NA[2] + 6 - issued[1])
            ha_wait[2].wait()
            cps_la[2].wait()
            v0loop(0, 4, take_a(1, 4 * EMBV))
            idle_a(1, IDLE_A[2])
            cps_w[3].wait()
            cps_w[4].wait()
            w1p[...] = pltpu.bitcast(w1[:, 0:FM], U32)
            w2p[...] = pltpu.bitcast(w2[N2 * Dh:FM, :], U32)
            w2f[...] = w2[0:N2 * Dh, :].astype(F32)
            w1t[...] = w1[:, FM:].astype(F32).T
            w2g[...] = w2[FM:, :].astype(F32)
            w1t[...] = w1t[...] - jnp.mean(w1t[...], axis=1, keepdims=True)
            c1[...] = jnp.dot(ones8, w1[:, 0:FM], preferred_element_type=F32)
            idle_a(1, S)
            ha_wait[3].wait()
            cps_la[3].wait()
            v0loop(4, 8, lambda q: hi_b(0, NK0, q))
            x = x + rowsum(acc_scr[...])
            x = x + ffn(x)
            compute_q(x)
            acc_scr[...] = jnp.zeros_like(acc_scr)

            def body2(h, c):
                attn_head0(h, EMB2, lambda j: hi_b(0, NK0, 4 * EMBV + h * EMB2 + j))
                return c
            lax.fori_loop(0, Hkv, body2, 0)
            x = x + rowsum(acc_scr[...])
            x = x + ffn(x)
            o_ref[0:1, :] = x[0:1, :].astype(o_ref.dtype)

        pl.run_scoped(part_a, pltpu.VMEM((2, Hkv, S, Dh), BF16))

        def part_b(ktbuf, vpk, vtf):
            def load_v(h, off, n):
                return pltpu.bitcast(vpk[h, off // 2:(off + n) // 2, :], BF16)

            def load_kt(h, off, n):
                return pltpu.bitcast(ktbuf[h, :, off:off + n], BF16)

            def pv_last(i):
                o_, n = lc_off[i], LAST_CHUNKS[i]
                v = kv1[1, HL, o_:o_ + n, :]
                vpk[HL, o_ // 2:(o_ + n) // 2, :] = pltpu.bitcast(v, U32)
                return jnp.dot(p_scr[HL, :, o_:o_ + n], v, preferred_element_type=F32)

            def kside1(h, st):
                ss = []
                for u in range(EMBK):
                    r0, r1 = (u * (S // Dh) // EMBK) * Dh, ((u + 1) * (S // Dh) // EMBK) * Dh
                    kt = kv1[0, h, r0:r1, :].T
                    ktbuf[h, :, r0:r1] = pltpu.bitcast(kt, U32)
                    ss.append(jnp.dot(kv1[0, h, S:S + 8, :], kt, preferred_element_type=F32))
                    st(u)
                p, l = softmax_parts(jnp.concatenate(ss, axis=1))
                p_scr[h] = p
                l_scr[h] = jnp.broadcast_to(1.0 / l, (8, Dh))

            def kloop(h0, h1, st, p0):
                def bd(h, c):
                    kside1(h, lambda j: st(p0 + (h - h0) * EMBK + j))
                    return c
                lax.fori_loop(h0, h1, bd, 0)

            def vside1(h, tr, emb, st):
                if tr:
                    for hf in range(2):
                        vtf[h, :, hf * NVP * Dh:(hf + 1) * NVP * Dh] = (
                            kv1[1, h, hf * SW + VP0:(hf + 1) * SW, :].astype(F32).T)
                o = None
                nv = max(emb, 1)
                for c in range(nv):
                    r0, r1 = (c * (S // Dh) // nv) * Dh, ((c + 1) * (S // Dh) // nv) * Dh
                    v = kv1[1, h, r0:r1, :]
                    vpk[h, r0 // 2:r1 // 2, :] = pltpu.bitcast(v, U32)
                    oc = jnp.dot(p_scr[h, :, r0:r1], v, preferred_element_type=F32)
                    o = oc if o is None else o + oc
                    if emb:
                        st(c)
                acc_scr[...] += out_proj(o * l_scr[h], h)

            def stv(p):
                hi_b(1, NV0, p)

            def vloop(h0, h1, tr, emb, st, p0):
                def bd(h, c):
                    vside1(h, tr, emb, lambda j: st(p0 + (h - h0) * emb + j))
                    return c
                lax.fori_loop(h0, h1, bd, 0)
                return p0 + (h1 - h0) * emb

            x = jnp.broadcast_to(xbuf[1:2, :].astype(F32), (8, D))
            compute_q(x)
            hi_wait[0].wait()
            cps_lb[0].wait()
            kloop(0, 3, lambda p: hi_b(0, NK0, p), 4 * EMBV + Hkv * EMB2)
            kloop(3, 4, stv, 0)
            hi_wait[1].wait()
            cps_lb[1].wait()
            kloop(4, 8, stv, EMBK)
            c0 = jnp.mean(x, axis=-1, keepdims=True)
            c_scr[...] = jnp.broadcast_to(c0, (8, Dh))
            acc_scr[...] = jnp.where(rowg == 0, x - c0, 0.0)
            assert vpu_p == list(range(6))
            idle_loop(IDLE_E[0], GAPE, lambda i: stv(5 * EMBK + i))
            hi_wait[2].wait()
            cps_lb[2].wait()
            ne = vloop(0, 4, True, EMBV, stv, NV0)
            idle_loop(IDLE_E[1], GAPE, lambda i: stv(ne + i))
            hi_wait[3].wait()
            cps_lb[3].wait()
            vloop(4, 6, True, 0, None, 0)
            cps_lb[4].wait()
            vloop(6, 7, False, 0, None, 0)
            v7 = kv1[1, HL, 0:R7, :]
            vpk[HL, 0:R7 // 2, :] = pltpu.bitcast(v7, U32)
            o_scr[...] = jnp.dot(p_scr[HL, :, 0:R7], v7, preferred_element_type=F32)
            for i in range(NL - 1):
                cps_l[i].wait()
                o_scr[...] += pv_last(i)
            cps_l[NL - 1].wait()
            o = o_scr[...] + pv_last(NL - 1)

            zero_i = z_scr[...]

            def mk_tok(v):
                return lax.bitcast_convert_type(lax.bitcast_convert_type(v, jnp.int32) & zero_i, F32)

            def sum_all(vs):
                t = vs[0]
                for v in vs[1:]:
                    t = t + v
                return t

            def blocks(a):
                return [a[:, c * Dh:(c + 1) * Dh] for c in range(a.shape[1] // Dh)]

            def halves(a):
                return [a[0:8, :], a[8:16, :]]

            def stats(x):
                s1 = sum_all(blocks(x))
                s2 = sum_all(blocks(x * x))
                m = jnp.sum(s1, axis=-1, keepdims=True) * (1.0 / D)
                m2 = jnp.sum(s2, axis=-1, keepdims=True) * (1.0 / D)
                v = jnp.maximum(m2 - m * m, 0.0)
                return m, lax.rsqrt(v + eps), mk_tok(s1 + s2)

            def silu_half(a):
                return a + a * jnp.tanh(a)

            tile_cache = {}

            def tile_rows(tok, n):
                if (id(tok), n) not in tile_cache:
                    tile_cache[(id(tok), n)] = (tok, jnp.concatenate([tok] * n, axis=0))
                return tile_cache[(id(tok), n)][1]

            class MatVec:
                def __init__(self, xb_ref, slot, w_ref, row0, col0, nkb=NKB):
                    self.xb_ref, self.slot, self.w_ref, self.row0, self.col0 = xb_ref, slot, w_ref, row0, col0
                    self.acc = None
                    self.kb = 0
                    self.nkb = nkb

                def step(self, n, tok):
                    xv = self.xb_ref[self.slot, self.kb * 8:(self.kb + n) * 8, :]
                    if tok is not None:
                        xv = xv + tile_rows(tok, n)
                    self.fma(self.kb, xv)
                    self.kb += n

                def fma(self, kb, xv):
                    r0, n = self.row0 + kb * 8, xv.shape[0]
                    t = jnp.concatenate([xv] * rep, axis=1) * self.w_ref[r0:r0 + n, self.col0:self.col0 + G]
                    for i in range(0, n, 8):
                        ti = t[i:i + 8, :] if n > 8 else t
                        self.acc = ti if self.acc is None else self.acc + ti

            def ffn_fast(x):
                m, r, _ = stats(x)
                rh = 0.5 * r
                y = jnp.dot(x.astype(BF16), pltpu.bitcast(w1p[...], BF16), preferred_element_type=F32)
                h1 = silu_half((y - m * c1[...]) * rh)
                out = sum_all([
                    jnp.dot(h1[:, k0:k0 + Dh].astype(BF16),
                            pltpu.bitcast(w2p[(k0 - N2 * Dh) // 2:(k0 - N2 * Dh + Dh) // 2, :], BF16),
                            preferred_element_type=F32)
                    for k0 in range(N2 * Dh, FM, Dh)])
                ta = MatVec(None, 0, w2g, 0, 0)
                for kb in range(NF * 16):
                    yc = lanesum(sum_all(blocks(w1t[kb * 8:kb * 8 + 8, :] * x)))
                    ta.fma(kb, silu_half(yc * rh))
                for c in range(N2):
                    hb_scr[0, c * Dh:(c + 1) * Dh, :] = col_bcast(h1[0:1, c * Dh:(c + 1) * Dh])
                tb = MatVec(hb_scr, 0, w2f, 0, 0, nkb=N2 * 16)
                while tb.kb < tb.nkb:
                    tb.step(4, None)
                return m, out + rowsum(ta.acc + tb.acc)

            x = rowsum(acc_scr[...] + out_proj_fast(o * l_scr[HL], HL))
            m1, y1 = ffn_fast(x)
            x = (x - m1) + y1

            m, r, stok = stats(x)
            rs = r * (scale * LOG2E)

            def fin_q(qa, g):
                return pick_rows((qa - m * cq[:, g * G:(g + 1) * G]) * rs)
            x16 = x.astype(BF16)
            for c, xr in enumerate(blocks(x)):
                if c == D // Dh - 1:
                    xr = xr + stok
                xb_scr[0, c * Dh:(c + 1) * Dh, :] = col_bcast(xr[0:1, :])

            qs, os_, linv_, mx_ = {}, {}, {}, {}
            state = {"acc": jnp.where(rowg == 0, x - m, 0.0)}
            shift = c_scr[:, 0:1] + m1 + m
            live, fin = [None], []
            chunk_no = [0]
            k_at, os_at, e_at = {}, {}, {}
            todo = list(QUEUE)
            stack, etasks, due = [], [], []
            credit = [0.0]
            e_started, ep_ok = set(), set()
            last_tok = [None]

            def matvec_gen(mv):
                while mv.kb < NKB:
                    tok = yield 36
                    mv.step(4, tok)
                    live[0] = mv

            def q_gen(g):
                mv = MatVec(xb_scr, 0, wqf, 0, g * G - Q0)
                yield from matvec_gen(mv)
                qs[g] = fin_q(rowsum(mv.acc), g)
                return mk_tok(qs[g])

            def e_gen(g):
                m_ = jnp.broadcast_to(jnp.max(mx_[g], axis=1, keepdims=True), (8, Dh))
                m_ = jnp.maximum(m_, pltpu.roll(m_, 4, 0))
                lp = None
                order_ = list(range(NBLK))
                if g in vpu_p:
                    order_ = order_[NBLK - NVP:] + order_[:NBLK - NVP]
                for u in range(0, NBLK, EUNIT):
                    tok = yield ECOST * EUNIT
                    mm = m_ if tok is None else m_ + tok
                    for c in order_[u:u + EUNIT]:
                        pc = jnp.exp2(pf_scr[g, :, c * Dh:(c + 1) * Dh] - mm)
                        pf_scr[g, :, c * Dh:(c + 1) * Dh] = pc
                        lp = pc if lp is None else lp + pc
                    fin.append(lp)
                    if g in vpu_p and u + EUNIT >= NVP:
                        ep_ok.add(g)
                lp = lp + pltpu.roll(lp, 4, 0)
                linv_[g] = jnp.broadcast_to(1.0 / jnp.sum(lp, axis=1, keepdims=True), (8, Dh))
                e_at[g] = chunk_no[0]

            def p_gen(g):
                slot = g % 3
                for dg in range(Dh // 16):
                    accs = [None] * rep
                    for blk in range(NVP):
                        for hf in range(2):
                            tok = yield 20
                            col = (hf * NVP + blk) * Dh
                            vt = vtf[g, dg * 16:dg * 16 + 16, col:col + Dh]
                            if tok is not None:
                                vt = vt + tile_rows(tok, 2)
                            for j in range(rep):
                                r_ = hf * 4 + j
                                t = pf_scr[g, r_:r_ + 1, VP0 + blk * Dh:VP0 + (blk + 1) * Dh] * vt
                                accs[j] = t if accs[j] is None else accs[j] + t
                            live[0] = list(accs)
                    for j in range(rep):
                        pa_scr[slot, j * Dh + dg * 16:j * Dh + dg * 16 + 16, :] = accs[j]
                    fin.extend(halves(sum_all(accs)))
                    live[0] = None

            def o_gen(g):
                slot = g % 2
                linv = linv_[g]
                for j in range(rep):
                    tok = yield 48
                    orow = os_[g] if tok is None else os_[g] + tok
                    z = jnp.where(eye, jnp.broadcast_to(orow[j:j + 1, :], (Dh, Dh)), 0.0)
                    if g in vpu_p:
                        z = z + pa_scr[g % 3, j * Dh:(j + 1) * Dh, :]
                    ob_scr[slot, j * Dh:(j + 1) * Dh, :] = lanesum(z) * jnp.broadcast_to(linv[j:j + 1, :], (Dh, Dh))
                mv = MatVec(ob_scr, slot, wof, g * G, 0)
                yield from matvec_gen(mv)
                state["acc"] = state["acc"] + mv.acc
                return mk_tok(sum_all(blocks(mv.acc)))

            def ready(t):
                k_, g_ = t[0], int(t[1])
                if k_ == "p":
                    return g_ in ep_ok
                if k_ == "o":
                    return g_ in os_ and chunk_no[0] >= os_at[g_] + OLAG
                return True

            def run_vpu(tok, budget, force_e=None, flush=False):
                live[0] = None
                for g_, a_ in k_at.items():
                    if g_ not in e_started and (chunk_no[0] >= a_ + ELAG or g_ == force_e):
                        e_started.add(g_)
                        gen = e_gen(g_)
                        etasks.append([gen, next(gen)])
                credit[0] = 1e12 if flush else min(credit[0] + budget, 2 * RATE)
                while etasks:
                    credit[0] -= etasks[0][1]
                    try:
                        etasks[0][1] = etasks[0][0].send(tok)
                    except StopIteration:
                        etasks.pop(0)
                    if not flush:
                        break
                while True:
                    if not stack:
                        if not todo or (not flush and not ready(todo[0])):
                            break
                        t = todo.pop(0)
                        gen = {"q": q_gen, "p": p_gen, "o": o_gen}[t[0]](int(t[1]))
                        stack.append([gen, next(gen)])
                    cur = stack[-1]
                    if credit[0] < cur[1]:
                        break
                    credit[0] -= cur[1]
                    try:
                        cur[1] = cur[0].send(tok)
                    except StopIteration as e:
                        if e.value is not None:
                            due.append((chunk_no[0] + LAG, e.value))
                        live[0] = None
                        stack.pop()
                cov = list(fin)
                if isinstance(live[0], MatVec):
                    cov += blocks(live[0].acc)
                elif live[0]:
                    cov += halves(sum_all(live[0]))
                del fin[:]
                if cov and not flush:
                    due.append((chunk_no[0] + LAG, mk_tok(sum_all(cov))))

            def take_due():
                toks = [t for c_, t in due if c_ <= chunk_no[0]]
                due[:] = [(c_, t) for c_, t in due if c_ > chunk_no[0]]
                return sum_all(toks) if toks else None

            def qk2(g):
                while g not in qs:
                    run_vpu(last_tok[0], RATE)
                qq = qs[g]
                mx = None
                n = CB * Dh
                for c0 in range(0, NBLK, CB):
                    dtok = take_due()
                    if c0 == 0 or dtok is not None:
                        if dtok is not None:
                            qq = qq + dtok
                        qa = qq.astype(BF16)
                        qb = pltpu.roll(qq, 4, 0).astype(BF16)
                    sc = (jnp.dot(qa, load_kt(g, c0 * Dh, n), preferred_element_type=F32)
                          + jnp.dot(qb, load_kt(g, SW + c0 * Dh, n), preferred_element_type=F32))
                    pf_scr[g, :, c0 * Dh:c0 * Dh + n] = sc
                    for v in blocks(sc):
                        mx = v if mx is None else jnp.maximum(mx, v)
                    chunk_no[0] += 1
                    last_tok[0] = mk_tok(sc[:, 0:Dh])
                    run_vpu(last_tok[0], RATE)
                mx_[g] = mx

            def pv2(g):
                while g not in e_at:
                    run_vpu(last_tok[0], RATE, force_e=g)
                nb = NBLK - (NVP if g in vpu_p else 0)
                o1 = None
                o2 = None
                n = CB * Dh
                for c0 in range(0, nb, CB):
                    pc = pf_scr[g, :, c0 * Dh:c0 * Dh + n]
                    dtok = take_due()
                    if dtok is not None:
                        pc = jnp.concatenate([pc[:, 0:Dh] + dtok, pc[:, Dh:]], axis=1)
                    pc = pc.astype(BF16)
                    oc = jnp.dot(pc, load_v(g, c0 * Dh, n), preferred_element_type=F32)
                    o1 = oc if o1 is None else o1 + oc
                    oc2 = jnp.dot(pc, load_v(g, SW + c0 * Dh, n), preferred_element_type=F32)
                    o2 = oc2 if o2 is None else o2 + oc2
                    chunk_no[0] += 1
                    last_tok[0] = mk_tok(oc)
                    run_vpu(last_tok[0], RATE)
                return o1 + pltpu.roll(o2, 4, 0)

            for g in mxu_q:
                qs[g] = fin_q(jnp.dot(x16, pltpu.bitcast(wqp[mxu_q.index(g)], BF16), preferred_element_type=F32), g)
            for _ in range(PRE):
                run_vpu(None, RATE)
            pending_o = []
            for ph in ORDER:
                kind, g = ph[0], int(ph[1])
                if kind == "K":
                    qk2(g)
                    k_at[g] = chunk_no[0]
                else:
                    os_[g] = pv2(g)
                    os_at[g] = chunk_no[0]
                for og in pending_o:
                    state["acc"] = state["acc"] + out_proj_fast(os_[og] * linv_[og], og)
                pending_o = [g] if (kind == "V" and g in mxu_o) else []
            run_vpu(last_tok[0], 0, flush=True)
            for og in pending_o:
                state["acc"] = state["acc"] + out_proj_fast(os_[og] * linv_[og], og)
            x = rowsum(state["acc"])
            x = (x + shift) + ffn_fast(x)[1]
            o_ref[1:2, :] = x[0:1, :].astype(o_ref.dtype)

        pl.run_scoped(
            part_b,
            pltpu.VMEM((Hkv, Dh // 2, S), U32),
            pltpu.VMEM((Hkv, S // 2, Dh), U32),
            pltpu.VMEM((len(vpu_p), Dh, 2 * NVP * Dh), F32),
        )

    def kernel(*refs):
        pl.run_scoped(lambda sems: body(*refs, sems), pltpu.SemaphoreType.DMA((NSEM,)))

    assert NBLK % CB == 0 and (NBLK - NVP) % CB == 0 and CB >= 2
    out = pl.pallas_call(
        kernel,
        out_shape=jax.ShapeDtypeStruct((B, D), A_x.dtype),
        in_specs=[pl.BlockSpec(memory_space=pl.ANY)] * 7,
        out_specs=pl.BlockSpec(memory_space=pltpu.VMEM),
        scratch_shapes=[
            pltpu.VMEM((B, D), BF16),
            pltpu.VMEM((2, Hkv, S + 16, Dh), BF16),
            pltpu.VMEM((D, Hq * Dh), BF16),
            pltpu.VMEM((Hq * Dh, D), BF16),
            pltpu.VMEM((D, Fdim), BF16),
            pltpu.VMEM((Fdim, D), BF16),
            pltpu.VMEM((D, Hq * Dh - Q0), F32),
            pltpu.VMEM((len(vpu_o) * G, D), F32),
            pltpu.VMEM((N2 * Dh, D), F32),
            pltpu.VMEM((NF * Dh, D), F32),
            pltpu.VMEM((NF * Dh, D), F32),
            pltpu.VMEM((len(mxu_q), D // 2, G), U32),
            pltpu.VMEM((len(mxu_o), G // 2, D), U32),
            pltpu.VMEM((D // 2, FM), U32),
            pltpu.VMEM(((FM - N2 * Dh) // 2, D), U32),
            pltpu.VMEM((8, Hq * Dh), F32),
            pltpu.VMEM((8, FM), F32),
            pltpu.VMEM((8, Dh), F32),
            pltpu.VMEM((8, D), F32),
            pltpu.VMEM((Hkv, 8, S), BF16),
            pltpu.VMEM((Hkv, 8, Dh), F32),
            pltpu.VMEM((8, Dh), F32),
            pltpu.VMEM((8, Dh), F32),
            pltpu.VMEM((1, D, Dh), F32),
            pltpu.VMEM((1, N2 * Dh, Dh), F32),
            pltpu.VMEM((2, G, Dh), F32),
            pltpu.VMEM((Hkv, 8, SW), F32),
            pltpu.VMEM((3, G, Dh), F32),
            pltpu.VMEM((8, Dh), jnp.int32),
        ],
        compiler_params=pltpu.CompilerParams(vmem_limit_bytes=120 * 1024 * 1024),
    )(A_x.reshape(B, D), A_k_cache, A_v_cache, A_wq, A_wo, B_w1, B_w2)
    return out.reshape(B, Sq, D)
```
